```python
import jax
import jax.numpy as jnp

def _softmax(x, axis=-1):
    return jax.nn.softmax(x, axis=axis)

def _gelu(x):
    return jax.nn.gelu(x, approximate=True)

def _silu(x):
    return jax.nn.silu(x)

def _sigmoid(x):
    return jax.nn.sigmoid(x)

def _layernorm(x, axis=-1, eps=1e-05):
    m = jnp.mean(x, axis=axis, keepdims=True)
    v = jnp.var(x, axis=axis, keepdims=True)
    return (x - m) / jnp.sqrt(v + eps)

def _scatter_add(tgt, idx, src, axis=0):
    return tgt.at[idx].add(src)

def _segment_sum(src, seg, n):
    return jax.ops.segment_sum(src, seg, n)

class _Rng:

    def __init__(self, key):
        self._k = key

    def _next(self):
        self._k, sub = jax.random.split(self._k)
        return sub

    def normal(self, shape):
        return jax.random.normal(self._next(), shape, dtype=jnp.bfloat16)

    def randint(self, lo, hi, shape):
        return jax.random.randint(self._next(), shape, lo, hi, dtype=jnp.int32)

    def uniform(self, shape, lo=0.0, hi=1.0):
        return jax.random.uniform(self._next(), shape, jnp.bfloat16, lo, hi)

    def permutation(self, n):
        return jax.random.permutation(self._next(), n)
kernel_name = 'adaLN_cond__mha_block_cached__moe_arch_mod__prompt'

def setup_inputs():
    _rng = _Rng(jax.random.key(int.from_bytes(__import__("os").urandom(4), "little")))
    _w = lambda a: (lambda t: t.astype(jnp.bfloat16) if jnp.issubdtype(t.dtype, jnp.floating) else t)(jnp.asarray(a))

    def _A_setup():
        B, Sq, D = (1, 2048, 1024)
        H, Sk, Dh = (32, 2048, 128)
        return {'x': _w((lambda *s: _rng.normal(s) * 0.05)(B, Sq, D)), 'k_cache': _w((lambda *s: _rng.normal(s) * 0.05)(B, H, Sk, Dh)), 'v_cache': _w((lambda *s: _rng.normal(s) * 0.05)(B, H, Sk, Dh)), 'wq': _w((lambda *s: _rng.normal(s) * 0.05)(D, H * Dh) * D ** (-0.5)), 'wo': _w((lambda *s: _rng.normal(s) * 0.05)(H * Dh, D) * (H * Dh) ** (-0.5))}
    _A_in = _A_setup()

    def _B_setup():
        B, S, D, F, C = (1, 2048, 1024, 3584, 2)
        return {'x': _w((lambda *s: _rng.normal(s) * 0.05)(B, S, D)), 'w_r': _w((lambda *s: _rng.normal(s) * 0.05)(D)), 'w_gate': _w((lambda *s: _rng.normal(s) * 0.05)(D, F)), 'w_up': _w((lambda *s: _rng.normal(s) * 0.05)(D, F)), 'w_down': _w((lambda *s: _rng.normal(s) * 0.05)(F, D))}
    _B_in = _B_setup()
    return {'A_x': _A_in['x'], 'A_k_cache': _A_in['k_cache'], 'A_v_cache': _A_in['v_cache'], 'A_wq': _A_in['wq'], 'A_wo': _A_in['wo'], 'B_x': _B_in['x'], 'B_w_r': _B_in['w_r'], 'B_w_gate': _B_in['w_gate'], 'B_w_up': _B_in['w_up'], 'B_w_down': _B_in['w_down'], 'c': _w((lambda *s: _rng.normal(s) * 0.05)(1, 1024)), 'w_mod': _w((lambda *s: _rng.normal(s) * 0.05)(1024, 6 * 1024) * 1024 ** (-0.5))}

def reference(A_x, A_k_cache, A_v_cache, A_wq, A_wo, B_x, B_w_r, B_w_gate, B_w_up, B_w_down, c, w_mod):

    def _A_ref(x, k_cache, v_cache, wq, wo):
        B, Sq, D = x.shape
        H, Dh = (32, 128)
        q = (lambda x, *d: x.transpose(*d))((x @ wq).reshape(B, Sq, H, Dh), 0, 2, 1, 3)
        scores = jnp.einsum('bhqd,bhkd->bhqk', q, k_cache) * Dh ** (-0.5)
        p = _softmax(scores, axis=-1)
        o = jnp.einsum('bhqk,bhkd->bhqd', p, v_cache)
        return (lambda x, *d: x.transpose(*d))(o, 0, 2, 1, 3).reshape(B, Sq, H * Dh) @ wo

    def _B_ref(x, w_r, w_gate, w_up, w_down):
        B, S, D = x.shape
        C = 2
        r = x @ w_r
        idx = jnp.argsort(-r, axis=-1)[:, :C]
        idx_e = jnp.repeat(idx.reshape(B, C, 1), D, axis=2)
        x_sel = jnp.take_along_axis(x, idx_e, axis=1)
        g = _silu(x_sel @ w_gate)
        u = x_sel @ w_up
        y = g * u @ w_down
        r_sel = _sigmoid(jnp.take_along_axis(r, idx, axis=1))
        y = y * r_sel.reshape(B, C, 1)
        b_off = (jnp.arange(B) * S).reshape(B, 1)
        flat_idx = (idx + b_off).reshape(B * C)
        zero = (x * 0.0).reshape(B * S, D)
        upd = _scatter_add(zero, flat_idx, y.reshape(B * C, D), axis=0)
        return x + upd.reshape(B, S, D)
    x = A_x
    mod = (_silu(c) @ w_mod).reshape(c.shape[0], 6, 1, -1)
    sa, ca, ga, sb, cb, gb = (mod[:, 0].copy(), mod[:, 1].copy(), mod[:, 2].copy(), mod[:, 3].copy(), mod[:, 4].copy(), mod[:, 5].copy())
    h = _layernorm(x, axis=-1) * (1 + ca) + sa
    x = x + ga * _A_ref(h, A_k_cache, A_v_cache, A_wq, A_wo)
    h = _layernorm(x, axis=-1) * (1 + cb) + sb
    x = x + gb * _B_ref(h, B_w_r, B_w_gate, B_w_up, B_w_down)
    return x
```

```python
import functools
import jax
import jax.numpy as jnp
from jax import lax
import jax.experimental.pallas as pl
import jax.experimental.pallas.tpu as pltpu

S = 2048
D = 1024
H = 32
DH = 128
F = 3584
EPS = 1e-5
LOG2E = 1.4426950408889634
TQ = 512
RG = 8
NCHAIN = 1
LINK = 15
RB = 256


def _ln(x):
    m = jnp.mean(x, axis=-1, keepdims=True)
    xc = x - m
    v = jnp.mean(xc * xc, axis=-1, keepdims=True)
    return xc * lax.rsqrt(v + EPS)


def _kernel(x_ref, k_ref, v_ref, wq0_ref, wq_ref, wo_ref, wr_ref, wg_ref, wu_ref, wd_ref, c_ref, wm_ref,
            o_ref, mod_ref, h_ref, h2_ref, acc_ref, q_ref, r_ref, s_ref, p_ref, m_ref, il_ref):
    hd = pl.program_id(0)

    @pl.when(hd == 0)
    def _():
        c = c_ref[...].astype(jnp.float32)
        sc = (c * jax.nn.sigmoid(c)).astype(jnp.bfloat16)
        sc8 = jnp.broadcast_to(sc, (8, D))
        mod_ref[...] = jnp.dot(sc8, wm_ref[...], preferred_element_type=jnp.float32)
        sa = mod_ref[0:1, 0:D]
        ca = mod_ref[0:1, D:2 * D]

        def body(i, _):
            rows = pl.ds(pl.multiple_of(i * RB, RB), RB)
            x = x_ref[rows, :].astype(jnp.float32)
            hrows = pl.ds(pl.multiple_of(i * (RB // 2), RB // 2), RB // 2)
            h_ref[hrows, :] = pltpu.bitcast((_ln(x) * (1.0 + ca) + sa).astype(jnp.bfloat16), jnp.uint32)
            acc_ref[rows, :] = jnp.zeros((RB, D), jnp.float32)
            s_ref[i % 2, 0:8, 0:128] = jnp.zeros((8, 128), jnp.float32)
            p_ref[i % 2, 0:16, 0:128] = jnp.zeros((16, 128), jnp.bfloat16)
            m_ref[i % 2, 0:8, 0:128] = jnp.zeros((8, 128), jnp.float32)
            il_ref[i % 2, 0:8, 0:128] = jnp.zeros((8, 128), jnp.float32)
            return 0
        lax.fori_loop(0, S // RB, body, 0)

    def qproj(w_ref):
        hb = pltpu.bitcast(h_ref[...], jnp.bfloat16)
        q = jnp.dot(hb, w_ref[...], preferred_element_type=jnp.float32)
        return pltpu.bitcast((q * (DH ** -0.5 * LOG2E)).astype(jnp.bfloat16), jnp.uint32)

    @pl.when(hd == 0)
    def _():
        q_ref[...] = qproj(wq0_ref)

    NQ = S // TQ

    def qk(j):
        qb = pltpu.bitcast(q_ref[j * TQ // 2:(j + 1) * TQ // 2, :], jnp.bfloat16)
        s = lax.dot_general(qb, k_ref[...], (((1,), (1,)), ((), ())), preferred_element_type=jnp.float32)
        s_ref[j % 2] = s
        m_ref[j % 2] = jnp.broadcast_to(jnp.max(s, axis=-1, keepdims=True), (TQ, 128))

    def sm(j):
        toks = [None] * NCHAIN
        for gi, r in enumerate(range(0, TQ, RG)):
            m = m_ref[j % 2, r:r + RG, :]
            tok = toks[gi % NCHAIN]
            if tok is not None:
                m = jnp.where(tok < 0.0, 0.0, m)
            acc = None
            ps = []
            for c in range(S // 128):
                pc = jnp.exp2(s_ref[j % 2, r:r + RG, c * 128:(c + 1) * 128] - m)
                ps.append(pc)
                acc = pc if acc is None else acc + pc
                if c == LINK:
                    toks[gi % NCHAIN] = acc
            p_ref[j % 2, r:r + RG, :] = jnp.concatenate(ps, axis=1).astype(jnp.bfloat16)
            l = jnp.broadcast_to(jnp.sum(acc, axis=-1, keepdims=True), (RG, 128))
            rl = pl.reciprocal(l, approx=True)
            rl = rl * (2.0 - l * rl)
            il_ref[j % 2, r:r + RG, :] = rl

    def pv(j, l):
        p = p_ref[j % 2]
        o = jnp.dot(p, v_ref[...], preferred_element_type=jnp.float32)
        o = (o * il_ref[j % 2]).astype(jnp.bfloat16)
        acc_ref[j * TQ:(j + 1) * TQ, :] += jnp.dot(o, wo_ref[...], preferred_element_type=jnp.float32)

    l_list = [None] * NQ
    qk(0)
    l_list[0] = sm(0)
    qn = qproj(wq_ref)
    for t in range(1, NQ):
        qk(t)
        l_list[t] = sm(t)
        pv(t - 1, l_list[t - 1])
    pv(NQ - 1, l_list[NQ - 1])
    q_ref[...] = qn

    @pl.when(hd == H - 1)
    def _():
        ga = mod_ref[0:1, 2 * D:3 * D]
        sb = mod_ref[0:1, 3 * D:4 * D]
        cb = mod_ref[0:1, 4 * D:5 * D]
        gb = mod_ref[0:1, 5 * D:6 * D]
        wr = wr_ref[...].astype(jnp.float32)

        def body(i, _):
            rows = pl.ds(pl.multiple_of(i * RB, RB), RB)
            x1 = x_ref[rows, :].astype(jnp.float32) + ga * acc_ref[rows, :]
            h2 = _ln(x1) * (1.0 + cb) + sb
            h2b = h2.astype(jnp.bfloat16)
            h2_ref[rows, :] = h2b
            acc_ref[rows, :] = x1
            r = jnp.sum(h2b.astype(jnp.float32) * wr, axis=-1, keepdims=True)
            r_ref[rows, :] = r.astype(jnp.bfloat16).astype(jnp.float32)
            o_ref[rows, :] = (x1 + gb * h2).astype(o_ref.dtype)
            return 0
        lax.fori_loop(0, S // RB, body, 0)

        r = r_ref[...]
        ids = lax.broadcasted_iota(jnp.int32, (S, 1), 0)
        m1 = jnp.max(r)
        i1 = jnp.min(jnp.where(r == m1, ids, S))
        r2 = jnp.where(ids == i1, -jnp.inf, r)
        m2 = jnp.max(r2)
        i2 = jnp.min(jnp.where(r2 == m2, ids, S))
        i1 = jnp.clip(i1, 0, S - 1)
        i2 = jnp.clip(i2, 0, S - 1)
        sub = lax.broadcasted_iota(jnp.int32, (16, D), 0)

        def pick(idx):
            base = pl.multiple_of((idx // 16) * 16, 16)
            blk = h2_ref[pl.ds(base, 16), :].astype(jnp.float32)
            return jnp.sum(jnp.where(sub == idx - base, blk, 0.0), axis=0, keepdims=True)
        xs1 = pick(i1)
        xs2 = pick(i2)
        sub8 = lax.broadcasted_iota(jnp.int32, (8, D), 0)
        xs = jnp.where(sub8 == 0, xs1, jnp.where(sub8 == 1, xs2, 0.0)).astype(jnp.bfloat16)
        g = jnp.dot(xs, wg_ref[...], preferred_element_type=jnp.float32)
        u = jnp.dot(xs, wu_ref[...], preferred_element_type=jnp.float32)
        a = (g * jax.nn.sigmoid(g) * u).astype(jnp.bfloat16)
        y = jnp.dot(a, wd_ref[...], preferred_element_type=jnp.float32)
        y1 = y[0:1, :] * jax.nn.sigmoid(jnp.full((1, D), m1, jnp.float32))
        y2 = y[1:2, :] * jax.nn.sigmoid(jnp.full((1, D), m2, jnp.float32))

        def fix(idx, hrow, yrow):
            base = pl.multiple_of((idx // 16) * 16, 16)
            x1 = acc_ref[pl.ds(base, 16), :]
            new = (x1 + gb * (hrow + yrow)).astype(o_ref.dtype)
            old = o_ref[pl.ds(base, 16), :]
            o_ref[pl.ds(base, 16), :] = jnp.where(sub == idx - base, new.astype(jnp.float32), old.astype(jnp.float32)).astype(o_ref.dtype)
        fix(i1, xs1, y1)
        fix(i2, xs2, y2)


@jax.jit
def pallas_adaLN_cond__mha_block_cached__moe_arch_mod__prompt_kernel(
    A_x, A_k_cache, A_v_cache, A_wq, A_wo, B_x, B_w_r, B_w_gate, B_w_up, B_w_down, c, w_mod,
):
    x = A_x.reshape(S, D)
    k = A_k_cache.reshape(H, S, DH)
    v = A_v_cache.reshape(H, S, DH)
    wr = B_w_r.reshape(1, D)
    const = lambda shape: pl.BlockSpec(shape, lambda h: (0,) * len(shape), pipeline_mode=pl.Buffered(1))
    out = pl.pallas_call(
        _kernel,
        grid=(H,),
        in_specs=[
            const((S, D)),
            pl.BlockSpec((None, S, DH), lambda h: (h, 0, 0)),
            pl.BlockSpec((None, S, DH), lambda h: (h, 0, 0)),
            pl.BlockSpec((D, DH), lambda h: (0, 0)),
            pl.BlockSpec((D, DH), lambda h: (0, jnp.minimum(h + 1, H - 1))),
            pl.BlockSpec((DH, D), lambda h: (h, 0)),
            const((1, D)),
            const((D, F)),
            const((D, F)),
            const((F, D)),
            const((1, D)),
            const((D, 6 * D)),
        ],
        out_specs=pl.BlockSpec((S, D), lambda h: (0, 0)),
        out_shape=jax.ShapeDtypeStruct((S, D), jnp.bfloat16),
        scratch_shapes=[
            pltpu.VMEM((8, 6 * D), jnp.float32),
            pltpu.VMEM((S // 2, D), jnp.uint32),
            pltpu.VMEM((S, D), jnp.bfloat16),
            pltpu.VMEM((S, D), jnp.float32),
            pltpu.VMEM((S // 2, DH), jnp.uint32),
            pltpu.VMEM((S, 1), jnp.float32),
            pltpu.VMEM((2, TQ, S), jnp.float32),
            pltpu.VMEM((2, TQ, S), jnp.bfloat16),
            pltpu.VMEM((2, TQ, 128), jnp.float32),
            pltpu.VMEM((2, TQ, 128), jnp.float32),
        ],
        compiler_params=pltpu.CompilerParams(
            dimension_semantics=("arbitrary",),
            vmem_limit_bytes=100 * 1024 * 1024,
        ),
    )(x, k, v, A_wq, A_wq, A_wo, wr, B_w_gate, B_w_up, B_w_down, c, w_mod)
    return out.reshape(1, S, D)
```

```python
import os, json
import jax
import jax.numpy as jnp
from jax import lax
import jax.experimental.pallas as pl
import jax.experimental.pallas.tpu as pltpu

S = 2048
D = 1024
H = 32
DH = 128
F = 3584
EPS = 1e-5
LOG2E = 1.4426950408889634
TQ = 512
NQB = S // TQ
HPS = 4
NHG = H // HPS
NSTEP = NQB * NHG
CH = TQ // NHG
NFP = 4
NMC = 4
MCW = 2 * D // NMC
_P = dict(PADS=[5, 5, 5, 2], PADS0=[5, 5, 5, 5], SCOPE=0)
_P.update(json.loads(os.environ.get('KP', '{}')))

f32 = jnp.float32
bf16 = jnp.bfloat16
u32 = jnp.uint32


class _Scope:
    def __init__(self):
        self.cur = None

    def __call__(self, name):
        if not _P['SCOPE']:
            return
        if self.cur is not None:
            self.cur.__exit__(None, None, None)
            self.cur = None
        if name:
            self.cur = jax.named_scope(name)
            self.cur.__enter__()


def _rb(x):
    return x.astype(bf16).astype(f32)


def _ln(x):
    m = jnp.mean(x, axis=-1, keepdims=True)
    mb = _rb(m)
    xc = x - mb
    dm = m - mb
    v = jnp.maximum(jnp.mean(xc * xc, axis=-1, keepdims=True) - dm * dm, 0.0)
    sd = _rb(jnp.sqrt(_rb(_rb(v) + EPS)))
    return xc * (1.0 / sd)


def _kernel(x_hbm, k_hbm, v_hbm, wq_hbm, wo_hbm, wr_hbm, wg_hbm, wu_hbm, wd_hbm, c_hbm, wm_hbm,
            o_hbm,
            xb, kb32, vb32, wqb, wob, wrb, wgb, wub, wdb, cb_, wmb,
            mod_ref, h_ref, acc_ref, ob, fixb, s0_ref, s1_ref, p0_ref, p1_ref, m_ref,
            l0_ref, l1_ref, l2_ref, l3_ref, top_ref, topi_ref, z_ref,
            sem_s, sem_x, sem_wm, sem_k, sem_v, sem_w, sem_0, sem_f, sem_o):
    scope = _Scope()
    kb, vb, wqb, wob, wgb, wub, wdb, wmb, h_ref, p0_ref, p1_ref = (
        r.bitcast(bf16) for r in (kb32, vb32, wqb, wob, wgb, wub, wdb, wmb, h_ref, p0_ref, p1_ref))
    X0 = TQ + 2 * CH
    X1 = X0 + TQ

    cp_c = pltpu.make_async_copy(c_hbm, cb_, sem_s.at[0])
    cp_wr = pltpu.make_async_copy(wr_hbm, wrb, sem_s.at[1])
    cp_x0 = pltpu.make_async_copy(x_hbm.at[pl.ds(0, TQ)], xb.at[pl.ds(0, TQ)], sem_x.at[0])
    cp_x0b = pltpu.make_async_copy(x_hbm.at[pl.ds(TQ, X0 - TQ)], xb.at[pl.ds(TQ, X0 - TQ)], sem_x.at[3])

    cp_x1 = pltpu.make_async_copy(x_hbm.at[pl.ds(X0, TQ)], xb.at[pl.ds(X0, TQ)], sem_x.at[1])
    cp_x2 = pltpu.make_async_copy(x_hbm.at[pl.ds(X1, S - X1)], xb.at[pl.ds(X1, S - X1)], sem_x.at[2])

    def cp_wm(i):
        return pltpu.make_async_copy(wm_hbm.at[:, pl.ds(i * MCW, MCW)], wmb.at[:, pl.ds(i * MCW, MCW)], sem_wm.at[i])

    def cp_wmr(i):
        cols = pl.ds(pl.multiple_of(i * D, D), D)
        return pltpu.make_async_copy(wm_hbm.at[:, cols], wmb.at[:, cols], sem_wm.at[NMC - 2 + i])

    def cp_k(g, slot):
        return pltpu.make_async_copy(k_hbm.at[g], kb.at[slot], sem_k.at[slot])

    def cp_v(g, slot):
        return pltpu.make_async_copy(v_hbm.at[g], vb.at[slot], sem_v.at[slot])

    def cp_wq(g):
        cols = pl.ds(pl.multiple_of(g * (HPS * DH), HPS * DH), HPS * DH)
        return pltpu.make_async_copy(wq_hbm.at[:, cols], wqb.at[g], sem_w.at[0])

    def cp_wo(g):
        return pltpu.make_async_copy(wo_hbm.at[g], wob.at[g], sem_w.at[1])

    cp0_wq = [pltpu.make_async_copy(wq_hbm.at[:, pl.ds(j * DH, DH)], wqb.at[0, :, pl.ds(j * DH, DH)], sem_0.at[j])
              for j in range(HPS)]
    cp0_k = [pltpu.make_async_copy(k_hbm.at[0, j], kb.at[0, j], sem_0.at[HPS + j]) for j in range(HPS)]
    cp0_v = [pltpu.make_async_copy(v_hbm.at[0, j], vb.at[0, j], sem_0.at[2 * HPS + j]) for j in range(HPS)]
    cp0_wo = pltpu.make_async_copy(wo_hbm.at[0], wob.at[0], sem_0.at[3 * HPS])

    cp_ffn = [pltpu.make_async_copy(wg_hbm, wgb, sem_f.at[0]),
              pltpu.make_async_copy(wu_hbm, wub, sem_f.at[1]),
              pltpu.make_async_copy(wd_hbm, wdb, sem_f.at[2])]

    def start_ffn_piece(t):
        ra, rb_ = D // NFP, F // NFP
        rows = pl.ds(pl.multiple_of(t * ra, ra), ra)
        pltpu.make_async_copy(wg_hbm.at[rows], wgb.at[rows], sem_f.at[0]).start()
        pltpu.make_async_copy(wu_hbm.at[rows], wub.at[rows], sem_f.at[1]).start()
        rows = pl.ds(pl.multiple_of(t * rb_, 16), rb_)
        pltpu.make_async_copy(wd_hbm.at[rows], wdb.at[rows], sem_f.at[2]).start()

    def cp_out(qb):
        rows = pl.ds(pl.multiple_of(qb * TQ, TQ), TQ)
        return pltpu.make_async_copy(ob.at[rows], o_hbm.at[rows], sem_o.at[qb])

    scope('pro_zero')
    cp_c.start()
    cp_x0.start()
    for i in range(NMC):
        cp_wm(i).start()
    for cp in (cp0_wq[0], cp0_k[0], cp0_wq[1], cp0_k[1], cp0_v[0], cp0_wq[2], cp0_k[2], cp0_v[1],
               cp0_wq[3], cp0_k[3], cp_x0b, cp0_v[2], cp0_wo, cp0_v[3], cp_wr,
               cp_wq(1), cp_k(1, 1), cp_v(1, 1), cp_wo(1)):
        cp.start()

    def zbody(i, _):
        rows = pl.ds(pl.multiple_of(i * 256, 256), 256)
        acc_ref[rows, :] = jnp.zeros((256, D), f32)
        z_ref[i] = 0
        return 0
    lax.fori_loop(0, S // 256, zbody, 0)
    mod_ref[...] = jnp.zeros(mod_ref.shape, f32)
    top_ref[...] = jnp.full(top_ref.shape, -jnp.inf, f32)
    topi_ref[0] = jnp.zeros((8, 128), jnp.int32)
    topi_ref[1] = jnp.ones((8, 128), jnp.int32)

    def bc(lo, n):
        p = mod_ref[:, lo * D:(lo + 1) * D]
        return p if n == 8 else jnp.concatenate([p] * (n // 8), axis=0)

    def tie(x, tok):
        if tok is None:
            return x
        return jnp.concatenate([jnp.where(tok < 0.0, 0.0, x[:, 0:128]), x[:, 128:]], axis=1)

    scope('pro_ln')
    cp_x0.wait()

    def nbody(i, _):
        rows = pl.ds(pl.multiple_of(i * 128, 128), 128)
        s1_ref[0, rows, 0:D] = _ln(xb[rows, :].astype(f32))
        return 0
    lax.fori_loop(0, TQ // 128, nbody, 0)

    scope('pro_mod')
    cp_c.wait()

    def silu_c():
        c = cb_[...].astype(f32)
        sc = (c * jax.nn.sigmoid(c)).astype(bf16)
        return jnp.broadcast_to(sc, (8, D))

    def mod_part(lo, width, plus_one):
        md = _rb(jnp.dot(silu_c(), wmb[:, lo:lo + width], preferred_element_type=f32))
        if plus_one:
            md = _rb(1.0 + md)
        mod_ref[:, lo:lo + width] = md

    for i in range(NMC):
        cp_wm(i).wait()
        mod_part(i * MCW, MCW, i * MCW >= D)

    def ln1_rows(r0, n, tok=None):
        x = tie(xb[pl.ds(r0, n), :].astype(f32), tok)
        h = _ln(x) * bc(1, n) + bc(0, n)
        h_ref[pl.ds(pl.multiple_of(r0, 16), n), :] = h.astype(bf16)
        return jnp.abs(h[:, 0:128])

    def fin_vals(r0, n, tok=None):
        x = tie(xb[pl.ds(r0, n), :].astype(f32), tok)
        x1 = x + bc(2, n) * acc_ref[pl.ds(r0, n), :]
        h2 = _ln(x1) * bc(4, n) + bc(3, n)
        return x1, h2

    def fin_rows(r0, d0, n, valid, top, tok=None):
        x1, h2 = fin_vals(r0, n, tok)
        ob[pl.ds(d0, n), :] = (x1 + bc(5, n) * h2).astype(bf16)
        r = _rb(jnp.sum(h2 * bc(6, n), axis=-1, keepdims=True))
        r = jnp.broadcast_to(r, (n, 128))
        tok = jnp.abs(r)
        if valid is not None:
            r = jnp.where(valid, r, -jnp.inf)
        b1, i1, b2, i2 = top
        sub = lax.broadcasted_iota(jnp.int32, (8, 128), 0)
        for g in range(n // 8):
            rg = r[g * 8:(g + 1) * 8, :]
            ids = sub + (r0 + g * 8)
            gt1 = rg > b1
            gt2 = rg > b2
            b2 = jnp.where(gt1, b1, jnp.where(gt2, rg, b2))
            i2 = jnp.where(gt1, i1, jnp.where(gt2, ids, i2))
            b1 = jnp.where(gt1, rg, b1)
            i1 = jnp.where(gt1, ids, i1)
        return (b1, i1, b2, i2), tok

    s_refs = (s0_ref, s1_ref)
    p_refs = (p0_ref, p1_ref)
    l_refs = (l0_ref, l1_ref, l2_ref, l3_ref)

    def attend(t, first):
        qb = t // NHG
        hg = t % NHG
        slot = t % 2
        pads = _P['PADS0'] if first else _P['PADS']
        z = z_ref[0]
        z2 = z_ref[1]
        zp = pl.multiple_of(z * 16, 16)
        arows = pl.ds(pl.multiple_of(qb * TQ, TQ), TQ)
        rlv = {}
        early = [None]

        def qp(j):
            if first and j == 1:
                d0 = jnp.dot(h_ref[arows, 0:512], wqb[hg, 0:512, j * DH:(j + 1) * DH], preferred_element_type=f32)
                early[0] = jnp.abs(d0[0:16])
                q = d0 + jnp.dot(h_ref[arows, 512:], wqb[hg, 512:, j * DH:(j + 1) * DH], preferred_element_type=f32)
            else:
                q = jnp.dot(h_ref[arows, :], wqb[hg, :, j * DH:(j + 1) * DH], preferred_element_type=f32)
            return q * (DH ** -0.5 * LOG2E)

        def qk(j, q):
            s = lax.dot_general(q.astype(bf16), pltpu.bitcast(kb32[slot, j], bf16), (((1,), (1,)), ((), ())),
                                preferred_element_type=f32)
            s_refs[j % 2][z] = s
            pm = s[:, 0:128]
            for c in range(1, S // 128):
                pm = jnp.maximum(pm, s[:, c * 128:(c + 1) * 128])
            m_ref[z, j] = jnp.broadcast_to(jnp.max(pm, axis=-1, keepdims=True), (TQ, 128))

        def sm(j, tok=None):
            R, W = 16, S // 2
            sref = s_refs[j % 2]
            zs = z_ref[3 + j]
            for r in range(0, TQ, R):
                m = m_ref[zs, j, r:r + R, :]
                acc = None
                for hf in range(2):
                    mm = m if tok is None else jnp.where(tok < 0.0, 0.0, m)
                    ps = []
                    for c in range(W // 128):
                        c0 = hf * W + c * 128
                        pc = jnp.exp2(sref[zs, r:r + R, c0:c0 + 128] - mm)
                        ps.append(pc)
                        acc = pc if acc is None else acc + pc
                    tok = acc
                    for _ in range(pads[j]):
                        tok = tok + tok
                    p_refs[j % 2][pl.ds(zp + r, R), hf * W:(hf + 1) * W] = jnp.concatenate(ps, axis=1).astype(bf16)
                l_refs[j][z, r:r + R, :] = acc

        def pv(j):
            vv = pltpu.bitcast(vb32[slot, j], bf16)
            pj = p_refs[j % 2]
            lp = l_refs[j][z2]
            d0 = jnp.dot(pj[pl.ds(zp, TQ), 0:512], vv[0:512], preferred_element_type=f32)
            o = d0 + jnp.dot(pj[pl.ds(zp, TQ), 512:], vv[512:], preferred_element_type=f32)
            early[0] = jnp.abs(d0[0:16])
            if j == 3:
                lp = jnp.maximum(lp, jnp.minimum(d0, 0.0))
            l = jnp.broadcast_to(jnp.sum(lp, axis=-1, keepdims=True), (TQ, 128))
            rl = pl.reciprocal(l, approx=True)
            rl = rl * (2.0 - l * rl)
            rlv[j] = rl
            return o * rl

        def qtie(q, j):
            return jnp.where(rlv[j] < 0.0, 0.0, q)

        def op(j, oa, ob_):
            o = jnp.concatenate([oa, ob_], axis=1).astype(bf16)
            acc_ref[arows, :] += jnp.dot(o, wob[hg, j * DH:(j + 2) * DH, :], preferred_element_type=f32)

        def wait(*cps):
            if first:
                for cp in cps:
                    cp.wait()

        ftok = None
        if first:
            wait(cp0_wq[0])
            h_ref[0:TQ, :] = (s1_ref[0, :, 0:D] * bc(1, TQ) + bc(0, TQ)).astype(bf16)
        else:
            valid = t >= NHG
            fsrc = pl.multiple_of(jnp.maximum(t - NHG, 0) * CH, CH)
            fdst = pl.multiple_of(jnp.where(valid, fsrc, S), CH)
            top = (top_ref[0], topi_ref[0], top_ref[1], topi_ref[1])
            for g in range(CH // 16):
                top, ftok = fin_rows(fsrc + g * 16, fdst + g * 16, 16, valid, top, ftok)
            top_ref[0], topi_ref[0], top_ref[1], topi_ref[1] = top
            ftok = jnp.minimum(ftok[0:8], ftok[8:16])
            ftok = jnp.concatenate([ftok, ftok], axis=0)

        if not first:
            cp_k((t + 1) % NHG, 1 - slot).start()
            cp_v((t + 1) % NHG, 1 - slot).start()
        q0 = qp(0)
        wait(cp0_k[0])
        qk(0, q0)
        wait(cp0_wq[1], cp0_k[1], cp0_v[0], cp0_wq[2])
        q1 = qp(1)
        sm(0, early[0] if first else ftok)
        qk(1, q1)
        sm(1)
        o0 = pv(0)
        q2 = qtie(qp(2), 0)
        wait(cp0_k[2], cp0_v[1], cp0_wq[3], cp0_k[3], cp_x0b)
        qk(2, q2)
        sm(2)
        o1 = pv(1)
        q3 = qp(3)
        qk(3, qtie(q3, 1))
        l0 = pl.multiple_of(jnp.minimum(t + NHG, NSTEP - 1) * CH, CH)
        tok = jnp.abs(q3[TQ - 16:TQ, :])
        for g in range(CH // 16):
            tok = ln1_rows(l0 + g * 16, 16, tok)
        wait(cp0_v[2], cp0_wo, cp0_v[3], cp_wr)
        if first:
            o2 = pv(2)
            sm(3, early[0])
        else:
            tok = jnp.minimum(tok[0:8], tok[8:16])
            sm(3, jnp.concatenate([tok, tok], axis=0))
            o2 = pv(2)
        op(0, o0, o1)
        o3 = pv(3)
        op(2, o2, o3)

    scope('step0')
    attend(0, True)
    mod_ref[:, 6 * D:7 * D] = jnp.broadcast_to(wrb[...].astype(f32), (8, D))
    scope(None)

    def step(t, _):
        scope('step_head')
        hg = t % NHG
        slot = t % 2
        cp_k(hg, slot).wait()
        cp_v(hg, slot).wait()

        @pl.when(jnp.logical_or(t <= NHG + NFP, hg == 0))
        def _():
            @pl.when(t < NHG)
            def _():
                cp_wq(hg).wait()
                cp_wo(hg).wait()

                @pl.when(t < NHG - 1)
                def _():
                    cp_wq(hg + 1).start()
                    cp_wo(hg + 1).start()

                @pl.when(t == 1)
                def _():
                    cp_x1.start()

                @pl.when(t == 2)
                def _():
                    cp_x1.wait()

                @pl.when(jnp.logical_and(t >= 2, t < 6))
                def _():
                    cp_wmr(t).start()

                @pl.when(t == 6)
                def _():
                    cp_x2.start()

            @pl.when(t == NHG)
            def _():
                cp_x2.wait()
                for i in range(2, 6):
                    cp_wmr(i).wait()
                mod_part(2 * D, 2 * D, False)
                mod_part(4 * D, D, True)
                mod_part(5 * D, D, False)

            @pl.when(jnp.logical_and(t > NHG, t <= NHG + NFP))
            def _():
                start_ffn_piece(t - NHG - 1)

            @pl.when(t >= 2 * NHG)
            def _():
                cp_out(t // NHG - 2).start()

        scope('step_body')
        attend(t, False)
        scope(None)
        return 0

    lax.fori_loop(1, NSTEP, step, 0)

    scope('epi_fin')
    cp_out(NQB - 2).start()

    def fbody(i, top):
        r0 = pl.multiple_of((NQB - 1) * TQ + i * 128, 128)
        top, _ = fin_rows(r0, r0, 128, None, top)
        return top
    top = lax.fori_loop(0, TQ // 128, fbody, (top_ref[0], topi_ref[0], top_ref[1], topi_ref[1]))
    cp_out(NQB - 1).start()

    scope('epi_ffn')
    cp_k(0, 0).wait()
    cp_v(0, 0).wait()
    for cp in cp_ffn:
        cp.wait()
    vals = jnp.concatenate([top[0], top[2]], axis=0)
    idxs = jnp.concatenate([top[1], top[3]], axis=0)
    m1 = jnp.max(vals, axis=0, keepdims=True)
    i1v = jnp.min(jnp.where(vals == m1, idxs, S - 1), axis=0, keepdims=True)
    vals2 = jnp.where(idxs == i1v, -jnp.inf, vals)
    m2 = jnp.max(vals2, axis=0, keepdims=True)
    i2v = jnp.min(jnp.where(jnp.logical_and(vals2 == m2, idxs != i1v), idxs, S - 1), axis=0, keepdims=True)
    i1 = jnp.clip(i1v[0, 0], 0, S - 1)
    i2 = jnp.clip(i2v[0, 0], 0, S - 1)
    b1 = pl.multiple_of((i1 // 16) * 16, 16)
    b2 = pl.multiple_of((i2 // 16) * 16, 16)

    sub = lax.broadcasted_iota(jnp.int32, (16, D), 0)
    x1a, h2a = fin_vals(b1, 16)
    x1b, h2b = fin_vals(b2, 16)
    xs1 = jnp.sum(jnp.where(sub == i1 - b1, h2a, 0.0), axis=0, keepdims=True)
    xs2 = jnp.sum(jnp.where(sub == i2 - b2, h2b, 0.0), axis=0, keepdims=True)
    sub8 = lax.broadcasted_iota(jnp.int32, (8, D), 0)
    xs = jnp.where(sub8 == 0, xs1, jnp.where(sub8 == 1, xs2, 0.0)).astype(bf16)
    g = jnp.dot(xs, wgb[...], preferred_element_type=f32)
    u = jnp.dot(xs, wub[...], preferred_element_type=f32)
    a = (g * jax.nn.sigmoid(g) * u).astype(bf16)
    y = jnp.dot(a, wdb[...], preferred_element_type=f32)
    y1 = y[0:1, :] * jax.nn.sigmoid(jnp.concatenate([m1] * (D // 128), axis=1))
    y2 = y[1:2, :] * jax.nn.sigmoid(jnp.concatenate([m2] * (D // 128), axis=1))
    gb = bc(5, 16)

    def fixed(base, x1, h2):
        upd = jnp.where(sub == i1 - base, y1, 0.0) + jnp.where(sub == i2 - base, y2, 0.0)
        return (x1 + gb * (h2 + upd)).astype(bf16)
    fixb[0] = fixed(b1, x1a, h2a)
    fixb[1] = fixed(b2, x1b, h2b)

    scope('epi_out')
    for qb in range(NQB):
        cp_out(qb).wait()
    cf1 = pltpu.make_async_copy(fixb.at[0], o_hbm.at[pl.ds(b1, 16)], sem_o.at[NQB])
    cf2 = pltpu.make_async_copy(fixb.at[1], o_hbm.at[pl.ds(b2, 16)], sem_o.at[NQB + 1])
    cf1.start()

    @pl.when(b1 != b2)
    def _():
        cf2.start()
        cf2.wait()
    cf1.wait()
    scope(None)


@jax.jit
def pallas_adaLN_cond__mha_block_cached__moe_arch_mod__prompt_kernel(
    A_x, A_k_cache, A_v_cache, A_wq, A_wo, B_x, B_w_r, B_w_gate, B_w_up, B_w_down, c, w_mod,
):
    x = A_x.reshape(S, D)
    k = A_k_cache.reshape(NHG, HPS, S, DH)
    v = A_v_cache.reshape(NHG, HPS, S, DH)
    wo = A_wo.reshape(NHG, HPS * DH, D)
    wr = B_w_r.reshape(1, D)
    anyspec = pl.BlockSpec(memory_space=pl.ANY)
    out = pl.pallas_call(
        _kernel,
        in_specs=[anyspec] * 11,
        out_specs=anyspec,
        out_shape=jax.ShapeDtypeStruct((S, D), bf16),
        scratch_shapes=[
            pltpu.VMEM((S, D), bf16),
            pltpu.VMEM((2, HPS, S // 2, DH), u32),
            pltpu.VMEM((2, HPS, S // 2, DH), u32),
            pltpu.VMEM((NHG, D // 2, HPS * DH), u32),
            pltpu.VMEM((NHG, HPS * DH // 2, D), u32),
            pltpu.VMEM((1, D), bf16),
            pltpu.VMEM((D // 2, F), u32),
            pltpu.VMEM((D // 2, F), u32),
            pltpu.VMEM((F // 2, D), u32),
            pltpu.VMEM((1, D), bf16),
            pltpu.VMEM((D // 2, 6 * D), u32),
            pltpu.VMEM((8, 7 * D), f32),
            pltpu.VMEM((S // 2, D), u32),
            pltpu.VMEM((S, D), f32),
            pltpu.VMEM((S + CH, D), bf16),
            pltpu.VMEM((2, 16, D), bf16),
            pltpu.VMEM((1, TQ, S), f32),
            pltpu.VMEM((1, TQ, S), f32),
            pltpu.VMEM((TQ // 2, S), u32),
            pltpu.VMEM((TQ // 2, S), u32),
            pltpu.VMEM((1, HPS, TQ, 128), f32),
            pltpu.VMEM((1, TQ, 128), f32),
            pltpu.VMEM((1, TQ, 128), f32),
            pltpu.VMEM((1, TQ, 128), f32),
            pltpu.VMEM((1, TQ, 128), f32),
            pltpu.VMEM((2, 8, 128), f32),
            pltpu.VMEM((2, 8, 128), jnp.int32),
            pltpu.SMEM((8,), jnp.int32),
            pltpu.SemaphoreType.DMA((2,)),
            pltpu.SemaphoreType.DMA((4,)),
            pltpu.SemaphoreType.DMA((NMC + 4,)),
            pltpu.SemaphoreType.DMA((2,)),
            pltpu.SemaphoreType.DMA((2,)),
            pltpu.SemaphoreType.DMA((2,)),
            pltpu.SemaphoreType.DMA((3 * HPS + 1,)),
            pltpu.SemaphoreType.DMA((3,)),
            pltpu.SemaphoreType.DMA((NQB + 2,)),
        ],
        compiler_params=pltpu.CompilerParams(vmem_limit_bytes=110 * 1024 * 1024, disable_bounds_checks=True,
                                             disable_semaphore_checks=True),
    )(x, k, v, A_wq, wo, wr, B_w_gate, B_w_up, B_w_down, c, w_mod)
    return out.reshape(1, S, D)
```

```python
import os, json
import jax
import jax.numpy as jnp
from jax import lax
import jax.experimental.pallas as pl
import jax.experimental.pallas.tpu as pltpu

S = 2048
D = 1024
H = 32
DH = 128
F = 3584
EPS = 1e-5
LOG2E = 1.4426950408889634
TQ = 512
NQB = S // TQ
HPS = 4
NHG = H // HPS
NSTEP = NQB * NHG
CH = TQ // NHG
NFP = 4
NMC = 4
MCW = 2 * D // NMC
_P = dict(PADS=[5, 5, 5, 2], PADS0=[5, 5, 5, 5], SCOPE=0)
_P.update(json.loads(os.environ.get('KP', '{}')))

f32 = jnp.float32
bf16 = jnp.bfloat16
u32 = jnp.uint32


class _Scope:
    def __init__(self):
        self.cur = None

    def __call__(self, name):
        if not _P['SCOPE']:
            return
        if self.cur is not None:
            self.cur.__exit__(None, None, None)
            self.cur = None
        if name:
            self.cur = jax.named_scope(name)
            self.cur.__enter__()


def _rb(x):
    return x.astype(bf16).astype(f32)


def _ln(x):
    m = jnp.mean(x, axis=-1, keepdims=True)
    mb = _rb(m)
    xc = x - mb
    dm = m - mb
    v = jnp.maximum(jnp.mean(xc * xc, axis=-1, keepdims=True) - dm * dm, 0.0)
    sd = _rb(jnp.sqrt(_rb(_rb(v) + EPS)))
    return xc * (1.0 / sd)


def _kernel(x_hbm, k_hbm, v_hbm, wq_hbm, wo_hbm, wr_hbm, wg_hbm, wu_hbm, wd_hbm, c_hbm, wm_hbm,
            o_hbm,
            xb, kb32, vb32, wqb, wob, wgb, wub, wdb, wmb,
            mod_ref, h_ref, acc_ref, ob, fixb, s0_ref, s1_ref, p0_ref, p1_ref, m_ref,
            l0_ref, l1_ref, l2_ref, l3_ref, top_ref, topi_ref, wrb, cb_, z_ref,
            sem_s, sem_x, sem_wm, sem_k, sem_v, sem_w, sem_0, sem_f, sem_o):
    scope = _Scope()
    kb, vb, wqb, wob, wgb, wub, wdb, wmb, h_ref, p0_ref, p1_ref = (
        r.bitcast(bf16) for r in (kb32, vb32, wqb, wob, wgb, wub, wdb, wmb, h_ref, p0_ref, p1_ref))
    X0 = TQ + 2 * CH
    X1 = X0 + TQ

    cp_c = pltpu.make_async_copy(c_hbm, cb_, sem_s.at[0])
    cp_wr = pltpu.make_async_copy(wr_hbm, wrb, sem_s.at[1])
    cp_x0 = pltpu.make_async_copy(x_hbm.at[pl.ds(0, TQ)], xb.at[pl.ds(0, TQ)], sem_x.at[0])
    cp_x0b = pltpu.make_async_copy(x_hbm.at[pl.ds(TQ, X0 - TQ)], xb.at[pl.ds(TQ, X0 - TQ)], sem_x.at[3])

    cp_x1 = pltpu.make_async_copy(x_hbm.at[pl.ds(X0, TQ)], xb.at[pl.ds(X0, TQ)], sem_x.at[1])
    cp_x2 = pltpu.make_async_copy(x_hbm.at[pl.ds(X1, S - X1)], xb.at[pl.ds(X1, S - X1)], sem_x.at[2])

    def cp_wm(i):
        return pltpu.make_async_copy(wm_hbm.at[:, pl.ds(i * MCW, MCW)], wmb.at[:, pl.ds(i * MCW, MCW)], sem_wm.at[i])

    def cp_wmr(i):
        cols = pl.ds(pl.multiple_of(i * D, D), D)
        return pltpu.make_async_copy(wm_hbm.at[:, cols], wmb.at[:, cols], sem_wm.at[NMC - 2 + i])

    def cp_k(g, slot):
        return pltpu.make_async_copy(k_hbm.at[g], kb.at[slot], sem_k.at[slot])

    def cp_v(g, slot):
        return pltpu.make_async_copy(v_hbm.at[g], vb.at[slot], sem_v.at[slot])

    def cp_wq(g):
        cols = pl.ds(pl.multiple_of(g * (HPS * DH), HPS * DH), HPS * DH)
        return pltpu.make_async_copy(wq_hbm.at[:, cols], wqb.at[g], sem_w.at[0])

    def cp_wo(g):
        return pltpu.make_async_copy(wo_hbm.at[g], wob.at[g], sem_w.at[1])

    cp0_wq = [pltpu.make_async_copy(wq_hbm.at[:, pl.ds(j * DH, DH)], wqb.at[0, :, pl.ds(j * DH, DH)], sem_0.at[j])
              for j in range(HPS)]
    cp0_k = [pltpu.make_async_copy(k_hbm.at[0, j], kb.at[0, j], sem_0.at[HPS + j]) for j in range(HPS)]
    cp0_v = [pltpu.make_async_copy(v_hbm.at[0, j], vb.at[0, j], sem_0.at[2 * HPS + j]) for j in range(HPS)]
    cp0_wo = pltpu.make_async_copy(wo_hbm.at[0], wob.at[0], sem_0.at[3 * HPS])

    cp_ffn = [pltpu.make_async_copy(wg_hbm, wgb, sem_f.at[0]),
              pltpu.make_async_copy(wu_hbm, wub, sem_f.at[1]),
              pltpu.make_async_copy(wd_hbm, wdb, sem_f.at[2])]

    def start_ffn_piece(t):
        ra, rb_ = D // NFP, F // NFP
        rows = pl.ds(pl.multiple_of(t * ra, ra), ra)
        pltpu.make_async_copy(wg_hbm.at[rows], wgb.at[rows], sem_f.at[0]).start()
        pltpu.make_async_copy(wu_hbm.at[rows], wub.at[rows], sem_f.at[1]).start()
        rows = pl.ds(pl.multiple_of(t * rb_, 16), rb_)
        pltpu.make_async_copy(wd_hbm.at[rows], wdb.at[rows], sem_f.at[2]).start()

    def cp_out(qb):
        rows = pl.ds(pl.multiple_of(qb * TQ, TQ), TQ)
        return pltpu.make_async_copy(ob.at[rows], o_hbm.at[rows], sem_o.at[qb])

    scope('pro_zero')
    cp_c.start()
    cp_x0.start()
    for i in range(NMC):
        cp_wm(i).start()
    for cp in (cp0_wq[0], cp0_k[0], cp0_wq[1], cp0_k[1], cp0_v[0], cp0_wq[2], cp0_k[2], cp0_v[1],
               cp0_wq[3], cp0_k[3], cp_x0b, cp0_v[2], cp0_wo, cp0_v[3], cp_wr,
               cp_wq(1), cp_k(1, 1), cp_v(1, 1), cp_wo(1)):
        cp.start()

    def zbody(i, _):
        rows = pl.ds(pl.multiple_of(i * 256, 256), 256)
        acc_ref[rows, :] = jnp.zeros((256, D), f32)
        z_ref[i] = 0
        return 0
    lax.fori_loop(0, S // 256, zbody, 0)
    mod_ref[...] = jnp.zeros(mod_ref.shape, f32)
    top_ref[...] = jnp.full(top_ref.shape, -jnp.inf, f32)
    topi_ref[0] = jnp.zeros((8, 128), jnp.int32)
    topi_ref[1] = jnp.ones((8, 128), jnp.int32)

    def bc(lo, n):
        p = mod_ref[:, lo * D:(lo + 1) * D]
        return p if n == 8 else jnp.concatenate([p] * (n // 8), axis=0)

    def tie(x, tok):
        if tok is None:
            return x
        return jnp.concatenate([jnp.where(tok < 0.0, 0.0, x[:, 0:128]), x[:, 128:]], axis=1)

    scope('pro_ln')
    cp_x0.wait()

    def nbody(i, _):
        rows = pl.ds(pl.multiple_of(i * 128, 128), 128)
        s1_ref[0, rows, 0:D] = _ln(xb[rows, :].astype(f32))
        return 0
    lax.fori_loop(0, TQ // 128, nbody, 0)

    scope('pro_mod')
    cp_c.wait()

    def silu_c():
        c = cb_[...].astype(f32)
        sc = (c * jax.nn.sigmoid(c)).astype(bf16)
        return jnp.broadcast_to(sc, (8, D))

    def mod_part(lo, width, plus_one):
        md = _rb(jnp.dot(silu_c(), wmb[:, lo:lo + width], preferred_element_type=f32))
        if plus_one:
            md = _rb(1.0 + md)
        mod_ref[:, lo:lo + width] = md

    for i in range(NMC):
        cp_wm(i).wait()
        mod_part(i * MCW, MCW, i * MCW >= D)

    def ln1_rows(r0, n, tok=None):
        x = tie(xb[pl.ds(r0, n), :].astype(f32), tok)
        h = _ln(x) * bc(1, n) + bc(0, n)
        h_ref[pl.ds(pl.multiple_of(r0, 16), n), :] = h.astype(bf16)
        return jnp.abs(h[:, 0:128])

    def fin_vals(r0, n, tok=None):
        x = tie(xb[pl.ds(r0, n), :].astype(f32), tok)
        x1 = x + bc(2, n) * acc_ref[pl.ds(r0, n), :]
        h2 = _ln(x1) * bc(4, n) + bc(3, n)
        return x1, h2

    def fin_rows(r0, d0, n, valid, top, tok=None):
        x1, h2 = fin_vals(r0, n, tok)
        ob[pl.ds(d0, n), :] = (x1 + bc(5, n) * h2).astype(bf16)
        r = _rb(jnp.sum(h2 * bc(6, n), axis=-1, keepdims=True))
        r = jnp.broadcast_to(r, (n, 128))
        tok = jnp.abs(r)
        if valid is not None:
            r = jnp.where(valid, r, -jnp.inf)
        b1, i1, b2, i2 = top
        sub = lax.broadcasted_iota(jnp.int32, (8, 128), 0)
        for g in range(n // 8):
            rg = r[g * 8:(g + 1) * 8, :]
            ids = sub + (r0 + g * 8)
            gt1 = rg > b1
            gt2 = rg > b2
            b2 = jnp.where(gt1, b1, jnp.where(gt2, rg, b2))
            i2 = jnp.where(gt1, i1, jnp.where(gt2, ids, i2))
            b1 = jnp.where(gt1, rg, b1)
            i1 = jnp.where(gt1, ids, i1)
        return (b1, i1, b2, i2), tok

    s_refs = (s0_ref, s1_ref)
    p_refs = (p0_ref, p1_ref)
    l_refs = (l0_ref, l1_ref, l2_ref, l3_ref)

    def attend(t, first):
        qb = t // NHG
        hg = t % NHG
        slot = t % 2
        pads = _P['PADS0'] if first else _P['PADS']
        z = z_ref[0]
        z2 = z_ref[1]
        zp = pl.multiple_of(z * 16, 16)
        arows = pl.ds(pl.multiple_of(qb * TQ, TQ), TQ)
        rlv = {}
        early = [None]

        r0q = pl.multiple_of(qb * TQ, TQ)

        def qp(j):
            if first and j == 1:
                d0 = jnp.dot(h_ref[arows, 0:512], wqb[hg, 0:512, j * DH:(j + 1) * DH], preferred_element_type=f32)
                early[0] = jnp.abs(d0[0:16])
                q = d0 + jnp.dot(h_ref[arows, 512:], wqb[hg, 512:, j * DH:(j + 1) * DH], preferred_element_type=f32)
            else:
                B = _P.get('BQP', TQ)
                q = jnp.concatenate([
                    jnp.dot(h_ref[pl.ds(r0q + r, B), :], wqb[hg, :, j * DH:(j + 1) * DH], preferred_element_type=f32)
                    for r in range(0, TQ, B)], axis=0)
            return q * (DH ** -0.5 * LOG2E)

        def qk(j, q):
            B = _P.get('BQK', TQ)
            for r in range(0, TQ, B):
                s = lax.dot_general(q[r:r + B].astype(bf16), pltpu.bitcast(kb32[slot, j], bf16), (((1,), (1,)), ((), ())),
                                    preferred_element_type=f32)
                s_refs[j % 2][z, r:r + B, :] = s
                pm = s[:, 0:128]
                for c in range(1, S // 128):
                    pm = jnp.maximum(pm, s[:, c * 128:(c + 1) * 128])
                m_ref[z, j, r:r + B, :] = jnp.broadcast_to(jnp.max(pm, axis=-1, keepdims=True), (B, 128))

        def sm(j, tok=None):
            R, W = 16, S // 2
            sref = s_refs[j % 2]
            zs = z_ref[3 + j]
            for r in range(0, TQ, R):
                m = m_ref[zs, j, r:r + R, :]
                acc = None
                for hf in range(2):
                    mm = m if tok is None else jnp.where(tok < 0.0, 0.0, m)
                    ps = []
                    for c in range(W // 128):
                        c0 = hf * W + c * 128
                        pc = jnp.exp2(sref[zs, r:r + R, c0:c0 + 128] - mm)
                        ps.append(pc)
                        acc = pc if acc is None else acc + pc
                    tok = acc
                    for _ in range(pads[j]):
                        tok = tok + tok
                    p_refs[j % 2][pl.ds(zp + r, R), hf * W:(hf + 1) * W] = jnp.concatenate(ps, axis=1).astype(bf16)
                l_refs[j][z, r:r + R, :] = acc

        def pv(j):
            pj = p_refs[j % 2]
            lp = l_refs[j][z2]
            B = _P.get('BPV', TQ)
            if B == TQ:
                vv = pltpu.bitcast(vb32[slot, j], bf16)
                d0 = jnp.dot(pj[pl.ds(zp, TQ), 0:512], vv[0:512], preferred_element_type=f32)
                o = d0 + jnp.dot(pj[pl.ds(zp, TQ), 512:], vv[512:], preferred_element_type=f32)
            else:
                os_ = [jnp.dot(pj[pl.ds(zp + r, B), :], pltpu.bitcast(vb32[slot, j], bf16), preferred_element_type=f32)
                       for r in range(0, TQ, B)]
                o = jnp.concatenate(os_, axis=0)
                d0 = jnp.concatenate([os_[0]] * (TQ // B), axis=0)
            early[0] = jnp.abs(d0[0:16])
            if j == 3:
                lp = jnp.maximum(lp, jnp.minimum(d0, 0.0))
            l = jnp.broadcast_to(jnp.sum(lp, axis=-1, keepdims=True), (TQ, 128))
            rl = pl.reciprocal(l, approx=True)
            rl = rl * (2.0 - l * rl)
            rlv[j] = rl
            return o * rl

        def qtie(q, j):
            if not _P.get('QTIE', 1):
                return q
            return jnp.where(rlv[j] < 0.0, 0.0, q)

        def op(j, oa, ob_):
            o = jnp.concatenate([oa, ob_], axis=1)
            B = _P.get('BOP', TQ)
            for r in range(0, TQ, B):
                acc_ref[pl.ds(r0q + r, B), :] += jnp.dot(o[r:r + B].astype(bf16), wob[hg, j * DH:(j + 2) * DH, :],
                                                         preferred_element_type=f32)

        def wait(*cps):
            if first:
                for cp in cps:
                    cp.wait()

        ftok = None
        if first:
            wait(cp0_wq[0])
            h_ref[0:TQ, :] = (s1_ref[0, :, 0:D] * bc(1, TQ) + bc(0, TQ)).astype(bf16)
        else:
            valid = t >= NHG
            fsrc = pl.multiple_of(jnp.maximum(t - NHG, 0) * CH, CH)
            fdst = pl.multiple_of(jnp.where(valid, fsrc, S), CH)
            top = (top_ref[0], topi_ref[0], top_ref[1], topi_ref[1])
            for g in range(CH // 16):
                top, ftok = fin_rows(fsrc + g * 16, fdst + g * 16, 16, valid, top, ftok)
            top_ref[0], topi_ref[0], top_ref[1], topi_ref[1] = top
            ftok = jnp.minimum(ftok[0:8], ftok[8:16])
            ftok = jnp.concatenate([ftok, ftok], axis=0)

        if not first:
            cp_k((t + 1) % NHG, 1 - slot).start()
            cp_v((t + 1) % NHG, 1 - slot).start()
        q0 = qp(0)
        wait(cp0_k[0])
        qk(0, q0)
        wait(cp0_wq[1], cp0_k[1], cp0_v[0], cp0_wq[2])
        q1 = qp(1)
        sm(0, early[0] if first else ftok)
        qk(1, q1)
        sm(1)
        o0 = pv(0)
        q2 = qtie(qp(2), 0)
        wait(cp0_k[2], cp0_v[1], cp0_wq[3], cp0_k[3], cp_x0b)
        qk(2, q2)
        sm(2)
        o1 = pv(1)
        q3 = qp(3)
        qk(3, qtie(q3, 1))
        l0 = pl.multiple_of(jnp.minimum(t + NHG, NSTEP - 1) * CH, CH)
        tok = jnp.abs(q3[TQ - 16:TQ, :])
        for g in range(CH // 16):
            tok = ln1_rows(l0 + g * 16, 16, tok)
        wait(cp0_v[2], cp0_wo, cp0_v[3], cp_wr)
        if first:
            o2 = pv(2)
            sm(3, early[0])
        else:
            tok = jnp.minimum(tok[0:8], tok[8:16])
            sm(3, jnp.concatenate([tok, tok], axis=0))
            o2 = pv(2)
        op(0, o0, o1)
        o3 = pv(3)
        op(2, o2, o3)

    scope('step0')
    attend(0, True)
    mod_ref[:, 6 * D:7 * D] = jnp.broadcast_to(wrb[...].astype(f32), (8, D))
    scope(None)

    def step(t, _):
        scope('step_head')
        hg = t % NHG
        slot = t % 2
        cp_k(hg, slot).wait()
        cp_v(hg, slot).wait()

        @pl.when(jnp.logical_or(t <= NHG + NFP, hg == 0))
        def _():
            @pl.when(t < NHG)
            def _():
                cp_wq(hg).wait()
                cp_wo(hg).wait()

                @pl.when(t < NHG - 1)
                def _():
                    cp_wq(hg + 1).start()
                    cp_wo(hg + 1).start()

                @pl.when(t == 1)
                def _():
                    cp_x1.start()

                @pl.when(t == 2)
                def _():
                    cp_x1.wait()

                @pl.when(jnp.logical_and(t >= 2, t < 6))
                def _():
                    cp_wmr(t).start()

                @pl.when(t == 6)
                def _():
                    cp_x2.start()

            @pl.when(t == NHG)
            def _():
                cp_x2.wait()
                for i in range(2, 6):
                    cp_wmr(i).wait()
                mod_part(2 * D, 2 * D, False)
                mod_part(4 * D, D, True)
                mod_part(5 * D, D, False)

            @pl.when(jnp.logical_and(t > NHG, t <= NHG + NFP))
            def _():
                start_ffn_piece(t - NHG - 1)

            @pl.when(t >= 2 * NHG)
            def _():
                cp_out(t // NHG - 2).start()

        scope('step_body')
        attend(t, False)
        scope(None)
        return 0

    lax.fori_loop(1, NSTEP, step, 0)

    scope('epi_fin')
    cp_out(NQB - 2).start()

    def fbody(i, top):
        r0 = pl.multiple_of((NQB - 1) * TQ + i * 128, 128)
        top, _ = fin_rows(r0, r0, 128, None, top)
        return top
    top = lax.fori_loop(0, TQ // 128, fbody, (top_ref[0], topi_ref[0], top_ref[1], topi_ref[1]))
    cp_out(NQB - 1).start()

    scope('epi_ffn')
    cp_k(0, 0).wait()
    cp_v(0, 0).wait()
    for cp in cp_ffn:
        cp.wait()
    vals = jnp.concatenate([top[0], top[2]], axis=0)
    idxs = jnp.concatenate([top[1], top[3]], axis=0)
    m1 = jnp.max(vals, axis=0, keepdims=True)
    i1v = jnp.min(jnp.where(vals == m1, idxs, S - 1), axis=0, keepdims=True)
    vals2 = jnp.where(idxs == i1v, -jnp.inf, vals)
    m2 = jnp.max(vals2, axis=0, keepdims=True)
    i2v = jnp.min(jnp.where(jnp.logical_and(vals2 == m2, idxs != i1v), idxs, S - 1), axis=0, keepdims=True)
    i1 = jnp.clip(i1v[0, 0], 0, S - 1)
    i2 = jnp.clip(i2v[0, 0], 0, S - 1)
    b1 = pl.multiple_of((i1 // 16) * 16, 16)
    b2 = pl.multiple_of((i2 // 16) * 16, 16)

    sub = lax.broadcasted_iota(jnp.int32, (16, D), 0)
    x1a, h2a = fin_vals(b1, 16)
    x1b, h2b = fin_vals(b2, 16)
    xs1 = jnp.sum(jnp.where(sub == i1 - b1, h2a, 0.0), axis=0, keepdims=True)
    xs2 = jnp.sum(jnp.where(sub == i2 - b2, h2b, 0.0), axis=0, keepdims=True)
    sub8 = lax.broadcasted_iota(jnp.int32, (8, D), 0)
    xs = jnp.where(sub8 == 0, xs1, jnp.where(sub8 == 1, xs2, 0.0)).astype(bf16)
    g = jnp.dot(xs, wgb[...], preferred_element_type=f32)
    u = jnp.dot(xs, wub[...], preferred_element_type=f32)
    a = (g * jax.nn.sigmoid(g) * u).astype(bf16)
    y = jnp.dot(a, wdb[...], preferred_element_type=f32)
    y1 = y[0:1, :] * jax.nn.sigmoid(jnp.concatenate([m1] * (D // 128), axis=1))
    y2 = y[1:2, :] * jax.nn.sigmoid(jnp.concatenate([m2] * (D // 128), axis=1))
    gb = bc(5, 16)

    def fixed(base, x1, h2):
        upd = jnp.where(sub == i1 - base, y1, 0.0) + jnp.where(sub == i2 - base, y2, 0.0)
        return (x1 + gb * (h2 + upd)).astype(bf16)
    fixb[0] = fixed(b1, x1a, h2a)
    fixb[1] = fixed(b2, x1b, h2b)

    scope('epi_out')
    for qb in range(NQB):
        cp_out(qb).wait()
    cf1 = pltpu.make_async_copy(fixb.at[0], o_hbm.at[pl.ds(b1, 16)], sem_o.at[NQB])
    cf2 = pltpu.make_async_copy(fixb.at[1], o_hbm.at[pl.ds(b2, 16)], sem_o.at[NQB + 1])
    cf1.start()

    @pl.when(b1 != b2)
    def _():
        cf2.start()
        cf2.wait()
    cf1.wait()
    scope(None)


@jax.jit
def pallas_adaLN_cond__mha_block_cached__moe_arch_mod__prompt_kernel(
    A_x, A_k_cache, A_v_cache, A_wq, A_wo, B_x, B_w_r, B_w_gate, B_w_up, B_w_down, c, w_mod,
):
    x = A_x.reshape(S, D)
    k = A_k_cache.reshape(NHG, HPS, S, DH)
    v = A_v_cache.reshape(NHG, HPS, S, DH)
    wo = A_wo.reshape(NHG, HPS * DH, D)
    wr = B_w_r.reshape(1, D)
    anyspec = pl.BlockSpec(memory_space=pl.ANY)
    out = pl.pallas_call(
        _kernel,
        in_specs=[anyspec] * 11,
        out_specs=anyspec,
        out_shape=jax.ShapeDtypeStruct((S, D), bf16),
        scratch_shapes=[
            pltpu.VMEM((S, D), bf16),
            pltpu.VMEM((2, HPS, S // 2, DH), u32),
            pltpu.VMEM((2, HPS, S // 2, DH), u32),
            pltpu.VMEM((NHG, D // 2, HPS * DH), u32),
            pltpu.VMEM((NHG, HPS * DH // 2, D), u32),
            pltpu.VMEM((D // 2, F), u32),
            pltpu.VMEM((D // 2, F), u32),
            pltpu.VMEM((F // 2, D), u32),
            pltpu.VMEM((D // 2, 6 * D), u32),
            pltpu.VMEM((8, 7 * D), f32),
            pltpu.VMEM((S // 2, D), u32),
            pltpu.VMEM((S, D), f32),
            pltpu.VMEM((S + CH, D), bf16),
            pltpu.VMEM((2, 16, D), bf16),
            pltpu.VMEM((1, TQ, S), f32),
            pltpu.VMEM((1, TQ, S), f32),
            pltpu.VMEM((TQ // 2, S), u32),
            pltpu.VMEM((TQ // 2, S), u32),
            pltpu.VMEM((1, HPS, TQ, 128), f32),
            pltpu.VMEM((1, TQ, 128), f32),
            pltpu.VMEM((1, TQ, 128), f32),
            pltpu.VMEM((1, TQ, 128), f32),
            pltpu.VMEM((1, TQ, 128), f32),
            pltpu.VMEM((2, 8, 128), f32),
            pltpu.VMEM((2, 8, 128), jnp.int32),
            pltpu.VMEM((1, D), bf16),
            pltpu.VMEM((1, D), bf16),
            pltpu.SMEM((8,), jnp.int32),
            pltpu.SemaphoreType.DMA((2,)),
            pltpu.SemaphoreType.DMA((4,)),
            pltpu.SemaphoreType.DMA((NMC + 4,)),
            pltpu.SemaphoreType.DMA((2,)),
            pltpu.SemaphoreType.DMA((2,)),
            pltpu.SemaphoreType.DMA((2,)),
            pltpu.SemaphoreType.DMA((3 * HPS + 1,)),
            pltpu.SemaphoreType.DMA((3,)),
            pltpu.SemaphoreType.DMA((NQB + 2,)),
        ],
        compiler_params=pltpu.CompilerParams(vmem_limit_bytes=110 * 1024 * 1024, disable_bounds_checks=True,
                                             disable_semaphore_checks=True),
    )(x, k, v, A_wq, wo, wr, B_w_gate, B_w_up, B_w_down, c, w_mod)
    return out.reshape(1, S, D)
```

```python
import os, json
import jax
import jax.numpy as jnp
from jax import lax
import jax.experimental.pallas as pl
import jax.experimental.pallas.tpu as pltpu

S = 2048
D = 1024
H = 32
DH = 128
F = 3584
EPS = 1e-5
LOG2E = 1.4426950408889634
TQ = 512
NQB = S // TQ
HPS = 4
NHG = H // HPS
NSTEP = NQB * NHG
CH = TQ // NHG
NFP = 4
NMC = 4
MCW = 2 * D // NMC
_P = dict(PADS=[5, 5, 5, 5], PADS0=[5, 5, 5, 0], SCOPE=0)
_P.update(json.loads(os.environ.get('KP', '{}')))

f32 = jnp.float32
bf16 = jnp.bfloat16
u32 = jnp.uint32


class _Scope:
    def __init__(self):
        self.cur = None

    def __call__(self, name):
        if not _P['SCOPE']:
            return
        if self.cur is not None:
            self.cur.__exit__(None, None, None)
            self.cur = None
        if name:
            self.cur = jax.named_scope(name)
            self.cur.__enter__()


def _rb(x):
    return x.astype(bf16).astype(f32)


def _recip(x):
    r = pl.reciprocal(x, approx=True)
    return r * (2.0 - x * r)


def _rowsum(x, late=None):
    p = x[:, 0:128]
    for c in range(1, x.shape[1] // 128):
        p = p + x[:, c * 128:(c + 1) * 128]
    if late is not None:
        p = jnp.where(late, 0.0, p)
    return jnp.sum(p, axis=-1, keepdims=True)


def _center(x, late=None):
    m = _rowsum(x, late) * (1.0 / D)
    mb = _rb(m)
    return x - mb, mb, m - mb


def _rstd(xc, dm, late=None):
    v = jnp.maximum(_rowsum(xc * xc, late) * (1.0 / D) - dm * dm, 0.0)
    y = _rb(_rb(v) + EPS)
    return _recip(_rb(y * lax.rsqrt(y)))


def _ln(x):
    xc, _, dm = _center(x)
    return xc * _rstd(xc, dm)


def _kernel(x_hbm, k_hbm, v_hbm, wq_hbm, wo_hbm, wr_hbm, wg_hbm, wu_hbm, wd_hbm, c_hbm, wm_hbm,
            o_hbm,
            xb, kb32, vb32, wqb, wob, wgb, wub, wdb, wmb,
            mod_ref, h_ref, acc_ref, ob, fixb, s0_ref, s1_ref, p0_ref, p1_ref, m_ref,
            l0_ref, l1_ref, l2_ref, l3_ref, hs_ref, o_ref, st_ref, top_ref, topi_ref, wrb, cb_, z_ref,
            sem_s, sem_x, sem_wm, sem_k, sem_v, sem_w, sem_0, sem_f, sem_o):
    scope = _Scope()
    h32 = h_ref
    kb, vb, wqb, wob, wgb, wub, wdb, wmb, h_ref, p0_ref, p1_ref = (
        r.bitcast(bf16) for r in (kb32, vb32, wqb, wob, wgb, wub, wdb, wmb, h_ref, p0_ref, p1_ref))
    o_ref = o_ref.bitcast(bf16)
    hs32 = hs_ref
    hs_ref = hs_ref.bitcast(bf16)
    X0 = TQ + 2 * CH
    X1 = X0 + TQ

    cp_c = pltpu.make_async_copy(c_hbm, cb_, sem_s.at[0])
    cp_wr = pltpu.make_async_copy(wr_hbm, wrb, sem_s.at[1])
    cp_x0 = pltpu.make_async_copy(x_hbm.at[pl.ds(0, TQ)], xb.at[pl.ds(0, TQ)], sem_x.at[0])
    cp_x0b = pltpu.make_async_copy(x_hbm.at[pl.ds(TQ, X0 - TQ)], xb.at[pl.ds(TQ, X0 - TQ)], sem_x.at[3])

    cp_x1 = pltpu.make_async_copy(x_hbm.at[pl.ds(X0, TQ)], xb.at[pl.ds(X0, TQ)], sem_x.at[1])
    cp_x2 = pltpu.make_async_copy(x_hbm.at[pl.ds(X1, S - X1)], xb.at[pl.ds(X1, S - X1)], sem_x.at[2])

    def cp_wm(i):
        return pltpu.make_async_copy(wm_hbm.at[:, pl.ds(i * MCW, MCW)], wmb.at[:, pl.ds(i * MCW, MCW)], sem_wm.at[i])

    def cp_wmr(i):
        cols = pl.ds(pl.multiple_of(i * D, D), D)
        return pltpu.make_async_copy(wm_hbm.at[:, cols], wmb.at[:, cols], sem_wm.at[NMC - 2 + i])

    def cp_k(g, slot):
        return pltpu.make_async_copy(k_hbm.at[g], kb.at[slot], sem_k.at[slot])

    def cp_v(g, slot):
        return pltpu.make_async_copy(v_hbm.at[g], vb.at[slot], sem_v.at[slot])

    def cp_wq(g):
        cols = pl.ds(pl.multiple_of(g * (HPS * DH), HPS * DH), HPS * DH)
        return pltpu.make_async_copy(wq_hbm.at[:, cols], wqb.at[g], sem_w.at[0])

    def cp_wo(g):
        return pltpu.make_async_copy(wo_hbm.at[g], wob.at[g], sem_w.at[1])

    cp0_wq = [pltpu.make_async_copy(wq_hbm.at[:, pl.ds(j * DH, DH)], wqb.at[0, :, pl.ds(j * DH, DH)], sem_0.at[j])
              for j in range(HPS)]
    cp0_k = [pltpu.make_async_copy(k_hbm.at[0, j], kb.at[0, j], sem_0.at[HPS + j]) for j in range(HPS)]
    cp0_v = [pltpu.make_async_copy(v_hbm.at[0, j], vb.at[0, j], sem_0.at[2 * HPS + j]) for j in range(HPS)]

    cp_ffn = [pltpu.make_async_copy(wg_hbm, wgb, sem_f.at[0]),
              pltpu.make_async_copy(wu_hbm, wub, sem_f.at[1]),
              pltpu.make_async_copy(wd_hbm, wdb, sem_f.at[2])]

    def start_ffn_piece(t):
        ra, rb_ = D // NFP, F // NFP
        rows = pl.ds(pl.multiple_of(t * ra, ra), ra)
        pltpu.make_async_copy(wg_hbm.at[rows], wgb.at[rows], sem_f.at[0]).start()
        pltpu.make_async_copy(wu_hbm.at[rows], wub.at[rows], sem_f.at[1]).start()
        rows = pl.ds(pl.multiple_of(t * rb_, 16), rb_)
        pltpu.make_async_copy(wd_hbm.at[rows], wdb.at[rows], sem_f.at[2]).start()

    def cp_out(qb):
        rows = pl.ds(pl.multiple_of(qb * TQ, TQ), TQ)
        return pltpu.make_async_copy(ob.at[rows], o_hbm.at[rows], sem_o.at[qb])

    scope('pro_zero')
    cp_c.start()
    cp_x0.start()
    for i in range(NMC):
        cp_wm(i).start()
    for cp in (cp0_wq[0], cp0_k[0], cp0_wq[1], cp0_k[1], cp0_v[0], cp0_wq[2], cp0_k[2], cp0_v[1],
               cp0_wq[3], cp0_k[3], cp_x0b, cp0_v[2], cp0_v[3], cp_wr,
               cp_wq(1), cp_k(1, 1), cp_v(1, 1), cp_wo(0)):
        cp.start()

    def zbody(i, _):
        rows = pl.ds(pl.multiple_of(i * 256, 256), 256)
        acc_ref[rows, :] = jnp.zeros((256, D), f32)
        z_ref[i] = 0
        return 0
    lax.fori_loop(0, S // 256, zbody, 0)
    mod_ref[...] = jnp.zeros(mod_ref.shape, f32)
    top_ref[...] = jnp.full(top_ref.shape, -jnp.inf, f32)
    topi_ref[0] = jnp.zeros((8, 128), jnp.int32)
    topi_ref[1] = jnp.ones((8, 128), jnp.int32)

    def bc(lo, n):
        p = mod_ref[:, lo * D:(lo + 1) * D]
        return p if n == 8 else jnp.concatenate([p] * (n // 8), axis=0)

    def tie(x, tok):
        if tok is None:
            return x
        return jnp.concatenate([jnp.where(tok < 0.0, 0.0, x[:, 0:128]), x[:, 128:]], axis=1)

    scope('pro_ln')
    cp_x0.wait()

    def nbody(i, _):
        rows = pl.ds(pl.multiple_of(i * 128, 128), 128)
        s1_ref[0, rows, 0:D] = _ln(xb[rows, :].astype(f32))
        return 0
    lax.fori_loop(0, TQ // 128, nbody, 0)

    scope('pro_mod')
    cp_c.wait()

    def silu_c():
        c = cb_[...].astype(f32)
        sc = (c * jax.nn.sigmoid(c)).astype(bf16)
        return jnp.broadcast_to(sc, (8, D))

    def mod_part(lo, width, plus_one):
        md = _rb(jnp.dot(silu_c(), wmb[:, lo:lo + width], preferred_element_type=f32))
        if plus_one:
            md = _rb(1.0 + md)
        mod_ref[:, lo:lo + width] = md

    for i in range(NMC):
        cp_wm(i).wait()
        mod_part(i * MCW, MCW, i * MCW >= D)

    def ln1_rows(r0, n, tok=None, dst=None):
        x = tie(xb[pl.ds(r0, n), :].astype(f32), tok)
        h = _ln(x) * bc(1, n) + bc(0, n)
        if dst is None:
            h_ref[pl.ds(pl.multiple_of(r0, 16), n), :] = h.astype(bf16)
        else:
            hs_ref[pl.ds(dst, n), :] = h.astype(bf16)
        return jnp.abs(h[:, 0:128])

    def derive_params():
        sb, cb1, gb, wr = bc(3, 8), bc(4, 8), bc(5, 8), bc(6, 8)
        mod_ref[:, 7 * D:8 * D] = gb * sb
        mod_ref[:, 8 * D:9 * D] = gb * cb1
        mod_ref[:, 9 * D:10 * D] = cb1 * wr
        mod_ref[:, 10 * D:10 * D + 128] = jnp.broadcast_to(jnp.sum(sb * wr, axis=-1, keepdims=True), (8, 128))

    def fin_rows(r0, d0, n, valid, top, tok=None, late1=None, late2=None):
        x = tie(xb[pl.ds(r0, n), :].astype(f32), tok)
        x1 = x + bc(2, n) * acc_ref[pl.ds(r0, n), :]
        xc, mb, dm = _center(x1, late1)
        rs = _rstd(xc, dm, late2)
        st_ref[0, pl.ds(d0, n), :] = jnp.broadcast_to(mb, (n, 128))
        st_ref[1, pl.ds(d0, n), :] = jnp.broadcast_to(rs, (n, 128))
        ob[pl.ds(d0, n), :] = ((x1 + bc(7, n)) + (xc * rs) * bc(8, n)).astype(bf16)
        rc = mod_ref[:, 10 * D:10 * D + 128]
        r = jnp.broadcast_to(_rowsum(xc * bc(9, n), late2) * rs, (n, 128))
        r = _rb(r + jnp.concatenate([rc] * (n // 8), axis=0))
        tok = jnp.abs(r)
        if valid is not None:
            r = jnp.where(valid, r, -jnp.inf)
        b1, i1, b2, i2 = top
        sub = lax.broadcasted_iota(jnp.int32, (8, 128), 0)
        for g in range(n // 8):
            rg = r[g * 8:(g + 1) * 8, :]
            ids = sub + (r0 + g * 8)
            gt1 = rg > b1
            gt2 = rg > b2
            b2 = jnp.where(gt1, b1, jnp.where(gt2, rg, b2))
            i2 = jnp.where(gt1, i1, jnp.where(gt2, ids, i2))
            b1 = jnp.where(gt1, rg, b1)
            i1 = jnp.where(gt1, ids, i1)
        return (b1, i1, b2, i2), tok

    s_refs = (s0_ref, s1_ref)
    p_refs = (p0_ref, p1_ref)
    l_refs = (l0_ref, l1_ref, l2_ref, l3_ref)

    def attend(t, first):
        qb = t // NHG
        hg = t % NHG
        slot = t % 2
        pads = _P['PADS0'] if first else _P['PADS']
        z = z_ref[0]
        z2 = z_ref[1]
        zp = pl.multiple_of(z * 16, 16)
        arows = pl.ds(pl.multiple_of(qb * TQ, TQ), TQ)
        rlv = {}
        early = [None]

        r0q = pl.multiple_of(qb * TQ, TQ)

        def qp(j):
            if first and j == 1:
                d0 = jnp.dot(h_ref[arows, 0:512], wqb[hg, 0:512, j * DH:(j + 1) * DH], preferred_element_type=f32)
                early[0] = jnp.abs(d0[0:16])
                q = d0 + jnp.dot(h_ref[arows, 512:], wqb[hg, 512:, j * DH:(j + 1) * DH], preferred_element_type=f32)
            else:
                B = _P.get('BQP', TQ)
                q = jnp.concatenate([
                    jnp.dot(h_ref[pl.ds(r0q + r, B), :], wqb[hg, :, j * DH:(j + 1) * DH], preferred_element_type=f32)
                    for r in range(0, TQ, B)], axis=0)
            return q * (DH ** -0.5 * LOG2E)

        def qk(j, q):
            B = _P.get('BQK', TQ)
            for r in range(0, TQ, B):
                s = lax.dot_general(q[r:r + B].astype(bf16), pltpu.bitcast(kb32[slot, j], bf16), (((1,), (1,)), ((), ())),
                                    preferred_element_type=f32)
                s_refs[j % 2][z, r:r + B, :] = s
                pm = s[:, 0:128]
                for c in range(1, S // 128):
                    pm = jnp.maximum(pm, s[:, c * 128:(c + 1) * 128])
                m_ref[z, j, r:r + B, :] = jnp.broadcast_to(jnp.max(pm, axis=-1, keepdims=True), (B, 128))

        def sm(j, tok=None):
            R, W = 16, S // 2
            sref = s_refs[j % 2]
            zs = z_ref[3 + j]
            for r in range(0, TQ, R):
                m = m_ref[zs, j, r:r + R, :]
                acc = None
                for hf in range(2):
                    mm = m if tok is None else jnp.where(tok < 0.0, 0.0, m)
                    ps = []
                    for c in range(W // 128):
                        c0 = hf * W + c * 128
                        pc = jnp.exp2(sref[zs, r:r + R, c0:c0 + 128] - mm)
                        ps.append(pc)
                        acc = pc if acc is None else acc + pc
                    tok = acc
                    for _ in range(pads[j]):
                        tok = tok + tok
                    p_refs[j % 2][pl.ds(zp + r, R), hf * W:(hf + 1) * W] = jnp.concatenate(ps, axis=1).astype(bf16)
                l_refs[j][z, r:r + R, :] = acc

        def pv(j):
            pj = p_refs[j % 2]
            lp = l_refs[j][z2]
            B = _P.get('BPV', TQ)
            if B == TQ:
                vv = pltpu.bitcast(vb32[slot, j], bf16)
                d0 = jnp.dot(pj[pl.ds(zp, TQ), 0:512], vv[0:512], preferred_element_type=f32)
                o = d0 + jnp.dot(pj[pl.ds(zp, TQ), 512:], vv[512:], preferred_element_type=f32)
            else:
                os_ = [jnp.dot(pj[pl.ds(zp + r, B), :], pltpu.bitcast(vb32[slot, j], bf16), preferred_element_type=f32)
                       for r in range(0, TQ, B)]
                o = jnp.concatenate(os_, axis=0)
                d0 = jnp.concatenate([os_[0]] * (TQ // B), axis=0)
            early[0] = jnp.abs(d0[0:16])
            if j >= 0:
                lp = jnp.maximum(lp, jnp.minimum(d0, 0.0))
            l = jnp.broadcast_to(jnp.sum(lp, axis=-1, keepdims=True), (TQ, 128))
            rl = _recip(l)
            rlv[j] = rl
            o_ref[pl.ds(pl.multiple_of(slot * TQ, TQ), TQ), j * DH:(j + 1) * DH] = (o * rl).astype(bf16)

        def qtie(q, j):
            if not _P.get('QTIE', 0):
                return q
            return jnp.where(rlv[j] < 0.0, 0.0, q)

        def op_prev():
            tp = t - 1
            o = o_ref[pl.ds(pl.multiple_of((1 - slot) * TQ, TQ), TQ), :]
            rows = pl.ds(pl.multiple_of((tp // NHG) * TQ, TQ), TQ)
            acc_ref[rows, :] += jnp.dot(o, wob[tp % NHG], preferred_element_type=f32)

        def wait(*cps):
            if first:
                for cp in cps:
                    cp.wait()

        ftok = None
        if first:
            wait(cp0_wq[0])
            h_ref[0:TQ, :] = (s1_ref[0, :, 0:D] * bc(1, TQ) + bc(0, TQ)).astype(bf16)
        else:
            valid = t > NHG
            fsrc = pl.multiple_of(jnp.maximum(t - NHG - 1, 0) * CH, CH)
            fdst = pl.multiple_of(jnp.where(valid, fsrc, S), CH)
            top = (top_ref[0], topi_ref[0], top_ref[1], topi_ref[1])
            for g in range(CH // 16):
                top, ftok = fin_rows(fsrc + g * 16, fdst + g * 16, 16, valid, top, ftok)
            top_ref[0], topi_ref[0], top_ref[1], topi_ref[1] = top
            ftok = jnp.minimum(ftok[0:8], ftok[8:16])
            ftok = jnp.concatenate([ftok, ftok], axis=0)

        l0 = pl.multiple_of(jnp.minimum(t + NHG, NSTEP - 1) * CH, CH)
        lnm = 'qk3' if first else _P.get('LNM', 'qp1')

        def ln1(tok, staged):
            for g in range(CH // 16):
                tok = ln1_rows(l0 + g * 16, 16, tok, zp + g * 16 if staged else None)
            tok = jnp.minimum(tok[0:8], tok[8:16])
            return jnp.concatenate([tok, tok], axis=0)

        if lnm == 'start':
            ftok = jnp.minimum(ftok, ln1(None, True))
        if lnm == 'after':
            ltok = ln1(ftok, True)
        if not first:
            cp_k((t + 1) % NHG, 1 - slot).start()
            cp_v((t + 1) % NHG, 1 - slot).start()
        q0 = qp(0)
        wait(cp0_k[0])
        qk(0, q0)
        wait(cp0_wq[1], cp0_k[1], cp0_v[0], cp0_wq[2])
        q1 = qp(1)
        sm(0, early[0] if first else ftok)
        if lnm == 'qp1':
            ltok = ln1(jnp.abs(q1[0:16]), True)
        qk(1, q1)
        sm(1, ltok if lnm in ('after', 'qp1') and _P.get('LPIN', 1) else None)
        pv(0)
        if lnm == 'pv0':
            ltok = ln1(early[0], True)
        q2 = qtie(qp(2), 0)
        wait(cp0_k[2], cp0_v[1], cp0_wq[3], cp0_k[3], cp_x0b)
        qk(2, q2)
        sm(2, ltok if lnm == 'pv0' and _P.get('LPIN', 1) else None)
        pv(1)
        if lnm == 'pv1':
            ltok = ln1(early[0], True)
        q3 = qp(3)
        qk(3, qtie(q3, 1))
        tok = None
        if lnm == 'qk3':
            tok = ln1(jnp.abs(q3[TQ - 16:TQ, :]), False)
        elif lnm == 'pv1' and _P.get('LPIN', 1):
            tok = ltok
        if tok is None:
            tok = jnp.abs(q3[TQ - 16:TQ, :])
        wait(cp0_v[2], cp0_v[3], cp_wr)
        if first:
            pv(2)
            sm(3, early[0])
        else:
            sm(3, tok)
            pv(2)
            if lnm != 'qk3':
                lm = jnp.concatenate([jnp.concatenate([early[0]] * 2, axis=0)] * (D // 128), axis=1) < 0.0
                h32[pl.ds(pl.multiple_of(l0 // 2, 8), CH // 2), :] = jnp.where(
                    lm, jnp.uint32(0), hs32[pl.ds(pl.multiple_of(z2 * 8, 8), CH // 2), :])
        if not first:
            op_prev()
        pv(3)

    scope('step0')
    attend(0, True)
    mod_ref[:, 6 * D:7 * D] = jnp.broadcast_to(wrb[...].astype(f32), (8, D))
    scope(None)

    def step(t, _):
        scope('step_head')
        hg = t % NHG
        slot = t % 2
        cp_k(hg, slot).wait()
        cp_v(hg, slot).wait()

        @pl.when(jnp.logical_or(t <= NHG + NFP, hg == 1))
        def _():
            @pl.when(t < NHG)
            def _():
                cp_wq(hg).wait()
                cp_wo(hg - 1).wait()
                cp_wo(hg).start()

                @pl.when(t < NHG - 1)
                def _():
                    cp_wq(hg + 1).start()

                @pl.when(t == 1)
                def _():
                    cp_x1.start()

                @pl.when(t == 2)
                def _():
                    cp_x1.wait()

                @pl.when(jnp.logical_and(t >= 2, t < 6))
                def _():
                    cp_wmr(t).start()

                @pl.when(t == 6)
                def _():
                    cp_x2.start()

            @pl.when(t == NHG)
            def _():
                cp_x2.wait()
                cp_wo(NHG - 1).wait()
                for i in range(2, 6):
                    cp_wmr(i).wait()
                mod_part(2 * D, 2 * D, False)
                mod_part(4 * D, D, True)
                mod_part(5 * D, D, False)
                derive_params()

            @pl.when(jnp.logical_and(t > NHG, t <= NHG + NFP))
            def _():
                start_ffn_piece(t - NHG - 1)

            @pl.when(t >= 2 * NHG)
            def _():
                cp_out(t // NHG - 2).start()

        scope('step_body')
        attend(t, False)
        scope(None)
        return 0

    lax.fori_loop(1, NSTEP, step, 0)

    scope('epi_fin')
    cp_k(0, 0).wait()
    cp_v(0, 0).wait()
    for cp in cp_ffn:
        cp.wait()
    top = (top_ref[0], topi_ref[0], top_ref[1], topi_ref[1])
    rl0 = (NQB - 1) * TQ
    EG, EB = 16, _P.get('EB', 64)
    oslot = ((NSTEP - 1) % 2) * TQ
    ds = []
    for r in range(0, TQ, EB):
        d = jnp.dot(o_ref[oslot + r:oslot + r + EB, :], wob[NHG - 1], preferred_element_type=f32)
        acc_ref[rl0 + r:rl0 + r + EB, :] += d
        ds.append(d)

    def late(tc):
        per = EB * 8
        if tc < 0 or tc >= len(ds) * per:
            return None
        d = ds[tc // per]
        c = (tc % per) // EB
        tk = jnp.abs(d[0:8, c * 128:(c + 1) * 128]) < 0.0
        return jnp.concatenate([tk] * (EG // 8), axis=0)

    L1, L2 = _P.get('EL', [100, 400])
    for r in range(-CH, TQ, EG):
        ready = (r // EB + 1) * EB * 8 + (r % EB) * 8
        top, _ = fin_rows(rl0 + r, rl0 + r, EG, None, top, None, late(ready + L1), late(ready + L2))
        if r == -EG:
            cp_out(NQB - 2).start()
    cp_out(NQB - 1).start()

    if _P.get('ESPLIT', 0):
        scope('epi_ffn')
    vals = jnp.concatenate([top[0], top[2]], axis=0)
    idxs = jnp.concatenate([top[1], top[3]], axis=0)
    m1 = jnp.max(vals, axis=0, keepdims=True)
    i1v = jnp.min(jnp.where(vals == m1, idxs, S - 1), axis=0, keepdims=True)
    vals2 = jnp.where(idxs == i1v, -jnp.inf, vals)
    m2 = jnp.max(vals2, axis=0, keepdims=True)
    i2v = jnp.min(jnp.where(jnp.logical_and(vals2 == m2, idxs != i1v), idxs, S - 1), axis=0, keepdims=True)
    b1 = pl.multiple_of(jnp.clip(i1v[0, 0], 0, S - 1) // 8 * 8, 8)
    b2 = pl.multiple_of(jnp.clip(i2v[0, 0], 0, S - 1) // 8 * 8, 8)

    def two(ref_rows):
        return jnp.concatenate([ref_rows(b1), ref_rows(b2)], axis=0)

    def lanes(v):
        return jnp.concatenate([v] * (D // 128), axis=1)

    x1 = two(lambda b: xb[pl.ds(b, 8), :].astype(f32)) + bc(2, 16) * two(lambda b: acc_ref[pl.ds(b, 8), :])
    xn = (x1 - lanes(two(lambda b: st_ref[0, pl.ds(b, 8), :]))) * lanes(two(lambda b: st_ref[1, pl.ds(b, 8), :]))
    h2 = xn * bc(4, 16) + bc(3, 16)
    xs = h2.astype(bf16)
    FC = _P.get('FC', 512)
    y = None
    prev = None
    for c in range(0, F + FC, FC):
        if c < F:
            g = jnp.dot(xs, wgb[:, c:c + FC], preferred_element_type=f32)
            u = jnp.dot(xs, wub[:, c:c + FC], preferred_element_type=f32)
        if prev is not None:
            d = jnp.dot(prev, wdb[c - FC:c, :], preferred_element_type=f32)
            y = d if y is None else y + d
        if c < F:
            prev = (g * jax.nn.sigmoid(g) * u).astype(bf16)
    sub = lax.broadcasted_iota(jnp.int32, (8, 128), 0)
    ids = jnp.concatenate([sub + b1, sub + b2], axis=0)
    is1 = lanes(ids == i1v)
    is2 = lanes(ids == i2v)
    upd = jnp.where(is1, y * lanes(jax.nn.sigmoid(m1)), jnp.where(is2, y * lanes(jax.nn.sigmoid(m2)), 0.0))
    fixb[...] = ((x1 + bc(7, 16)) + xn * bc(8, 16) + bc(5, 16) * upd).astype(bf16)

    scope('epi_out')
    for qb in range(NQB):
        cp_out(qb).wait()
    cf1 = pltpu.make_async_copy(fixb.at[pl.ds(0, 8)], o_hbm.at[pl.ds(b1, 8)], sem_o.at[NQB])
    cf2 = pltpu.make_async_copy(fixb.at[pl.ds(8, 8)], o_hbm.at[pl.ds(b2, 8)], sem_o.at[NQB + 1])
    cf1.start()

    @pl.when(b1 != b2)
    def _():
        cf2.start()
        cf2.wait()
    cf1.wait()
    scope(None)


@jax.jit
def pallas_adaLN_cond__mha_block_cached__moe_arch_mod__prompt_kernel(
    A_x, A_k_cache, A_v_cache, A_wq, A_wo, B_x, B_w_r, B_w_gate, B_w_up, B_w_down, c, w_mod,
):
    x = A_x.reshape(S, D)
    k = A_k_cache.reshape(NHG, HPS, S, DH)
    v = A_v_cache.reshape(NHG, HPS, S, DH)
    wo = A_wo.reshape(NHG, HPS * DH, D)
    wr = B_w_r.reshape(1, D)
    anyspec = pl.BlockSpec(memory_space=pl.ANY)
    out = pl.pallas_call(
        _kernel,
        in_specs=[anyspec] * 11,
        out_specs=anyspec,
        out_shape=jax.ShapeDtypeStruct((S, D), bf16),
        scratch_shapes=[
            pltpu.VMEM((S, D), bf16),
            pltpu.VMEM((2, HPS, S // 2, DH), u32),
            pltpu.VMEM((2, HPS, S // 2, DH), u32),
            pltpu.VMEM((NHG, D // 2, HPS * DH), u32),
            pltpu.VMEM((NHG, HPS * DH // 2, D), u32),
            pltpu.VMEM((D // 2, F), u32),
            pltpu.VMEM((D // 2, F), u32),
            pltpu.VMEM((F // 2, D), u32),
            pltpu.VMEM((D // 2, 6 * D), u32),
            pltpu.VMEM((8, 11 * D), f32),
            pltpu.VMEM((S // 2, D), u32),
            pltpu.VMEM((S, D), f32),
            pltpu.VMEM((S + CH, D), bf16),
            pltpu.VMEM((16, D), bf16),
            pltpu.VMEM((1, TQ, S), f32),
            pltpu.VMEM((1, TQ, S), f32),
            pltpu.VMEM((TQ // 2, S), u32),
            pltpu.VMEM((TQ // 2, S), u32),
            pltpu.VMEM((1, HPS, TQ, 128), f32),
            pltpu.VMEM((1, TQ, 128), f32),
            pltpu.VMEM((1, TQ, 128), f32),
            pltpu.VMEM((1, TQ, 128), f32),
            pltpu.VMEM((1, TQ, 128), f32),
            pltpu.VMEM((CH // 2, D), u32),
            pltpu.VMEM((TQ, HPS * DH), u32),
            pltpu.VMEM((2, S + CH, 128), f32),
            pltpu.VMEM((2, 8, 128), f32),
            pltpu.VMEM((2, 8, 128), jnp.int32),
            pltpu.VMEM((1, D), bf16),
            pltpu.VMEM((1, D), bf16),
            pltpu.SMEM((8,), jnp.int32),
            pltpu.SemaphoreType.DMA((2,)),
            pltpu.SemaphoreType.DMA((4,)),
            pltpu.SemaphoreType.DMA((NMC + 4,)),
            pltpu.SemaphoreType.DMA((2,)),
            pltpu.SemaphoreType.DMA((2,)),
            pltpu.SemaphoreType.DMA((2,)),
            pltpu.SemaphoreType.DMA((3 * HPS + 1,)),
            pltpu.SemaphoreType.DMA((3,)),
            pltpu.SemaphoreType.DMA((NQB + 2,)),
        ],
        compiler_params=pltpu.CompilerParams(vmem_limit_bytes=110 * 1024 * 1024, disable_bounds_checks=True,
                                             disable_semaphore_checks=True),
    )(x, k, v, A_wq, wo, wr, B_w_gate, B_w_up, B_w_down, c, w_mod)
    return out.reshape(1, S, D)
```

```python
import os, json
import jax
import jax.numpy as jnp
from jax import lax
import jax.experimental.pallas as pl
import jax.experimental.pallas.tpu as pltpu

S = 2048
D = 1024
H = 32
DH = 128
F = 3584
EPS = 1e-5
LOG2E = 1.4426950408889634
TQ = 512
NQB = S // TQ
HPS = 4
NHG = H // HPS
NSTEP = NQB * NHG
CH = TQ // NHG
MPW = json.loads(os.environ.get('KP', '{}')).get('MPW', 640)
NMP = -(-4 * D // MPW)
NMC = 4
MCW = 2 * D // NMC
_P = dict(PADS=[5, 5, 5, 5], PADS0=[5, 5, 5, 0], SCOPE=0)
_P.update(json.loads(os.environ.get('KP', '{}')))

f32 = jnp.float32
bf16 = jnp.bfloat16
u32 = jnp.uint32


class _Scope:
    def __init__(self):
        self.cur = None

    def __call__(self, name):
        if not _P['SCOPE']:
            return
        if self.cur is not None:
            self.cur.__exit__(None, None, None)
            self.cur = None
        if name:
            self.cur = jax.named_scope(name)
            self.cur.__enter__()


def _rb(x):
    return x.astype(bf16).astype(f32)


def _recip(x):
    r = pl.reciprocal(x, approx=True)
    return r * (2.0 - x * r)


def _rowsum(x, late=None):
    p = x[:, 0:128]
    for c in range(1, x.shape[1] // 128):
        p = p + x[:, c * 128:(c + 1) * 128]
    if late is not None:
        p = jnp.where(late, 0.0, p)
    return jnp.sum(p, axis=-1, keepdims=True)


def _center(x, late=None):
    m = _rowsum(x, late) * (1.0 / D)
    mb = _rb(m)
    return x - mb, mb, m - mb


def _rstd(xc, dm, late=None):
    v = jnp.maximum(_rowsum(xc * xc, late) * (1.0 / D) - dm * dm, 0.0)
    y = _rb(_rb(v) + EPS)
    return _recip(_rb(y * lax.rsqrt(y)))


def _ln(x, late1=None, late2=None):
    xc, _, dm = _center(x, late1)
    return xc * _rstd(xc, dm, late2)


def _kernel(x_hbm, k_hbm, v_hbm, wq_hbm, wo_hbm, wr_hbm, wg_hbm, wu_hbm, wd_hbm, c_hbm, wm_hbm,
            o_hbm,
            xb, kb32, vb32, wqb, wob, wgb, wub, wdb, wmb,
            mod_ref, h_ref, acc_ref, ob, fixb, s0_ref, s1_ref, p0_ref, p1_ref, m_ref,
            l0_ref, l1_ref, l2_ref, l3_ref, hs_ref, o_ref, st_ref, scb_ref, mp_ref, top_ref, topi_ref, wrb, cb_, z_ref,
            sem_s, sem_x, sem_wm, sem_k, sem_v, sem_w, sem_0, sem_f, sem_o):
    scope = _Scope()
    h32 = h_ref
    wm32 = wmb
    kb, vb, wqb, wob, wgb, wub, wdb, wmb, h_ref, p0_ref, p1_ref = (
        r.bitcast(bf16) for r in (kb32, vb32, wqb, wob, wgb, wub, wdb, wmb, h_ref, p0_ref, p1_ref))
    o_ref = o_ref.bitcast(bf16)
    wm0 = s0_ref.bitcast(bf16)
    hs32 = hs_ref
    hs_ref = hs_ref.bitcast(bf16)
    X0 = TQ + 2 * CH
    X1 = X0 + TQ

    cp_c = pltpu.make_async_copy(c_hbm, cb_, sem_s.at[0])
    cp_wr = pltpu.make_async_copy(wr_hbm, wrb, sem_s.at[1])
    cp_x0 = pltpu.make_async_copy(x_hbm.at[pl.ds(0, TQ)], xb.at[pl.ds(0, TQ)], sem_x.at[0])
    cp_x0b = pltpu.make_async_copy(x_hbm.at[pl.ds(TQ, X0 - TQ)], xb.at[pl.ds(TQ, X0 - TQ)], sem_x.at[3])

    cp_x1 = pltpu.make_async_copy(x_hbm.at[pl.ds(X0, TQ)], xb.at[pl.ds(X0, TQ)], sem_x.at[1])
    cp_x2 = pltpu.make_async_copy(x_hbm.at[pl.ds(X1, S - X1)], xb.at[pl.ds(X1, S - X1)], sem_x.at[2])

    def cp_wm(i):
        return pltpu.make_async_copy(wm_hbm.at[:, pl.ds(i * MCW, MCW)], wm0.at[0, :, pl.ds(i * MCW, MCW)], sem_wm.at[i])

    def cp_wmr(p):
        w = min(MPW, 4 * D - p * MPW)
        return pltpu.make_async_copy(wm_hbm.at[:, pl.ds(2 * D + p * MPW, w)], wmb.at[p, :, pl.ds(0, w)], sem_wm.at[NMC + p])

    def cp_k(g):
        return pltpu.make_async_copy(k_hbm.at[g], kb.at[g], sem_k.at[g])

    def cp_v(g):
        return pltpu.make_async_copy(v_hbm.at[g], vb.at[g], sem_v.at[g])

    def cp_wq(g):
        cols = pl.ds(pl.multiple_of(g * (HPS * DH), HPS * DH), HPS * DH)
        return pltpu.make_async_copy(wq_hbm.at[:, cols], wqb.at[g], sem_w.at[g])

    def cp_wo(g):
        return pltpu.make_async_copy(wo_hbm.at[g], wob.at[g], sem_w.at[NHG + g])

    cp0_wq = [pltpu.make_async_copy(wq_hbm.at[:, pl.ds(j * DH, DH)], wqb.at[0, :, pl.ds(j * DH, DH)], sem_0.at[j])
              for j in range(HPS)]
    cp0_k = [pltpu.make_async_copy(k_hbm.at[0, j], kb.at[0, j], sem_0.at[HPS + j]) for j in range(HPS)]
    cp0_v = [pltpu.make_async_copy(v_hbm.at[0, j], vb.at[0, j], sem_0.at[2 * HPS + j]) for j in range(HPS)]

    cp_ffn = [pltpu.make_async_copy(wg_hbm, wgb, sem_f.at[0]),
              pltpu.make_async_copy(wu_hbm, wub, sem_f.at[1]),
              pltpu.make_async_copy(wd_hbm, wdb, sem_f.at[2])]

    def cp_out(qb):
        rows = pl.ds(pl.multiple_of(qb * TQ, TQ), TQ)
        return pltpu.make_async_copy(ob.at[rows], o_hbm.at[rows], sem_o.at[qb])

    scope('pro_zero')
    cp_c.start()
    cp_x0.start()
    for i in range(NMC):
        cp_wm(i).start()
    for cp in (cp0_wq[0], cp0_k[0], cp0_wq[1], cp0_k[1], cp0_v[0], cp0_wq[2], cp0_k[2], cp0_v[1],
               cp0_wq[3], cp0_k[3], cp_x0b, cp0_v[2], cp0_v[3], cp_wr):
        cp.start()
    for g in range(1, NHG):
        for cp in [cp_wq(g), cp_k(g), cp_v(g), cp_wo(g - 1)] + ([cp_x1] if g == 1 else []) + ([cp_wmr(g - 1)] if g <= NMP else []):
            cp.start()
    for cp in [cp_wo(NHG - 1), cp_x2] + cp_ffn:
        cp.start()

    def zbody(i, _):
        rows = pl.ds(pl.multiple_of(i * 256, 256), 256)
        acc_ref[rows, :] = jnp.zeros((256, D), f32)
        z_ref[i] = 0
        return 0
    lax.fori_loop(0, S // 256, zbody, 0)
    mod_ref[...] = jnp.zeros(mod_ref.shape, f32)
    top_ref[...] = jnp.full(top_ref.shape, -jnp.inf, f32)
    topi_ref[0] = jnp.zeros((8, 128), jnp.int32)
    topi_ref[1] = jnp.ones((8, 128), jnp.int32)

    def bc(lo, n):
        p = mod_ref[:, lo * D:(lo + 1) * D]
        return p if n == 8 else jnp.concatenate([p] * (n // 8), axis=0)

    def tie(x, tok):
        if tok is None:
            return x
        return jnp.concatenate([jnp.where(tok < 0.0, 0.0, x[:, 0:128]), x[:, 128:]], axis=1)

    scope('pro_ln')
    cp_x0.wait()

    def nbody(i, _):
        rows = pl.ds(pl.multiple_of(i * 128, 128), 128)
        s1_ref[0, rows, 0:D] = _ln(xb[rows, :].astype(f32))
        return 0
    lax.fori_loop(0, TQ // 128, nbody, 0)

    scope('pro_mod')
    cp_c.wait()

    def silu_c():
        c = cb_[...].astype(f32)
        sc = (c * jax.nn.sigmoid(c)).astype(bf16)
        return jnp.broadcast_to(sc, (8, D))

    def mod_part(lo, width, plus_one):
        w = pltpu.bitcast(s0_ref[0, :, lo:lo + width], bf16)
        md = _rb(jnp.dot(silu_c(), w, preferred_element_type=f32))
        if plus_one:
            md = _rb(1.0 + md)
        mod_ref[:, lo:lo + width] = md

    scf = silu_c().astype(f32)
    for b in range(D // 128):
        blk = jnp.concatenate([scf[:, b * 128:(b + 1) * 128]] * 16, axis=0)
        scb_ref[b * 128:(b + 1) * 128, :] = blk.T

    for i in range(NMC):
        cp_wm(i).wait()
        mod_part(i * MCW, MCW, i * MCW >= D)

    def ln1_rows(r0, n, tok=None, dst=None, late1=None, late2=None):
        x = tie(xb[pl.ds(r0, n), :].astype(f32), tok)
        h = _ln(x, late1, late2) * bc(1, n) + bc(0, n)
        if dst is None:
            h_ref[pl.ds(pl.multiple_of(r0, 16), n), :] = h.astype(bf16)
        else:
            hs_ref[pl.ds(dst, n), :] = h.astype(bf16)
        return jnp.abs(h[:, 0:128])

    def derive_params():
        for c in range(4 * D // 128):
            p, o = divmod(c * 128, MPW)
            md = _rb(jnp.broadcast_to(jnp.sum(mp_ref[p, :, o:o + 128], axis=0, keepdims=True), (8, 128)))
            if 2 * D <= c * 128 < 3 * D:
                md = _rb(1.0 + md)
            mod_ref[:, 2 * D + c * 128:2 * D + (c + 1) * 128] = md
        sb, cb1, gb, wr = bc(3, 8), bc(4, 8), bc(5, 8), bc(6, 8)
        mod_ref[:, 7 * D:8 * D] = gb * sb
        mod_ref[:, 8 * D:9 * D] = gb * cb1
        mod_ref[:, 9 * D:10 * D] = cb1 * wr
        mod_ref[:, 10 * D:10 * D + 128] = jnp.broadcast_to(jnp.sum(sb * wr, axis=-1, keepdims=True), (8, 128))

    def fin_rows(r0, d0, n, valid, top, tok=None, late1=None, late2=None):
        x = tie(xb[pl.ds(r0, n), :].astype(f32), tok)
        x1 = x + bc(2, n) * acc_ref[pl.ds(r0, n), :]
        xc, mb, dm = _center(x1, late1)
        rs = _rstd(xc, dm, late2)
        st_ref[0, pl.ds(d0, n), :] = jnp.broadcast_to(mb, (n, 128))
        st_ref[1, pl.ds(d0, n), :] = jnp.broadcast_to(rs, (n, 128))
        ob[pl.ds(d0, n), :] = ((x1 + bc(7, n)) + (xc * rs) * bc(8, n)).astype(bf16)
        rc = mod_ref[:, 10 * D:10 * D + 128]
        r = jnp.broadcast_to(_rowsum(xc * bc(9, n), late2) * rs, (n, 128))
        r = _rb(r + jnp.concatenate([rc] * (n // 8), axis=0))
        tok = jnp.abs(r)
        if valid is not None:
            r = jnp.where(valid, r, -jnp.inf)
        b1, i1, b2, i2 = top
        sub = lax.broadcasted_iota(jnp.int32, (8, 128), 0)
        for g in range(n // 8):
            rg = r[g * 8:(g + 1) * 8, :]
            ids = sub + (r0 + g * 8)
            gt1 = rg > b1
            gt2 = rg > b2
            b2 = jnp.where(gt1, b1, jnp.where(gt2, rg, b2))
            i2 = jnp.where(gt1, i1, jnp.where(gt2, ids, i2))
            b1 = jnp.where(gt1, rg, b1)
            i1 = jnp.where(gt1, ids, i1)
        return (b1, i1, b2, i2), tok

    s_refs = (s0_ref, s1_ref)
    p_refs = (p0_ref, p1_ref)
    l_refs = (l0_ref, l1_ref, l2_ref, l3_ref)

    def attend(t, first):
        qb = t // NHG
        hg = t % NHG
        slot = t % 2
        pads = _P['PADS0'] if first else _P['PADS']
        z = z_ref[0]
        z2 = z_ref[1]
        zp = pl.multiple_of(z * 16, 16)
        arows = pl.ds(pl.multiple_of(qb * TQ, TQ), TQ)
        early = [None]
        svals = {}
        mv = [jnp.zeros((8, 128), f32), 0]
        mpi = jnp.where(jnp.logical_and(t >= 2, t < 2 + NMP), t - 2, NMP)

        def qp(j):
            if first and j == 1:
                d0 = jnp.dot(h_ref[arows, 0:512], wqb[hg, 0:512, j * DH:(j + 1) * DH], preferred_element_type=f32)
                early[0] = jnp.abs(d0[0:16])
                q = d0 + jnp.dot(h_ref[arows, 512:], wqb[hg, 512:, j * DH:(j + 1) * DH], preferred_element_type=f32)
            else:
                q = jnp.dot(h_ref[arows, :], wqb[hg, :, j * DH:(j + 1) * DH], preferred_element_type=f32)
            return q * (DH ** -0.5 * LOG2E)

        def qk(j, q):
            s = lax.dot_general(q.astype(bf16), pltpu.bitcast(kb32[hg, j], bf16), (((1,), (1,)), ((), ())),
                                preferred_element_type=f32)
            svals[j] = s
            s_refs[j % 2][z] = s
            pm = s[:, 0:128]
            for c in range(1, S // 128):
                pm = jnp.maximum(pm, s[:, c * 128:(c + 1) * 128])
            m_ref[z, j] = jnp.broadcast_to(jnp.max(pm, axis=-1, keepdims=True), (TQ, 128))

        def sm(j, tok=None):
            R, W = 16, S // 2
            sref = s_refs[j % 2]
            zs = z_ref[3 + j]
            for r in range(0, TQ, R):
                m = m_ref[zs, j, r:r + R, :]
                acc = None
                for hf in range(2):
                    mm = m if tok is None else jnp.where(tok < 0.0, 0.0, m)
                    ps = []
                    for c in range(W // 128):
                        c0 = hf * W + c * 128
                        pc = jnp.exp2(sref[zs, r:r + R, c0:c0 + 128] - mm)
                        ps.append(pc)
                        acc = pc if acc is None else acc + pc
                    if first or j != 1:
                        tok = acc
                        for _ in range(pads[j]):
                            tok = tok + tok
                    else:
                        never = jnp.minimum(acc[0:8], acc[8:16]) < 0.0
                        a = jnp.where(never, 1.0, mv[0])
                        for _ in range(MPW // 128):
                            mc, k0 = divmod(mv[1], D)
                            mv[1] += 16
                            w = pltpu.bitcast(wm32[mpi, k0 // 2:k0 // 2 + 8, mc * 128:(mc + 1) * 128], bf16).astype(f32)
                            pr = w * scb_ref[k0:k0 + 16, :]
                            a = (a + pr[0:8]) + pr[8:16]
                            tok = a
                            if k0 + 16 == D:
                                mp_ref[mpi, :, mc * 128:(mc + 1) * 128] = a
                                a = jnp.where(jnp.abs(a) < 0.0, 1.0, 0.0)
                        mv[0] = a
                        tok = jnp.abs(tok)
                        tok = jnp.concatenate([tok, tok], axis=0)
                    p_refs[j % 2][pl.ds(zp + r, R), hf * W:(hf + 1) * W] = jnp.concatenate(ps, axis=1).astype(bf16)
                l_refs[j][z, r:r + R, :] = acc

        def pv(j):
            pj = p_refs[j % 2]
            vv = pltpu.bitcast(vb32[hg, j], bf16)
            d0 = jnp.dot(pj[pl.ds(zp, TQ), 0:512], vv[0:512], preferred_element_type=f32)
            o = d0 + jnp.dot(pj[pl.ds(zp, TQ), 512:], vv[512:], preferred_element_type=f32)
            early[0] = jnp.abs(d0[0:16])
            lp = jnp.maximum(l_refs[j][z2], jnp.minimum(d0, 0.0))
            l = jnp.broadcast_to(jnp.sum(lp, axis=-1, keepdims=True), (TQ, 128))
            o_ref[pl.ds(pl.multiple_of(slot * TQ, TQ), TQ), j * DH:(j + 1) * DH] = (o * _recip(l)).astype(bf16)

        def op_prev():
            tp = t - 1
            o = o_ref[pl.ds(pl.multiple_of((1 - slot) * TQ, TQ), TQ), :]
            rows = pl.ds(pl.multiple_of((tp // NHG) * TQ, TQ), TQ)
            d = jnp.dot(o, wob[tp % NHG], preferred_element_type=f32)
            acc_ref[rows, :] += d

        def wait(*cps):
            if first:
                for cp in cps:
                    cp.wait()

        def both(tok):
            tok = jnp.minimum(tok[0:8], tok[8:16])
            return jnp.concatenate([tok, tok], axis=0)

        def late(j, tc):
            c, r8 = (tc // TQ) * 4, (tc % TQ) // 8 * 8
            tk = jnp.abs(svals[j][r8:r8 + 8, c * 128:(c + 1) * 128]) < 0.0
            return jnp.concatenate([tk, tk], axis=0)

        def finalize():
            valid = t > NHG
            fsrc = pl.multiple_of(jnp.maximum(t - NHG - 1, 0) * CH, CH)
            fdst = pl.multiple_of(jnp.where(valid, fsrc, S), CH)
            top = (top_ref[0], topi_ref[0], top_ref[1], topi_ref[1])
            tok = None
            fp = _P.get('FP')
            for g in range(CH // 16):
                if fp:
                    top, tk = fin_rows(fsrc + g * 16, fdst + g * 16, 16, valid, top, None,
                                       late(0, fp[0] + g * fp[1]), late(0, fp[0] + g * fp[1] + fp[2]))
                    tok = tk if tok is None else jnp.minimum(tok, tk)
                else:
                    top, tok = fin_rows(fsrc + g * 16, fdst + g * 16, 16, valid, top, tok)
            top_ref[0], topi_ref[0], top_ref[1], topi_ref[1] = top
            return both(tok)

        l0 = pl.multiple_of(jnp.minimum(t + NHG, NSTEP - 1) * CH, CH)

        def ln1(tok, staged, j=None):
            lp_ = _P.get('LP') if j is not None else None
            out = None
            for g in range(CH // 16):
                if lp_:
                    tk = ln1_rows(l0 + g * 16, 16, None, zp + g * 16,
                                  late(j, lp_[0] + g * lp_[1]), late(j, lp_[0] + g * lp_[1] + lp_[2]))
                    out = tk if out is None else jnp.minimum(out, tk)
                else:
                    out = tok = ln1_rows(l0 + g * 16, 16, tok, zp + g * 16 if staged else None)
            return both(out)

        if first:
            wait(cp0_wq[0])
            h_ref[0:TQ, :] = (s1_ref[0, :, 0:D] * bc(1, TQ) + bc(0, TQ)).astype(bf16)
            q0 = qp(0)
            wait(cp0_k[0])
            qk(0, q0)
            wait(cp0_wq[1], cp0_k[1], cp0_v[0], cp0_wq[2])
            q1 = qp(1)
            sm(0, early[0])
            qk(1, q1)
            sm(1)
            pv(0)
            q2 = qp(2)
            wait(cp0_k[2], cp0_v[1], cp0_wq[3], cp0_k[3], cp_x0b)
            qk(2, q2)
            sm(2)
            pv(1)
            q3 = qp(3)
            qk(3, q3)
            ln1(jnp.abs(q3[TQ - 16:TQ, :]), False)
            wait(cp0_v[2], cp0_v[3], cp_wr)
            pv(2)
            sm(3, early[0])
            pv(3)
            return

        if not _P.get('FP'):
            ftok = finalize()
        qk(0, qp(0))
        if _P.get('FP'):
            ftok = finalize()
        q1 = qp(1)
        sm(0, ftok)
        lj = _P.get('LJ', 1)
        if not _P.get('LP'):
            ltok = ln1(jnp.abs(q1[0:16]), True)
        qk(1, q1)
        if _P.get('LP') and lj == 1:
            ltok = ln1(None, True, 1)
        sm(1, ltok if lj == 1 else None)
        pv(0)
        qk(2, qp(2))
        if _P.get('LP') and lj == 2:
            ltok = ln1(None, True, 2)
        sm(2, ltok if lj == 2 else None)
        pv(1)
        qk(3, qp(3))
        sm(3)
        pv(2)
        lm = jnp.concatenate([jnp.concatenate([early[0]] * 2, axis=0)] * (D // 128), axis=1) < 0.0
        h32[pl.ds(pl.multiple_of(l0 // 2, 8), CH // 2), :] = jnp.where(
            lm, jnp.uint32(0), hs32[pl.ds(pl.multiple_of(z2 * 8, 8), CH // 2), :])
        op_prev()
        pv(3)

    scope('step0')
    attend(0, True)
    mod_ref[:, 6 * D:7 * D] = jnp.broadcast_to(wrb[...].astype(f32).reshape(1, D), (8, D))
    scope(None)

    def step(t, _):
        scope('step_head')
        hg = t % NHG

        @pl.when(jnp.logical_or(t <= NHG, hg == 1))
        def _():
            @pl.when(t < NHG)
            def _():
                cp_wq(hg).wait()
                cp_k(hg).wait()
                cp_v(hg).wait()
                cp_wo(hg - 1).wait()

            @pl.when(t == 2)
            def _():
                cp_x1.wait()

            for p in range(NMP):
                @pl.when(t == 2 + p)
                def _():
                    cp_wmr(p).wait()

            @pl.when(t == NHG)
            def _():
                cp_x2.wait()
                cp_wo(NHG - 1).wait()

            @pl.when(t == NHG + 1)
            def _():
                derive_params()

            @pl.when(t >= 2 * NHG)
            def _():
                cp_out(t // NHG - 2).start()

        scope('step_body')
        attend(t, False)
        scope(None)
        return 0

    lax.fori_loop(1, NSTEP, step, 0)

    scope('epi_fin')
    for cp in cp_ffn:
        cp.wait()
    top = (top_ref[0], topi_ref[0], top_ref[1], topi_ref[1])
    rl0 = (NQB - 1) * TQ
    EG, EB = 16, _P.get('EB', 64)
    oslot = ((NSTEP - 1) % 2) * TQ
    ds = []
    for r in range(0, TQ, EB):
        d = jnp.dot(o_ref[oslot + r:oslot + r + EB, :], wob[NHG - 1], preferred_element_type=f32)
        acc_ref[rl0 + r:rl0 + r + EB, :] += d
        ds.append(d)

    def late(tc):
        per = EB * 8
        if tc < 0 or tc >= len(ds) * per:
            return None
        d = ds[tc // per]
        c = (tc % per) // EB
        tk = jnp.abs(d[0:8, c * 128:(c + 1) * 128]) < 0.0
        return jnp.concatenate([tk] * (EG // 8), axis=0)

    L1, L2 = _P.get('EL', [100, 400])
    for r in range(-CH, TQ, EG):
        ready = (r // EB + 1) * EB * 8 + (r % EB) * 8
        top, _ = fin_rows(rl0 + r, rl0 + r, EG, None, top, None, late(ready + L1), late(ready + L2))
        if r == -EG:
            cp_out(NQB - 2).start()
    cp_out(NQB - 1).start()

    if _P.get('ESPLIT', 0):
        scope('epi_ffn')
    vals = jnp.concatenate([top[0], top[2]], axis=0)
    idxs = jnp.concatenate([top[1], top[3]], axis=0)
    m1 = jnp.max(vals, axis=0, keepdims=True)
    i1v = jnp.min(jnp.where(vals == m1, idxs, S - 1), axis=0, keepdims=True)
    vals2 = jnp.where(idxs == i1v, -jnp.inf, vals)
    m2 = jnp.max(vals2, axis=0, keepdims=True)
    i2v = jnp.min(jnp.where(jnp.logical_and(vals2 == m2, idxs != i1v), idxs, S - 1), axis=0, keepdims=True)
    b1 = pl.multiple_of(jnp.clip(i1v[0, 0], 0, S - 1) // 8 * 8, 8)
    b2 = pl.multiple_of(jnp.clip(i2v[0, 0], 0, S - 1) // 8 * 8, 8)

    def two(ref_rows):
        return jnp.concatenate([ref_rows(b1), ref_rows(b2)], axis=0)

    def lanes(v):
        return jnp.concatenate([v] * (D // 128), axis=1)

    x1 = two(lambda b: xb[pl.ds(b, 8), :].astype(f32)) + bc(2, 16) * two(lambda b: acc_ref[pl.ds(b, 8), :])
    xn = (x1 - lanes(two(lambda b: st_ref[0, pl.ds(b, 8), :]))) * lanes(two(lambda b: st_ref[1, pl.ds(b, 8), :]))
    h2 = xn * bc(4, 16) + bc(3, 16)
    xs = h2.astype(bf16)
    FC = _P.get('FC', 512)
    y = None
    prev = None
    for c in range(0, F + FC, FC):
        if c < F:
            g = jnp.dot(xs, wgb[:, c:c + FC], preferred_element_type=f32)
            u = jnp.dot(xs, wub[:, c:c + FC], preferred_element_type=f32)
        if prev is not None:
            d = jnp.dot(prev, wdb[c - FC:c, :], preferred_element_type=f32)
            y = d if y is None else y + d
        if c < F:
            prev = (g * jax.nn.sigmoid(g) * u).astype(bf16)
    sub = lax.broadcasted_iota(jnp.int32, (8, 128), 0)
    ids = jnp.concatenate([sub + b1, sub + b2], axis=0)
    is1 = lanes(ids == i1v)
    is2 = lanes(ids == i2v)
    upd = jnp.where(is1, y * lanes(jax.nn.sigmoid(m1)), jnp.where(is2, y * lanes(jax.nn.sigmoid(m2)), 0.0))
    fixb[...] = ((x1 + bc(7, 16)) + xn * bc(8, 16) + bc(5, 16) * upd).astype(bf16)

    scope('epi_out')
    for qb in range(NQB):
        cp_out(qb).wait()
    cf1 = pltpu.make_async_copy(fixb.at[pl.ds(0, 8)], o_hbm.at[pl.ds(b1, 8)], sem_o.at[NQB])
    cf2 = pltpu.make_async_copy(fixb.at[pl.ds(8, 8)], o_hbm.at[pl.ds(b2, 8)], sem_o.at[NQB + 1])
    cf1.start()

    @pl.when(b1 != b2)
    def _():
        cf2.start()
        cf2.wait()
    cf1.wait()
    scope(None)


@jax.jit
def pallas_adaLN_cond__mha_block_cached__moe_arch_mod__prompt_kernel(
    A_x, A_k_cache, A_v_cache, A_wq, A_wo, B_x, B_w_r, B_w_gate, B_w_up, B_w_down, c, w_mod,
):
    x = A_x.reshape(S, D)
    k = A_k_cache.reshape(NHG, HPS, S, DH)
    v = A_v_cache.reshape(NHG, HPS, S, DH)
    wo = A_wo.reshape(NHG, HPS * DH, D)
    wr = B_w_r
    anyspec = pl.BlockSpec(memory_space=pl.ANY)
    out = pl.pallas_call(
        _kernel,
        in_specs=[anyspec] * 11,
        out_specs=anyspec,
        out_shape=jax.ShapeDtypeStruct((S, D), bf16),
        scratch_shapes=[
            pltpu.VMEM((S, D), bf16),
            pltpu.VMEM((NHG, HPS, S // 2, DH), u32),
            pltpu.VMEM((NHG, HPS, S // 2, DH), u32),
            pltpu.VMEM((NHG, D // 2, HPS * DH), u32),
            pltpu.VMEM((NHG, HPS * DH // 2, D), u32),
            pltpu.VMEM((D // 2, F), u32),
            pltpu.VMEM((D // 2, F), u32),
            pltpu.VMEM((F // 2, D), u32),
            pltpu.VMEM((NMP + 1, D // 2, MPW), u32),
            pltpu.VMEM((8, 11 * D), f32),
            pltpu.VMEM((S // 2, D), u32),
            pltpu.VMEM((S, D), f32),
            pltpu.VMEM((S + CH, D), bf16),
            pltpu.VMEM((16, D), bf16),
            pltpu.VMEM((1, TQ, S), f32),
            pltpu.VMEM((1, TQ, S), f32),
            pltpu.VMEM((TQ // 2, S), u32),
            pltpu.VMEM((TQ // 2, S), u32),
            pltpu.VMEM((1, HPS, TQ, 128), f32),
            pltpu.VMEM((1, TQ, 128), f32),
            pltpu.VMEM((1, TQ, 128), f32),
            pltpu.VMEM((1, TQ, 128), f32),
            pltpu.VMEM((1, TQ, 128), f32),
            pltpu.VMEM((CH // 2, D), u32),
            pltpu.VMEM((TQ, HPS * DH), u32),
            pltpu.VMEM((2, S + CH, 128), f32),
            pltpu.VMEM((D, 128), f32),
            pltpu.VMEM((NMP + 1, 8, MPW), f32),
            pltpu.VMEM((2, 8, 128), f32),
            pltpu.VMEM((2, 8, 128), jnp.int32),
            pltpu.VMEM((D,), bf16),
            pltpu.VMEM((1, D), bf16),
            pltpu.SMEM((8,), jnp.int32),
            pltpu.SemaphoreType.DMA((2,)),
            pltpu.SemaphoreType.DMA((4,)),
            pltpu.SemaphoreType.DMA((NMC + NMP,)),
            pltpu.SemaphoreType.DMA((NHG,)),
            pltpu.SemaphoreType.DMA((NHG,)),
            pltpu.SemaphoreType.DMA((2 * NHG,)),
            pltpu.SemaphoreType.DMA((3 * HPS + 1,)),
            pltpu.SemaphoreType.DMA((3,)),
            pltpu.SemaphoreType.DMA((NQB + 2,)),
        ],
        compiler_params=pltpu.CompilerParams(vmem_limit_bytes=124 * 1024 * 1024, disable_bounds_checks=True,
                                             disable_semaphore_checks=True),
    )(x, k, v, A_wq, wo, wr, B_w_gate, B_w_up, B_w_down, c, w_mod)
    return out.reshape(1, S, D)
```

```python
import os, json
import jax
import jax.numpy as jnp
from jax import lax
import jax.experimental.pallas as pl
import jax.experimental.pallas.tpu as pltpu

S = 2048
S2 = S // 2
D = 1024
H = 32
DH = 128
F = 3584
EPS = 1e-5
LOG2E = 1.4426950408889634
TQ = 512
NQB = S // TQ
HPS = 4
NHG = H // HPS
NSTEP = NQB * NHG
CH = TQ // NHG
MPW = json.loads(os.environ.get('KP', '{}')).get('MPW', 640)
NMP = -(-4 * D // MPW)
NMC = 4
MCW = 2 * D // NMC
_P = dict(PADS=[5, 5, 5, 5], PADS0=[5, 5, 5, 0], SCOPE=0)
_P.update(json.loads(os.environ.get('KP', '{}')))

f32 = jnp.float32
bf16 = jnp.bfloat16
u32 = jnp.uint32


class _Scope:
    def __init__(self):
        self.cur = None

    def __call__(self, name):
        if not _P['SCOPE']:
            return
        if self.cur is not None:
            self.cur.__exit__(None, None, None)
            self.cur = None
        if name:
            self.cur = jax.named_scope(name)
            self.cur.__enter__()


def _mp_col(p):
    return min(p * MPW, 4 * D - MPW)


def _rb(x):
    return x.astype(bf16).astype(f32)


def _recip(x):
    r = pl.reciprocal(x, approx=True)
    return r * (2.0 - x * r)


def _rowsum(x, late=None):
    p = x[:, 0:128]
    for c in range(1, x.shape[1] // 128):
        p = p + x[:, c * 128:(c + 1) * 128]
    if late is not None:
        p = jnp.where(late, 0.0, p)
    return jnp.sum(p, axis=-1, keepdims=True)


def _center(x, late=None):
    m = _rowsum(x, late) * (1.0 / D)
    mb = _rb(m)
    return x - mb, mb, m - mb


def _rstd(xc, dm, late=None):
    v = jnp.maximum(_rowsum(xc * xc, late) * (1.0 / D) - dm * dm, 0.0)
    y = _rb(_rb(v) + EPS)
    return _recip(_rb(y * lax.rsqrt(y)))


def _ln(x, late1=None, late2=None):
    xc, _, dm = _center(x, late1)
    return xc * _rstd(xc, dm, late2)


def _kernel(x_hbm, k_hbm, v_hbm, wq_hbm, wo_hbm, wr_hbm, wg_hbm, wu_hbm, wd_hbm, c_hbm, wm_hbm,
            o_hbm,
            xb, kb, vb, wqb, wob, wgb, wub, wdb, wmb,
            mod_ref, h_ref, acc_ref, ob, fixb, s0_ref, s1_ref, p0_ref, p1_ref, m_ref,
            l0_ref, l1_ref, l2_ref, l3_ref, hs_ref, o_ref, st_ref, scb_ref, mp_ref, top_ref, topi_ref, wrb, cb_, z_ref,
            sem_s, sem_x, sem_wm, sem_k, sem_v, sem_w, sem_0, sem_f, sem_o):
    scope = _Scope()
    h_ref, p0_ref, p1_ref, o_ref, hs_ref = (r.bitcast(bf16) for r in (h_ref, p0_ref, p1_ref, o_ref, hs_ref))
    wm0_hbm = wm_hbm.bitcast(f32)
    k_hbm, v_hbm, wq_hbm, wo_hbm, wg_hbm, wu_hbm, wd_hbm, wm_hbm = (
        r.bitcast(u32) for r in (k_hbm, v_hbm, wq_hbm, wo_hbm, wg_hbm, wu_hbm, wd_hbm, wm_hbm))

    def w16(x):
        return pltpu.bitcast(x, bf16)

    X0 = TQ + 2 * CH
    X1 = X0 + TQ

    cp_c = pltpu.make_async_copy(c_hbm, cb_, sem_s.at[0])
    cp_wr = pltpu.make_async_copy(wr_hbm, wrb, sem_s.at[1])
    cp_x0 = pltpu.make_async_copy(x_hbm.at[pl.ds(0, TQ)], xb.at[pl.ds(0, TQ)], sem_x.at[0])
    cp_x0b = pltpu.make_async_copy(x_hbm.at[pl.ds(TQ, X0 - TQ)], xb.at[pl.ds(TQ, X0 - TQ)], sem_x.at[3])

    cp_x1 = pltpu.make_async_copy(x_hbm.at[pl.ds(X0, TQ)], xb.at[pl.ds(X0, TQ)], sem_x.at[1])
    cp_x2 = pltpu.make_async_copy(x_hbm.at[pl.ds(X1, S - X1)], xb.at[pl.ds(X1, S - X1)], sem_x.at[2])

    def cp_wm(i):
        return pltpu.make_async_copy(wm0_hbm.at[:, pl.ds(i * MCW, MCW)], s0_ref.at[0, :, pl.ds(i * MCW, MCW)], sem_wm.at[i])

    def cp_wmr(p):
        return pltpu.make_async_copy(wm_hbm.at[:, pl.ds(2 * D + _mp_col(p), MPW)], wmb.at[p], sem_wm.at[NMC + p])

    def cp_k(g):
        rows = pl.ds(pl.multiple_of(g * (HPS * S2), HPS * S2), HPS * S2)
        return pltpu.make_async_copy(k_hbm.at[rows], kb.at[rows], sem_k.at[g])

    def cp_v(g):
        rows = pl.ds(pl.multiple_of(g * (HPS * S2), HPS * S2), HPS * S2)
        return pltpu.make_async_copy(v_hbm.at[rows], vb.at[rows], sem_v.at[g])

    def cp_wq(g):
        cols = pl.ds(pl.multiple_of(g * (HPS * DH), HPS * DH), HPS * DH)
        return pltpu.make_async_copy(wq_hbm.at[:, cols], wqb.at[g], sem_w.at[g])

    def cp_wo(g):
        return pltpu.make_async_copy(wo_hbm.at[g], wob.at[g], sem_w.at[NHG + g])

    cp0_wq = [pltpu.make_async_copy(wq_hbm.at[:, pl.ds(j * DH, DH)], wqb.at[0, :, pl.ds(j * DH, DH)], sem_0.at[j])
              for j in range(HPS)]
    cp0_k = [pltpu.make_async_copy(k_hbm.at[pl.ds(j * S2, S2)], kb.at[pl.ds(j * S2, S2)], sem_0.at[HPS + j]) for j in range(HPS)]
    cp0_v = [pltpu.make_async_copy(v_hbm.at[pl.ds(j * S2, S2)], vb.at[pl.ds(j * S2, S2)], sem_0.at[2 * HPS + j]) for j in range(HPS)]

    cp_ffn = [pltpu.make_async_copy(wg_hbm, wgb, sem_f.at[0]),
              pltpu.make_async_copy(wu_hbm, wub, sem_f.at[1]),
              pltpu.make_async_copy(wd_hbm, wdb, sem_f.at[2])]

    def cp_out(qb):
        rows = pl.ds(pl.multiple_of(qb * TQ, TQ), TQ)
        return pltpu.make_async_copy(ob.at[rows], o_hbm.at[rows], sem_o.at[qb])

    scope('pro_zero')
    cp_c.start()
    cp_x0.start()
    for i in range(NMC):
        cp_wm(i).start()
    for cp in (cp0_wq[0], cp0_k[0], cp0_wq[1], cp0_k[1], cp0_v[0], cp0_wq[2], cp0_k[2], cp0_v[1],
               cp0_wq[3], cp0_k[3], cp_x0b, cp0_v[2], cp0_v[3], cp_wr):
        cp.start()
    for g in range(1, NHG):
        for cp in [cp_wq(g), cp_k(g), cp_v(g), cp_wo(g - 1)] + ([cp_x1] if g == 1 else []) + ([cp_wmr(g - 1)] if g <= NMP else []):
            cp.start()
    for cp in [cp_wo(NHG - 1), cp_x2] + cp_ffn:
        cp.start()

    def zbody(i, _):
        rows = pl.ds(pl.multiple_of(i * 256, 256), 256)
        acc_ref[rows, :] = jnp.zeros((256, D), f32)
        wmb[NMP, pl.ds(pl.multiple_of(i * 64, 64), 64), :] = jnp.zeros((64, MPW), u32)
        z_ref[i] = 0
        return 0
    lax.fori_loop(0, S // 256, zbody, 0)
    mod_ref[...] = jnp.zeros(mod_ref.shape, f32)
    top_ref[...] = jnp.full(top_ref.shape, -jnp.inf, f32)
    topi_ref[0] = jnp.zeros((8, 128), jnp.int32)
    topi_ref[1] = jnp.ones((8, 128), jnp.int32)

    def bc(lo, n):
        p = mod_ref[:, lo * D:(lo + 1) * D]
        return p if n == 8 else jnp.concatenate([p] * (n // 8), axis=0)

    def tie(x, tok):
        if tok is None:
            return x
        return jnp.concatenate([jnp.where(tok < 0.0, 0.0, x[:, 0:128]), x[:, 128:]], axis=1)

    scope('pro_ln')
    cp_x0.wait()

    def nbody(i, _):
        rows = pl.ds(pl.multiple_of(i * 128, 128), 128)
        s1_ref[0, rows, 0:D] = _ln(xb[rows, :].astype(f32))
        return 0
    lax.fori_loop(0, TQ // 128, nbody, 0)

    scope('pro_mod')
    cp_c.wait()

    def silu_c():
        c = cb_[...].astype(f32)
        sc = (c * jax.nn.sigmoid(c)).astype(bf16)
        return jnp.broadcast_to(sc, (8, D))

    def mod_part(lo, width, plus_one):
        w = w16(s0_ref[0, :, lo:lo + width])
        md = _rb(jnp.dot(silu_c(), w, preferred_element_type=f32))
        if plus_one:
            md = _rb(1.0 + md)
        mod_ref[:, lo:lo + width] = md

    scf = silu_c().astype(f32)
    for b in range(D // 128):
        blk = jnp.concatenate([scf[:, b * 128:(b + 1) * 128]] * 16, axis=0)
        scb_ref[b * 128:(b + 1) * 128, :] = blk.T

    for i in range(NMC):
        cp_wm(i).wait()
        mod_part(i * MCW, MCW, i * MCW >= D)

    def ln1_rows(r0, n, tok=None, dst=None, late1=None, late2=None):
        x = tie(xb[pl.ds(r0, n), :].astype(f32), tok)
        h = _ln(x, late1, late2) * bc(1, n) + bc(0, n)
        if dst is None:
            h_ref[pl.ds(pl.multiple_of(r0, 16), n), :] = h.astype(bf16)
        else:
            hs_ref[pl.ds(dst, n), :] = h.astype(bf16)
        return jnp.abs(h[:, 0:128])

    def derive_params():
        for c in range(4 * D // 128):
            p = c * 128 // MPW
            o = c * 128 - _mp_col(p)
            md = _rb(jnp.broadcast_to(jnp.sum(mp_ref[p, :, o:o + 128], axis=0, keepdims=True), (8, 128)))
            if 2 * D <= c * 128 < 3 * D:
                md = _rb(1.0 + md)
            mod_ref[:, 2 * D + c * 128:2 * D + (c + 1) * 128] = md
        sb, cb1, gb, wr = bc(3, 8), bc(4, 8), bc(5, 8), bc(6, 8)
        mod_ref[:, 7 * D:8 * D] = gb * sb
        mod_ref[:, 8 * D:9 * D] = gb * cb1
        mod_ref[:, 9 * D:10 * D] = cb1 * wr
        mod_ref[:, 10 * D:10 * D + 128] = jnp.broadcast_to(jnp.sum(sb * wr, axis=-1, keepdims=True), (8, 128))

    def fin_rows(r0, d0, n, valid, top, tok=None, late1=None, late2=None):
        x = tie(xb[pl.ds(r0, n), :].astype(f32), tok)
        x1 = x + bc(2, n) * acc_ref[pl.ds(r0, n), :]
        xc, mb, dm = _center(x1, late1)
        rs = _rstd(xc, dm, late2)
        st_ref[0, pl.ds(d0, n), :] = jnp.broadcast_to(mb, (n, 128))
        st_ref[1, pl.ds(d0, n), :] = jnp.broadcast_to(rs, (n, 128))
        ob[pl.ds(d0, n), :] = ((x1 + bc(7, n)) + (xc * rs) * bc(8, n)).astype(bf16)
        rc = mod_ref[:, 10 * D:10 * D + 128]
        r = jnp.broadcast_to(_rowsum(xc * bc(9, n), late2) * rs, (n, 128))
        r = _rb(r + jnp.concatenate([rc] * (n // 8), axis=0))
        tok = jnp.abs(r)
        if valid is not None:
            r = jnp.where(valid, r, -jnp.inf)
        b1, i1, b2, i2 = top
        sub = lax.broadcasted_iota(jnp.int32, (8, 128), 0)
        for g in range(n // 8):
            rg = r[g * 8:(g + 1) * 8, :]
            ids = sub + (r0 + g * 8)
            gt1 = rg > b1
            gt2 = rg > b2
            b2 = jnp.where(gt1, b1, jnp.where(gt2, rg, b2))
            i2 = jnp.where(gt1, i1, jnp.where(gt2, ids, i2))
            b1 = jnp.where(gt1, rg, b1)
            i1 = jnp.where(gt1, ids, i1)
        return (b1, i1, b2, i2), tok

    s_refs = (s0_ref, s1_ref)
    p_refs = (p0_ref, p1_ref)
    l_refs = (l0_ref, l1_ref, l2_ref, l3_ref)

    def attend(t, first):
        qb = t // NHG
        hg = t % NHG
        slot = t % 2
        pads = _P['PADS0'] if first else _P['PADS']
        z = z_ref[0]
        z2 = z_ref[1]
        zp = pl.multiple_of(z * 16, 16)
        arows = pl.ds(pl.multiple_of(qb * TQ, TQ), TQ)
        kv0 = 0 if first else pl.multiple_of(hg * (HPS * S2), HPS * S2)
        early = [None]
        svals = {}
        mv = [jnp.zeros((8, 128), f32), 0]
        mpi = jnp.where(jnp.logical_and(t >= 2, t < 2 + NMP), t - 2, NMP)

        def qp(j):
            if first and j == 1:
                d0 = jnp.dot(h_ref[arows, 0:512], w16(wqb[hg, 0:256, j * DH:(j + 1) * DH]), preferred_element_type=f32)
                early[0] = jnp.abs(d0[0:16])
                q = d0 + jnp.dot(h_ref[arows, 512:], w16(wqb[hg, 256:, j * DH:(j + 1) * DH]), preferred_element_type=f32)
            else:
                q = jnp.dot(h_ref[arows, :], w16(wqb[hg, :, j * DH:(j + 1) * DH]), preferred_element_type=f32)
            return q * (DH ** -0.5 * LOG2E)

        def qk(j, q):
            s = lax.dot_general(q.astype(bf16), w16(kb[pl.ds(kv0 + j * S2, S2), :]), (((1,), (1,)), ((), ())),
                                preferred_element_type=f32)
            svals[j] = s
            s_refs[j % 2][z] = s
            pm = s[:, 0:128]
            for c in range(1, S // 128):
                pm = jnp.maximum(pm, s[:, c * 128:(c + 1) * 128])
            m_ref[z, j] = jnp.broadcast_to(jnp.max(pm, axis=-1, keepdims=True), (TQ, 128))

        def sm(j, tok=None):
            R, W = 16, S // 2
            sref = s_refs[j % 2]
            zs = z_ref[3 + j]
            for r in range(0, TQ, R):
                m = m_ref[zs, j, r:r + R, :]
                acc = None
                for hf in range(2):
                    mm = m if tok is None else jnp.where(tok < 0.0, 0.0, m)
                    ps = []
                    for c in range(W // 128):
                        c0 = hf * W + c * 128
                        pc = jnp.exp2(sref[zs, r:r + R, c0:c0 + 128] - mm)
                        ps.append(pc)
                        acc = pc if acc is None else acc + pc
                    if first or j != 1:
                        tok = acc
                        for _ in range(pads[j]):
                            tok = tok + tok
                    else:
                        never = jnp.minimum(acc[0:8], acc[8:16]) < 0.0
                        a = jnp.where(never, 1.0, mv[0])
                        for _ in range(MPW // 128):
                            mc, k0 = divmod(mv[1], D)
                            mv[1] += 16
                            w = w16(wmb[mpi, k0 // 2:k0 // 2 + 8, mc * 128:(mc + 1) * 128]).astype(f32)
                            pr = w * scb_ref[k0:k0 + 16, :]
                            a = (a + pr[0:8]) + pr[8:16]
                            tok = a
                            if k0 + 16 == D:
                                mp_ref[mpi, :, mc * 128:(mc + 1) * 128] = a
                                a = jnp.where(jnp.abs(a) < 0.0, 1.0, 0.0)
                        mv[0] = a
                        tok = jnp.abs(tok)
                        tok = jnp.concatenate([tok, tok], axis=0)
                    p_refs[j % 2][pl.ds(zp + r, R), hf * W:(hf + 1) * W] = jnp.concatenate(ps, axis=1).astype(bf16)
                l_refs[j][z, r:r + R, :] = acc

        def pv(j):
            pj = p_refs[j % 2]
            vv = w16(vb[pl.ds(kv0 + j * S2, S2), :])
            d0 = jnp.dot(pj[pl.ds(zp, TQ), 0:512], vv[0:512], preferred_element_type=f32)
            o = d0 + jnp.dot(pj[pl.ds(zp, TQ), 512:], vv[512:], preferred_element_type=f32)
            early[0] = jnp.abs(d0[0:16])
            lp = jnp.maximum(l_refs[j][z2], jnp.minimum(d0, 0.0))
            l = jnp.broadcast_to(jnp.sum(lp, axis=-1, keepdims=True), (TQ, 128))
            o_ref[pl.ds(pl.multiple_of(slot * TQ, TQ), TQ), j * DH:(j + 1) * DH] = (o * _recip(l)).astype(bf16)

        def op_prev():
            tp = t - 1
            o = o_ref[pl.ds(pl.multiple_of((1 - slot) * TQ, TQ), TQ), :]
            rows = pl.ds(pl.multiple_of((tp // NHG) * TQ, TQ), TQ)
            d = jnp.dot(o, w16(wob[tp % NHG]), preferred_element_type=f32)
            acc_ref[rows, :] += d

        def wait(*cps):
            if first:
                for cp in cps:
                    cp.wait()

        def both(tok):
            tok = jnp.minimum(tok[0:8], tok[8:16])
            return jnp.concatenate([tok, tok], axis=0)

        def late(j, tc):
            c, r8 = (tc // TQ) * 4, (tc % TQ) // 8 * 8
            tk = jnp.abs(svals[j][r8:r8 + 8, c * 128:(c + 1) * 128]) < 0.0
            return jnp.concatenate([tk, tk], axis=0)

        def finalize():
            valid = t > NHG
            fsrc = pl.multiple_of(jnp.maximum(t - NHG - 1, 0) * CH, CH)
            fdst = pl.multiple_of(jnp.where(valid, fsrc, S), CH)
            top = (top_ref[0], topi_ref[0], top_ref[1], topi_ref[1])
            tok = None
            fp = _P.get('FP')
            for g in range(CH // 16):
                if fp:
                    top, tk = fin_rows(fsrc + g * 16, fdst + g * 16, 16, valid, top, None,
                                       late(0, fp[0] + g * fp[1]), late(0, fp[0] + g * fp[1] + fp[2]))
                    tok = tk if tok is None else jnp.minimum(tok, tk)
                else:
                    top, tok = fin_rows(fsrc + g * 16, fdst + g * 16, 16, valid, top, tok)
            top_ref[0], topi_ref[0], top_ref[1], topi_ref[1] = top
            return both(tok)

        l0 = pl.multiple_of(jnp.minimum(t + NHG, NSTEP - 1) * CH, CH)

        def ln1(tok, staged, j=None):
            lp_ = _P.get('LP') if j is not None else None
            out = None
            for g in range(CH // 16):
                if lp_:
                    tk = ln1_rows(l0 + g * 16, 16, None, zp + g * 16,
                                  late(j, lp_[0] + g * lp_[1]), late(j, lp_[0] + g * lp_[1] + lp_[2]))
                    out = tk if out is None else jnp.minimum(out, tk)
                else:
                    out = tok = ln1_rows(l0 + g * 16, 16, tok, zp + g * 16 if staged else None)
            return both(out)

        if first:
            wait(cp0_wq[0])
            h_ref[0:TQ, :] = (s1_ref[0, :, 0:D] * bc(1, TQ) + bc(0, TQ)).astype(bf16)
            q0 = qp(0)
            wait(cp0_k[0])
            qk(0, q0)
            wait(cp0_wq[1], cp0_k[1], cp0_v[0], cp0_wq[2])
            q1 = qp(1)
            sm(0, early[0])
            qk(1, q1)
            sm(1)
            pv(0)
            q2 = qp(2)
            wait(cp0_k[2], cp0_v[1], cp0_wq[3], cp0_k[3], cp_x0b)
            qk(2, q2)
            sm(2)
            pv(1)
            q3 = qp(3)
            qk(3, q3)
            ln1(jnp.abs(q3[TQ - 16:TQ, :]), False)
            wait(cp0_v[2], cp0_v[3], cp_wr)
            pv(2)
            sm(3, early[0])
            pv(3)
            return

        if not _P.get('FP'):
            ftok = finalize()
        qk(0, qp(0))
        if _P.get('FP'):
            ftok = finalize()
        q1 = qp(1)
        sm(0, ftok)
        lj = _P.get('LJ', 1)
        if not _P.get('LP'):
            ltok = ln1(jnp.abs(q1[0:16]), True)
        qk(1, q1)
        if _P.get('LP') and lj == 1:
            ltok = ln1(None, True, 1)
        sm(1, ltok if lj == 1 else None)
        pv(0)
        qk(2, qp(2))
        if _P.get('LP') and lj == 2:
            ltok = ln1(None, True, 2)
        sm(2, ltok if lj == 2 else None)
        pv(1)
        qk(3, qp(3))
        sm(3)
        pv(2)
        lm = jnp.concatenate([early[0][0:8]] * (D // 128), axis=1) < 0.0
        for g in range(0, CH, 16):
            hv = hs_ref[pl.ds(pl.multiple_of(z2 * 16, 16) + g, 16), :].astype(f32)
            hv = jnp.concatenate([jnp.where(lm, 0.0, hv[0:8]), hv[8:16]], axis=0)
            h_ref[pl.ds(l0 + g, 16), :] = hv.astype(bf16)
        op_prev()
        pv(3)

    scope('step0')
    attend(0, True)
    mod_ref[:, 6 * D:7 * D] = jnp.broadcast_to(wrb[...].astype(f32).reshape(1, D), (8, D))
    scope(None)

    def step(t, _):
        scope('step_head')
        hg = t % NHG

        @pl.when(jnp.logical_or(t <= NHG, hg == 1))
        def _():
            @pl.when(t < NHG)
            def _():
                cp_wq(hg).wait()
                cp_k(hg).wait()
                cp_v(hg).wait()
                cp_wo(hg - 1).wait()

            @pl.when(t == 2)
            def _():
                cp_x1.wait()

            for p in range(NMP):
                @pl.when(t == 2 + p)
                def _():
                    cp_wmr(p).wait()

            @pl.when(t == NHG)
            def _():
                cp_x2.wait()
                cp_wo(NHG - 1).wait()

            @pl.when(t == NHG + 1)
            def _():
                derive_params()

            @pl.when(t >= 2 * NHG)
            def _():
                cp_out(t // NHG - 2).start()

        scope('step_body')
        attend(t, False)
        scope(None)
        return 0

    lax.fori_loop(1, NSTEP, step, 0)

    scope('epi_fin')
    for cp in cp_ffn:
        cp.wait()
    top = (top_ref[0], topi_ref[0], top_ref[1], topi_ref[1])
    rl0 = (NQB - 1) * TQ
    EG, EB = 16, _P.get('EB', 64)
    oslot = ((NSTEP - 1) % 2) * TQ
    ds = []
    for r in range(0, TQ, EB):
        d = jnp.dot(o_ref[oslot + r:oslot + r + EB, :], w16(wob[NHG - 1]), preferred_element_type=f32)
        acc_ref[rl0 + r:rl0 + r + EB, :] += d
        ds.append(d)

    def late(tc):
        per = EB * 8
        if tc < 0 or tc >= len(ds) * per:
            return None
        d = ds[tc // per]
        c = (tc % per) // EB
        tk = jnp.abs(d[0:8, c * 128:(c + 1) * 128]) < 0.0
        return jnp.concatenate([tk] * (EG // 8), axis=0)

    L1, L2 = _P.get('EL', [100, 400])
    for r in range(-CH, TQ, EG):
        ready = (r // EB + 1) * EB * 8 + (r % EB) * 8
        top, _ = fin_rows(rl0 + r, rl0 + r, EG, None, top, None, late(ready + L1), late(ready + L2))
        if r == -EG:
            cp_out(NQB - 2).start()
    cp_out(NQB - 1).start()

    if _P.get('ESPLIT', 0):
        scope('epi_ffn')
    vals = jnp.concatenate([top[0], top[2]], axis=0)
    idxs = jnp.concatenate([top[1], top[3]], axis=0)
    m1 = jnp.max(vals, axis=0, keepdims=True)
    i1v = jnp.min(jnp.where(vals == m1, idxs, S - 1), axis=0, keepdims=True)
    vals2 = jnp.where(idxs == i1v, -jnp.inf, vals)
    m2 = jnp.max(vals2, axis=0, keepdims=True)
    i2v = jnp.min(jnp.where(jnp.logical_and(vals2 == m2, idxs != i1v), idxs, S - 1), axis=0, keepdims=True)
    b1 = pl.multiple_of(jnp.clip(i1v[0, 0], 0, S - 1) // 8 * 8, 8)
    b2 = pl.multiple_of(jnp.clip(i2v[0, 0], 0, S - 1) // 8 * 8, 8)

    def two(ref_rows):
        return jnp.concatenate([ref_rows(b1), ref_rows(b2)], axis=0)

    def lanes(v):
        return jnp.concatenate([v] * (D // 128), axis=1)

    x1 = two(lambda b: xb[pl.ds(b, 8), :].astype(f32)) + bc(2, 16) * two(lambda b: acc_ref[pl.ds(b, 8), :])
    xn = (x1 - lanes(two(lambda b: st_ref[0, pl.ds(b, 8), :]))) * lanes(two(lambda b: st_ref[1, pl.ds(b, 8), :]))
    h2 = xn * bc(4, 16) + bc(3, 16)
    xs = h2.astype(bf16)
    FC = _P.get('FC', 512)
    y = None
    prev = None
    for c in range(0, F + FC, FC):
        if c < F:
            g = jnp.dot(xs, w16(wgb[:, c:c + FC]), preferred_element_type=f32)
            u = jnp.dot(xs, w16(wub[:, c:c + FC]), preferred_element_type=f32)
        if prev is not None:
            d = jnp.dot(prev, w16(wdb[(c - FC) // 2:c // 2, :]), preferred_element_type=f32)
            y = d if y is None else y + d
        if c < F:
            prev = (g * jax.nn.sigmoid(g) * u).astype(bf16)
    sub = lax.broadcasted_iota(jnp.int32, (8, 128), 0)
    ids = jnp.concatenate([sub + b1, sub + b2], axis=0)
    is1 = lanes(ids == i1v)
    is2 = lanes(ids == i2v)
    upd = jnp.where(is1, y * lanes(jax.nn.sigmoid(m1)), jnp.where(is2, y * lanes(jax.nn.sigmoid(m2)), 0.0))
    fixb[...] = ((x1 + bc(7, 16)) + xn * bc(8, 16) + bc(5, 16) * upd).astype(bf16)

    scope('epi_out')
    for qb in range(NQB):
        cp_out(qb).wait()
    cf1 = pltpu.make_async_copy(fixb.at[pl.ds(0, 8)], o_hbm.at[pl.ds(b1, 8)], sem_o.at[NQB])
    cf2 = pltpu.make_async_copy(fixb.at[pl.ds(8, 8)], o_hbm.at[pl.ds(b2, 8)], sem_o.at[NQB + 1])
    cf1.start()

    @pl.when(b1 != b2)
    def _():
        cf2.start()
        cf2.wait()
    cf1.wait()
    scope(None)


@jax.jit
def pallas_adaLN_cond__mha_block_cached__moe_arch_mod__prompt_kernel(
    A_x, A_k_cache, A_v_cache, A_wq, A_wo, B_x, B_w_r, B_w_gate, B_w_up, B_w_down, c, w_mod,
):
    x = A_x.reshape(S, D)
    k = A_k_cache.reshape(H * S, DH)
    v = A_v_cache.reshape(H * S, DH)
    wo = A_wo.reshape(NHG, HPS * DH, D)
    wr = B_w_r
    anyspec = pl.BlockSpec(memory_space=pl.ANY)
    out = pl.pallas_call(
        _kernel,
        in_specs=[anyspec] * 11,
        out_specs=anyspec,
        out_shape=jax.ShapeDtypeStruct((S, D), bf16),
        scratch_shapes=[
            pltpu.VMEM((S, D), bf16),
            pltpu.VMEM((H * S // 2, DH), u32),
            pltpu.VMEM((H * S // 2, DH), u32),
            pltpu.VMEM((NHG, D // 2, HPS * DH), u32),
            pltpu.VMEM((NHG, HPS * DH // 2, D), u32),
            pltpu.VMEM((D // 2, F), u32),
            pltpu.VMEM((D // 2, F), u32),
            pltpu.VMEM((F // 2, D), u32),
            pltpu.VMEM((NMP + 1, D // 2, MPW), u32),
            pltpu.VMEM((8, 11 * D), f32),
            pltpu.VMEM((S // 2, D), u32),
            pltpu.VMEM((S, D), f32),
            pltpu.VMEM((S + CH, D), bf16),
            pltpu.VMEM((16, D), bf16),
            pltpu.VMEM((1, TQ, S), f32),
            pltpu.VMEM((1, TQ, S), f32),
            pltpu.VMEM((TQ // 2, S), u32),
            pltpu.VMEM((TQ // 2, S), u32),
            pltpu.VMEM((1, HPS, TQ, 128), f32),
            pltpu.VMEM((1, TQ, 128), f32),
            pltpu.VMEM((1, TQ, 128), f32),
            pltpu.VMEM((1, TQ, 128), f32),
            pltpu.VMEM((1, TQ, 128), f32),
            pltpu.VMEM((CH // 2, D), u32),
            pltpu.VMEM((TQ, HPS * DH), u32),
            pltpu.VMEM((2, S + CH, 128), f32),
            pltpu.VMEM((D, 128), f32),
            pltpu.VMEM((NMP + 1, 8, MPW), f32),
            pltpu.VMEM((2, 8, 128), f32),
            pltpu.VMEM((2, 8, 128), jnp.int32),
            pltpu.VMEM((D,), bf16),
            pltpu.VMEM((1, D), bf16),
            pltpu.SMEM((8,), jnp.int32),
            pltpu.SemaphoreType.DMA((2,)),
            pltpu.SemaphoreType.DMA((4,)),
            pltpu.SemaphoreType.DMA((NMC + NMP,)),
            pltpu.SemaphoreType.DMA((NHG,)),
            pltpu.SemaphoreType.DMA((NHG,)),
            pltpu.SemaphoreType.DMA((2 * NHG,)),
            pltpu.SemaphoreType.DMA((3 * HPS + 1,)),
            pltpu.SemaphoreType.DMA((3,)),
            pltpu.SemaphoreType.DMA((NQB + 2,)),
        ],
        compiler_params=pltpu.CompilerParams(vmem_limit_bytes=124 * 1024 * 1024, disable_bounds_checks=True,
                                             disable_semaphore_checks=True),
    )(x, k, v, A_wq, wo, wr, B_w_gate, B_w_up, B_w_down, c, w_mod)
    return out.reshape(1, S, D)
```

```python
import jax
import jax.numpy as jnp
from jax import lax
import jax.experimental.pallas as pl
import jax.experimental.pallas.tpu as pltpu

S = 2048
S2 = S // 2
D = 1024
H = 32
DH = 128
F = 3584
EPS = 1e-5
LOG2E = 1.4426950408889634
TQ = 512
NQB = S // TQ
HPS = 4
NHG = H // HPS
NSTEP = NQB * NHG
CH = TQ // NHG
MPW = 768
NMP = -(-4 * D // MPW)
NMC = 4
MCW = 2 * D // NMC
PADS = (6, 5, 6, 4)
PADS0 = (5, 5, 5, 0)

f32 = jnp.float32
bf16 = jnp.bfloat16
u32 = jnp.uint32


def _mp_col(p):
    return min(p * MPW, 4 * D - MPW)


def _rb(x):
    return x.astype(bf16).astype(f32)


def _recip(x):
    r = pl.reciprocal(x, approx=True)
    return r * (2.0 - x * r)


def _rowsum(x, late=None):
    p = x[:, 0:128]
    for c in range(1, x.shape[1] // 128):
        p = p + x[:, c * 128:(c + 1) * 128]
    if late is not None:
        p = jnp.where(late, 0.0, p)
    return jnp.sum(p, axis=-1, keepdims=True)


def _center(x, late=None):
    m = _rowsum(x, late) * (1.0 / D)
    mb = _rb(m)
    return x - mb, mb, m - mb


def _rstd(xc, dm, late=None):
    v = jnp.maximum(_rowsum(xc * xc, late) * (1.0 / D) - dm * dm, 0.0)
    y = _rb(_rb(v) + EPS)
    return _recip(_rb(y * lax.rsqrt(y)))


def _ln(x):
    xc, _, dm = _center(x)
    return xc * _rstd(xc, dm)


def _tie(x, tok):
    if tok is None:
        return x
    return jnp.concatenate([jnp.where(tok < 0.0, 0.0, x[:, 0:128]), x[:, 128:]], axis=1)


def _both(tok):
    tok = jnp.minimum(tok[0:8], tok[8:16])
    return jnp.concatenate([tok, tok], axis=0)


def _lanes(v):
    return jnp.concatenate([v] * (D // 128), axis=1)


def _w16(x):
    return pltpu.bitcast(x, bf16)


def _kernel(x_hbm, k_hbm, v_hbm, wq_hbm, wo_hbm, wr_hbm, wg_hbm, wu_hbm, wd_hbm, c_hbm, wm_hbm,
            o_hbm,
            xb, kb, vb, wqb, wob, wgb, wub, wdb, wmb,
            mod_ref, h_ref, acc_ref, ob, fixb, s0_ref, s1_ref, p0_ref, p1_ref, m_ref,
            l0_ref, l1_ref, l2_ref, l3_ref, hs_ref, o_ref, st_ref, scb_ref, mp_ref, top_ref, topi_ref,
            wrb, cb_, z_ref,
            sem_s, sem_x, sem_wm, sem_k, sem_v, sem_w, sem_0, sem_f, sem_o):
    h_ref, p0_ref, p1_ref, o_ref, hs_ref = (r.bitcast(bf16) for r in (h_ref, p0_ref, p1_ref, o_ref, hs_ref))
    wm0_hbm = wm_hbm.bitcast(f32)
    k_hbm, v_hbm, wq_hbm, wo_hbm, wg_hbm, wu_hbm, wd_hbm, wm_hbm = (
        r.bitcast(u32) for r in (k_hbm, v_hbm, wq_hbm, wo_hbm, wg_hbm, wu_hbm, wd_hbm, wm_hbm))

    cp_c = pltpu.make_async_copy(c_hbm, cb_, sem_s.at[0])
    cp_wr = pltpu.make_async_copy(wr_hbm, wrb, sem_s.at[1])
    xcuts = (0, TQ, TQ + 2 * CH, 2 * TQ + 2 * CH, S)
    cp_x = [pltpu.make_async_copy(x_hbm.at[pl.ds(a, b - a)], xb.at[pl.ds(a, b - a)], sem_x.at[i])
            for i, (a, b) in enumerate(zip(xcuts, xcuts[1:]))]

    def cp_wm(i):
        cols = pl.ds(i * MCW, MCW)
        return pltpu.make_async_copy(wm0_hbm.at[:, cols], s0_ref.at[0, :, cols], sem_wm.at[i])

    def cp_wmr(p):
        return pltpu.make_async_copy(wm_hbm.at[:, pl.ds(2 * D + _mp_col(p), MPW)], wmb.at[p], sem_wm.at[NMC + p])

    def cp_k(g):
        rows = pl.ds(pl.multiple_of(g * (HPS * S2), HPS * S2), HPS * S2)
        return pltpu.make_async_copy(k_hbm.at[rows], kb.at[rows], sem_k.at[g])

    def cp_v(g):
        rows = pl.ds(pl.multiple_of(g * (HPS * S2), HPS * S2), HPS * S2)
        return pltpu.make_async_copy(v_hbm.at[rows], vb.at[rows], sem_v.at[g])

    def cp_wq(g):
        cols = pl.ds(pl.multiple_of(g * (HPS * DH), HPS * DH), HPS * DH)
        return pltpu.make_async_copy(wq_hbm.at[:, cols], wqb.at[g], sem_w.at[g])

    def cp_wo(g):
        return pltpu.make_async_copy(wo_hbm.at[g], wob.at[g], sem_w.at[NHG + g])

    cp0_wq = [pltpu.make_async_copy(wq_hbm.at[:, pl.ds(j * DH, DH)], wqb.at[0, :, pl.ds(j * DH, DH)], sem_0.at[j])
              for j in range(HPS)]
    cp0_k = [pltpu.make_async_copy(k_hbm.at[pl.ds(j * S2, S2)], kb.at[pl.ds(j * S2, S2)], sem_0.at[HPS + j])
             for j in range(HPS)]
    cp0_v = [pltpu.make_async_copy(v_hbm.at[pl.ds(j * S2, S2)], vb.at[pl.ds(j * S2, S2)], sem_0.at[2 * HPS + j])
             for j in range(HPS)]

    cp_ffn = [pltpu.make_async_copy(wg_hbm, wgb, sem_f.at[0]),
              pltpu.make_async_copy(wu_hbm, wub, sem_f.at[1]),
              pltpu.make_async_copy(wd_hbm, wdb, sem_f.at[2])]

    def cp_out(qb):
        rows = pl.ds(pl.multiple_of(qb * TQ, TQ), TQ)
        return pltpu.make_async_copy(ob.at[rows], o_hbm.at[rows], sem_o.at[qb])

    cp_c.start()
    cp_x[0].start()
    for i in range(NMC):
        cp_wm(i).start()
    for cp in (cp0_wq[0], cp0_k[0], cp0_wq[1], cp0_k[1], cp0_v[0], cp0_wq[2], cp0_k[2], cp0_v[1],
               cp0_wq[3], cp0_k[3], cp_x[1], cp0_v[2], cp0_v[3], cp_wr):
        cp.start()
    for g in range(1, NHG):
        cps = [cp_wq(g), cp_k(g), cp_v(g), cp_wo(g - 1)]
        cps += [cp_x[2]] if g == 1 else []
        cps += [cp_wmr(g - 1)] if g <= NMP else []
        for cp in cps:
            cp.start()
    for cp in [cp_wo(NHG - 1), cp_x[3]] + cp_ffn:
        cp.start()

    def zbody(i, _):
        acc_ref[pl.ds(pl.multiple_of(i * 256, 256), 256), :] = jnp.zeros((256, D), f32)
        wmb[NMP, pl.ds(pl.multiple_of(i * 64, 64), 64), :] = jnp.zeros((64, MPW), u32)
        z_ref[i] = 0
        return 0
    lax.fori_loop(0, S // 256, zbody, 0)
    mod_ref[...] = jnp.zeros(mod_ref.shape, f32)
    top_ref[...] = jnp.full(top_ref.shape, -jnp.inf, f32)
    topi_ref[0] = jnp.zeros((8, 128), jnp.int32)
    topi_ref[1] = jnp.ones((8, 128), jnp.int32)

    def bc(k, n):
        p = mod_ref[:, k * D:(k + 1) * D]
        return p if n == 8 else jnp.concatenate([p] * (n // 8), axis=0)

    cp_x[0].wait()

    def nbody(i, _):
        rows = pl.ds(pl.multiple_of(i * 128, 128), 128)
        s1_ref[0, rows, 0:D] = _ln(xb[rows, :].astype(f32))
        return 0
    lax.fori_loop(0, TQ // 128, nbody, 0)

    cp_c.wait()

    def silu_c():
        c = cb_[...].astype(f32)
        sc = (c * jax.nn.sigmoid(c)).astype(bf16)
        return jnp.broadcast_to(sc, (8, D))

    scf = silu_c().astype(f32)
    for b in range(D // 128):
        blk = jnp.concatenate([scf[:, b * 128:(b + 1) * 128]] * 16, axis=0)
        scb_ref[b * 128:(b + 1) * 128, :] = blk.T

    for i in range(NMC):
        cp_wm(i).wait()
        lo = i * MCW
        md = _rb(jnp.dot(silu_c(), _w16(s0_ref[0, :, lo:lo + MCW]), preferred_element_type=f32))
        mod_ref[:, lo:lo + MCW] = _rb(1.0 + md) if lo >= D else md

    def ln1_rows(r0, n, tok, dst_ref, d0):
        x = _tie(xb[pl.ds(r0, n), :].astype(f32), tok)
        h = _ln(x) * bc(1, n) + bc(0, n)
        dst_ref[pl.ds(d0, n), :] = h.astype(bf16)
        return jnp.abs(h[:, 0:128])

    def derive_params():
        for c in range(4 * D // 128):
            p = c * 128 // MPW
            o = c * 128 - _mp_col(p)
            md = _rb(jnp.broadcast_to(jnp.sum(mp_ref[p, :, o:o + 128], axis=0, keepdims=True), (8, 128)))
            if 2 * D <= c * 128 < 3 * D:
                md = _rb(1.0 + md)
            mod_ref[:, 2 * D + c * 128:2 * D + (c + 1) * 128] = md
        sb, cb1, gb, wr = bc(3, 8), bc(4, 8), bc(5, 8), bc(6, 8)
        mod_ref[:, 7 * D:8 * D] = gb * sb
        mod_ref[:, 8 * D:9 * D] = gb * cb1
        mod_ref[:, 9 * D:10 * D] = cb1 * wr
        mod_ref[:, 10 * D:10 * D + 128] = jnp.broadcast_to(jnp.sum(sb * wr, axis=-1, keepdims=True), (8, 128))

    def fin_rows(r0, d0, n, valid, top, tok=None, late1=None, late2=None, write=True):
        x = _tie(xb[pl.ds(r0, n), :].astype(f32), tok)
        x1 = x + bc(2, n) * acc_ref[pl.ds(r0, n), :]
        xc, mb, dm = _center(x1, late1)
        rs = _rstd(xc, dm, late2)
        st_ref[0, pl.ds(d0, n), :] = jnp.broadcast_to(mb, (n, 128))
        st_ref[1, pl.ds(d0, n), :] = jnp.broadcast_to(rs, (n, 128))
        if write:
            ob[pl.ds(d0, n), :] = ((x1 + bc(7, n)) + (xc * rs) * bc(8, n)).astype(bf16)
        rc = mod_ref[:, 10 * D:10 * D + 128]
        r = jnp.broadcast_to(_rowsum(xc * bc(9, n), late2) * rs, (n, 128))
        r = _rb(r + jnp.concatenate([rc] * (n // 8), axis=0))
        tok = jnp.abs(r)
        if valid is not None:
            r = jnp.where(valid, r, -jnp.inf)
        b1, i1, b2, i2 = top
        sub = lax.broadcasted_iota(jnp.int32, (8, 128), 0)
        for g in range(n // 8):
            rg = r[g * 8:(g + 1) * 8, :]
            ids = sub + (r0 + g * 8)
            gt1 = rg > b1
            gt2 = rg > b2
            b2 = jnp.where(gt1, b1, jnp.where(gt2, rg, b2))
            i2 = jnp.where(gt1, i1, jnp.where(gt2, ids, i2))
            b1 = jnp.where(gt1, rg, b1)
            i1 = jnp.where(gt1, ids, i1)
        return (b1, i1, b2, i2), tok

    s_refs = (s0_ref, s1_ref)
    p_refs = (p0_ref, p1_ref)
    l_refs = (l0_ref, l1_ref, l2_ref, l3_ref)

    def attend(t, first):
        qb = t // NHG
        hg = t % NHG
        slot = t % 2
        pads = PADS0 if first else PADS
        z = z_ref[0]
        z2 = z_ref[1]
        zp = pl.multiple_of(z * 16, 16)
        arows = pl.ds(pl.multiple_of(qb * TQ, TQ), TQ)
        kv0 = 0 if first else pl.multiple_of(hg * (HPS * S2), HPS * S2)
        early = [None]
        mv = [jnp.zeros((8, 128), f32), 0]
        mpi = jnp.where(jnp.logical_and(t >= 2, t < 2 + NMP), t - 2, NMP)

        def qp(j):
            cols = slice(j * DH, (j + 1) * DH)
            if first and j == 1:
                d0 = jnp.dot(h_ref[arows, 0:512], _w16(wqb[hg, 0:256, cols]), preferred_element_type=f32)
                early[0] = jnp.abs(d0[0:16])
                q = d0 + jnp.dot(h_ref[arows, 512:], _w16(wqb[hg, 256:, cols]), preferred_element_type=f32)
            else:
                q = jnp.dot(h_ref[arows, :], _w16(wqb[hg, :, cols]), preferred_element_type=f32)
            return q * (DH ** -0.5 * LOG2E)

        def qk(j, q):
            s = lax.dot_general(q.astype(bf16), _w16(kb[pl.ds(kv0 + j * S2, S2), :]), (((1,), (1,)), ((), ())),
                                preferred_element_type=f32)
            s_refs[j % 2][z] = s
            pm = s[:, 0:128]
            for c in range(1, S // 128):
                pm = jnp.maximum(pm, s[:, c * 128:(c + 1) * 128])
            m_ref[z, j] = jnp.broadcast_to(jnp.max(pm, axis=-1, keepdims=True), (TQ, 128))
            return jnp.abs(s[0:16, 0:128])

        def sm(j, tok=None):
            R, W = 16, S // 2
            sref = s_refs[j % 2]
            zs = z_ref[3 + j]
            for r in range(0, TQ, R):
                m = m_ref[zs, j, r:r + R, :]
                acc = None
                for hf in range(2):
                    mm = m if tok is None else jnp.where(tok < 0.0, 0.0, m)
                    ps = []
                    for c in range(W // 128):
                        c0 = hf * W + c * 128
                        pc = jnp.exp2(sref[zs, r:r + R, c0:c0 + 128] - mm)
                        ps.append(pc)
                        acc = pc if acc is None else acc + pc
                    if first or j != 1:
                        tok = acc
                        for _ in range(pads[j]):
                            tok = tok + tok
                    else:
                        a = jnp.where(jnp.minimum(acc[0:8], acc[8:16]) < 0.0, 1.0, mv[0])
                        for _ in range(MPW // 128):
                            mc, k0 = divmod(mv[1], D)
                            mv[1] += 16
                            w = _w16(wmb[mpi, k0 // 2:k0 // 2 + 8, mc * 128:(mc + 1) * 128]).astype(f32)
                            pr = w * scb_ref[k0:k0 + 16, :]
                            a = (a + pr[0:8]) + pr[8:16]
                            tok = a
                            if k0 + 16 == D:
                                mp_ref[mpi, :, mc * 128:(mc + 1) * 128] = a
                                a = jnp.where(jnp.abs(a) < 0.0, 1.0, 0.0)
                        mv[0] = a
                        tok = jnp.abs(tok)
                        tok = jnp.concatenate([tok, tok], axis=0)
                    p_refs[j % 2][pl.ds(zp + r, R), hf * W:(hf + 1) * W] = jnp.concatenate(ps, axis=1).astype(bf16)
                l_refs[j][z, r:r + R, :] = acc

        def pv(j, between=None):
            pj = p_refs[j % 2]
            vv = _w16(vb[pl.ds(kv0 + j * S2, S2), :])
            d0 = jnp.dot(pj[pl.ds(zp, TQ), 0:512], vv[0:512], preferred_element_type=f32)
            o = d0 + jnp.dot(pj[pl.ds(zp, TQ), 512:], vv[512:], preferred_element_type=f32)
            early[0] = jnp.abs(d0[0:16])
            lp = jnp.maximum(l_refs[j][z2], jnp.minimum(d0, 0.0))
            l = jnp.broadcast_to(jnp.sum(lp, axis=-1, keepdims=True), (TQ, 128))
            if between is not None:
                between()
            o_ref[pl.ds(pl.multiple_of(slot * TQ, TQ), TQ), j * DH:(j + 1) * DH] = (o * _recip(l)).astype(bf16)

        def op_prev(c0, c1):
            tp = t - 1
            o = o_ref[pl.ds(pl.multiple_of((1 - slot) * TQ, TQ), TQ), :]
            rows = pl.ds(pl.multiple_of((tp // NHG) * TQ, TQ), TQ)
            d = jnp.dot(o, _w16(wob[tp % NHG, :, c0:c1]), preferred_element_type=f32)
            acc_ref[rows, c0:c1] += d
            return d

        def wait(*cps):
            for cp in cps:
                cp.wait()

        l0 = pl.multiple_of(jnp.minimum(t + NHG, NSTEP - 1) * CH, CH)

        if first:
            wait(cp0_wq[0])
            h_ref[0:TQ, :] = (s1_ref[0, :, 0:D] * bc(1, TQ) + bc(0, TQ)).astype(bf16)
            q0 = qp(0)
            wait(cp0_k[0])
            qk(0, q0)
            wait(cp0_wq[1], cp0_k[1], cp0_v[0], cp0_wq[2])
            q1 = qp(1)
            sm(0, early[0])
            qk(1, q1)
            sm(1)
            pv(0)
            q2 = qp(2)
            wait(cp0_k[2], cp0_v[1], cp0_wq[3], cp0_k[3], cp_x[1])
            qk(2, q2)
            sm(2)
            pv(1)
            q3 = qp(3)
            qk(3, q3)
            tok = jnp.abs(q3[TQ - 16:TQ, :])
            for g in range(0, CH, 16):
                tok = ln1_rows(l0 + g, 16, tok, h_ref, pl.multiple_of(l0 + g, 16))
            wait(cp0_v[2], cp0_v[3], cp_wr)
            pv(2)
            sm(3, early[0])
            pv(3)
            return

        valid = t > NHG
        fsrc = pl.multiple_of(jnp.maximum(t - NHG - 1, 0) * CH, CH)
        fdst = pl.multiple_of(jnp.where(valid, fsrc, S), CH)
        top = (top_ref[0], topi_ref[0], top_ref[1], topi_ref[1])
        tok = None
        for g in range(0, CH, 16):
            top, tok = fin_rows(fsrc + g, fdst + g, 16, valid, top, tok)
        top_ref[0], topi_ref[0], top_ref[1], topi_ref[1] = top

        qk(0, qp(0))
        q1 = qp(1)
        sm(0, _both(tok))
        tok = jnp.abs(q1[0:16])
        for g in range(0, CH, 16):
            tok = ln1_rows(l0 + g, 16, tok, hs_ref, zp + g)
        qk(1, q1)
        sm(1, _both(tok))
        pv(0)
        qk(2, qp(2))
        sm(2)
        pv(1)
        sm(3, qk(3, qp(3)))
        pv(2)
        never = _lanes(jnp.abs(op_prev(0, D // 2)[0:8, 0:128])) < 0.0
        for g in range(0, CH, 16):
            hv = hs_ref[pl.ds(pl.multiple_of(z2 * 16, 16) + g, 16), :].astype(f32)
            hv = jnp.concatenate([jnp.where(never, 0.0, hv[0:8]), hv[8:16]], axis=0)
            h_ref[pl.ds(l0 + g, 16), :] = hv.astype(bf16)
        op_prev(D // 2, D - 128)
        pv(3, lambda: op_prev(D - 128, D))

    attend(0, True)
    mod_ref[:, 6 * D:7 * D] = jnp.broadcast_to(wrb[...].astype(f32).reshape(1, D), (8, D))

    def step(t, _):
        hg = t % NHG

        @pl.when(jnp.logical_or(t <= NHG, hg == 1))
        def _():
            @pl.when(t < NHG)
            def _():
                cp_wq(hg).wait()
                cp_k(hg).wait()
                cp_v(hg).wait()
                cp_wo(hg - 1).wait()

            @pl.when(t == 2)
            def _():
                cp_x[2].wait()

            for p in range(NMP):
                @pl.when(t == 2 + p)
                def _():
                    cp_wmr(p).wait()

            @pl.when(t == NHG)
            def _():
                cp_x[3].wait()
                cp_wo(NHG - 1).wait()

            @pl.when(t == NHG + 1)
            def _():
                derive_params()

            @pl.when(t >= 2 * NHG)
            def _():
                cp_out(t // NHG - 2).start()

        attend(t, False)
        return 0

    lax.fori_loop(1, NSTEP, step, 0)

    for cp in cp_ffn:
        cp.wait()
    top = (top_ref[0], topi_ref[0], top_ref[1], topi_ref[1])
    rl0 = (NQB - 1) * TQ
    EG, EB = 16, 64
    oslot = ((NSTEP - 1) % 2) * TQ
    ds = []
    for r in range(0, TQ, EB):
        d = jnp.dot(o_ref[oslot + r:oslot + r + EB, :], _w16(wob[NHG - 1]), preferred_element_type=f32)
        acc_ref[rl0 + r:rl0 + r + EB, :] += d
        ds.append(d)

    def late(tc):
        if tc >= TQ * 8:
            return None
        c = (tc % (EB * 8)) // EB
        tk = jnp.abs(ds[tc // (EB * 8)][0:8, c * 128:(c + 1) * 128]) < 0.0
        return jnp.concatenate([tk] * (EG // 8), axis=0)

    for r in range(-CH, TQ, EG):
        ready = (r + EB) * 8
        top, _ = fin_rows(rl0 + r, rl0 + r, EG, None, top, None, late(ready + 100), late(ready + 400),
                          write=r < TQ - EB)
        if r == -EG:
            cp_out(NQB - 2).start()

    vals = jnp.concatenate([top[0], top[2]], axis=0)
    idxs = jnp.concatenate([top[1], top[3]], axis=0)
    m1 = jnp.max(vals, axis=0, keepdims=True)
    i1v = jnp.min(jnp.where(vals == m1, idxs, S - 1), axis=0, keepdims=True)
    vals2 = jnp.where(idxs == i1v, -jnp.inf, vals)
    m2 = jnp.max(vals2, axis=0, keepdims=True)
    i2v = jnp.min(jnp.where(jnp.logical_and(vals2 == m2, idxs != i1v), idxs, S - 1), axis=0, keepdims=True)
    b1 = pl.multiple_of(jnp.clip(i1v[0, 0] // 8 * 8, 0, S - 8), 8)
    b2 = pl.multiple_of(jnp.clip(i2v[0, 0] // 8 * 8, 0, S - 8), 8)

    def two(ref_rows):
        return jnp.concatenate([ref_rows(b1), ref_rows(b2)], axis=0)

    x1 = two(lambda b: xb[pl.ds(b, 8), :].astype(f32)) + bc(2, 16) * two(lambda b: acc_ref[pl.ds(b, 8), :])
    xn = (x1 - _lanes(two(lambda b: st_ref[0, pl.ds(b, 8), :]))) * _lanes(two(lambda b: st_ref[1, pl.ds(b, 8), :]))
    xs = (xn * bc(4, 16) + bc(3, 16)).astype(bf16)
    FC = 512
    y = None
    prev = None
    for c in range(0, F + FC, FC):
        if c < F:
            g = jnp.dot(xs, _w16(wgb[:, c:c + FC]), preferred_element_type=f32)
            u = jnp.dot(xs, _w16(wub[:, c:c + FC]), preferred_element_type=f32)
        if prev is not None:
            d = jnp.dot(prev, _w16(wdb[(c - FC) // 2:c // 2, :]), preferred_element_type=f32)
            y = d if y is None else y + d
        if c < F:
            prev = (g * jax.nn.sigmoid(g) * u).astype(bf16)
        if c == 0:
            for gi, r0 in enumerate(range(S - EB, S, EG)):
                never = jnp.abs(g[:, gi * 128:(gi + 1) * 128]) < 0.0
                xx = xb[r0:r0 + EG, :].astype(f32) + bc(2, EG) * acc_ref[r0:r0 + EG, :]
                rs = jnp.where(never, 0.0, st_ref[1, r0:r0 + EG, :])
                mb = jnp.where(never, 0.0, st_ref[0, r0:r0 + EG, :])
                ob[r0:r0 + EG, :] = ((xx + bc(7, EG)) + ((xx - _lanes(mb)) * _lanes(rs)) * bc(8, EG)).astype(bf16)
            cp_out(NQB - 1).start()
    sub = lax.broadcasted_iota(jnp.int32, (8, 128), 0)
    ids = jnp.concatenate([sub + b1, sub + b2], axis=0)
    upd = jnp.where(_lanes(ids == i1v), y * _lanes(jax.nn.sigmoid(m1)),
                    jnp.where(_lanes(ids == i2v), y * _lanes(jax.nn.sigmoid(m2)), 0.0))
    fixb[...] = ((x1 + bc(7, 16)) + xn * bc(8, 16) + bc(5, 16) * upd).astype(bf16)

    for qb in range(NQB):
        cp_out(qb).wait()
    cf1 = pltpu.make_async_copy(fixb.at[pl.ds(0, 8)], o_hbm.at[pl.ds(b1, 8)], sem_o.at[NQB])
    cf2 = pltpu.make_async_copy(fixb.at[pl.ds(8, 8)], o_hbm.at[pl.ds(b2, 8)], sem_o.at[NQB + 1])
    cf1.start()

    @pl.when(b1 != b2)
    def _():
        cf2.start()
        cf2.wait()
    cf1.wait()


@jax.jit
def pallas_adaLN_cond__mha_block_cached__moe_arch_mod__prompt_kernel(
    A_x: jax.Array,
    A_k_cache: jax.Array,
    A_v_cache: jax.Array,
    A_wq: jax.Array,
    A_wo: jax.Array,
    B_x: jax.Array,
    B_w_r: jax.Array,
    B_w_gate: jax.Array,
    B_w_up: jax.Array,
    B_w_down: jax.Array,
    c: jax.Array,
    w_mod: jax.Array,
):
    x = A_x.reshape(S, D)
    k = A_k_cache.reshape(H * S, DH)
    v = A_v_cache.reshape(H * S, DH)
    wo = A_wo.reshape(NHG, HPS * DH, D)
    anyspec = pl.BlockSpec(memory_space=pl.ANY)
    out = pl.pallas_call(
        _kernel,
        in_specs=[anyspec] * 11,
        out_specs=anyspec,
        out_shape=jax.ShapeDtypeStruct((S, D), bf16),
        scratch_shapes=[
            pltpu.VMEM((S, D), bf16),
            pltpu.VMEM((H * S2, DH), u32),
            pltpu.VMEM((H * S2, DH), u32),
            pltpu.VMEM((NHG, D // 2, HPS * DH), u32),
            pltpu.VMEM((NHG, HPS * DH // 2, D), u32),
            pltpu.VMEM((D // 2, F), u32),
            pltpu.VMEM((D // 2, F), u32),
            pltpu.VMEM((F // 2, D), u32),
            pltpu.VMEM((NMP + 1, D // 2, MPW), u32),
            pltpu.VMEM((8, 11 * D), f32),
            pltpu.VMEM((S // 2, D), u32),
            pltpu.VMEM((S, D), f32),
            pltpu.VMEM((S + CH, D), bf16),
            pltpu.VMEM((16, D), bf16),
            pltpu.VMEM((1, TQ, S), f32),
            pltpu.VMEM((1, TQ, S), f32),
            pltpu.VMEM((TQ // 2, S), u32),
            pltpu.VMEM((TQ // 2, S), u32),
            pltpu.VMEM((1, HPS, TQ, 128), f32),
            pltpu.VMEM((1, TQ, 128), f32),
            pltpu.VMEM((1, TQ, 128), f32),
            pltpu.VMEM((1, TQ, 128), f32),
            pltpu.VMEM((1, TQ, 128), f32),
            pltpu.VMEM((CH // 2, D), u32),
            pltpu.VMEM((TQ, HPS * DH), u32),
            pltpu.VMEM((2, S + CH, 128), f32),
            pltpu.VMEM((D, 128), f32),
            pltpu.VMEM((NMP + 1, 8, MPW), f32),
            pltpu.VMEM((2, 8, 128), f32),
            pltpu.VMEM((2, 8, 128), jnp.int32),
            pltpu.VMEM((D,), bf16),
            pltpu.VMEM((1, D), bf16),
            pltpu.SMEM((8,), jnp.int32),
            pltpu.SemaphoreType.DMA((2,)),
            pltpu.SemaphoreType.DMA((4,)),
            pltpu.SemaphoreType.DMA((NMC + NMP,)),
            pltpu.SemaphoreType.DMA((NHG,)),
            pltpu.SemaphoreType.DMA((NHG,)),
            pltpu.SemaphoreType.DMA((2 * NHG,)),
            pltpu.SemaphoreType.DMA((3 * HPS,)),
            pltpu.SemaphoreType.DMA((3,)),
            pltpu.SemaphoreType.DMA((NQB + 2,)),
        ],
        compiler_params=pltpu.CompilerParams(vmem_limit_bytes=124 * 1024 * 1024, disable_bounds_checks=True,
                                             disable_semaphore_checks=True),
    )(x, k, v, A_wq, wo, B_w_r, B_w_gate, B_w_up, B_w_down, c, w_mod)
    return out.reshape(1, S, D)
```

```python
import jax
import jax.numpy as jnp
from jax import lax
import jax.experimental.pallas as pl
import jax.experimental.pallas.tpu as pltpu

S = 2048
S2 = S // 2
D = 1024
H = 32
DH = 128
F = 3584
EPS = 1e-5
LOG2E = 1.4426950408889634
TQ = 512
NQB = S // TQ
HPS = 4
NHG = H // HPS
NSTEP = NQB * NHG
CH = TQ // NHG
MPW = 768
NMP = -(-4 * D // MPW)
NMC = 4
MCW = 2 * D // NMC
PADS = (6, 5, 6, 4)
PADS0 = (5, 5, 5, 0)

f32 = jnp.float32
bf16 = jnp.bfloat16
u32 = jnp.uint32


def _mp_col(p):
    return min(p * MPW, 4 * D - MPW)


def _rb(x):
    return x.astype(bf16).astype(f32)


def _recip(x):
    r = pl.reciprocal(x, approx=True)
    return r * (2.0 - x * r)


def _rowsum(x, late=None):
    p = x[:, 0:128]
    for c in range(1, x.shape[1] // 128):
        p = p + x[:, c * 128:(c + 1) * 128]
    if late is not None:
        p = jnp.where(late, 0.0, p)
    return jnp.sum(p, axis=-1, keepdims=True)


def _center(x, late=None):
    m = _rowsum(x, late) * (1.0 / D)
    mb = _rb(m)
    return x - mb, mb, m - mb


def _rstd(xc, dm, late=None):
    v = jnp.maximum(_rowsum(xc * xc, late) * (1.0 / D) - dm * dm, 0.0)
    y = _rb(_rb(v) + EPS)
    return _recip(_rb(y * lax.rsqrt(y)))


def _ln(x):
    xc, _, dm = _center(x)
    return xc * _rstd(xc, dm)


def _tie(x, tok):
    if tok is None:
        return x
    return jnp.concatenate([jnp.where(tok < 0.0, 0.0, x[:, 0:128]), x[:, 128:]], axis=1)


def _both(tok):
    tok = jnp.minimum(tok[0:8], tok[8:16])
    return jnp.concatenate([tok, tok], axis=0)


def _lanes(v):
    return jnp.concatenate([v] * (D // 128), axis=1)


def _w16(x):
    return pltpu.bitcast(x, bf16)


def _kernel(x_hbm, k_hbm, v_hbm, wq_hbm, wo_hbm, wr_hbm, wg_hbm, wu_hbm, wd_hbm, c_hbm, wm_hbm,
            o_hbm,
            xb, kb, vb, wqb, wob, wgb, wub, wdb, wmb,
            mod_ref, h_ref, acc_ref, ob, fixb, s0_ref, s1_ref, p0_ref, p1_ref, m_ref,
            l0_ref, l1_ref, l2_ref, l3_ref, hs_ref, o_ref, st_ref, scb_ref, mp_ref, top_ref, topi_ref,
            wrb, cb_, z_ref,
            sem_s, sem_x, sem_wm, sem_k, sem_v, sem_w, sem_0, sem_f, sem_o):
    h_ref, p0_ref, p1_ref, o_ref, hs_ref = (r.bitcast(bf16) for r in (h_ref, p0_ref, p1_ref, o_ref, hs_ref))
    wm0_hbm = wm_hbm.bitcast(f32)
    k_hbm, v_hbm, wq_hbm, wo_hbm, wg_hbm, wu_hbm, wd_hbm, wm_hbm = (
        r.bitcast(u32) for r in (k_hbm, v_hbm, wq_hbm, wo_hbm, wg_hbm, wu_hbm, wd_hbm, wm_hbm))

    cp_c = pltpu.make_async_copy(c_hbm, cb_, sem_s.at[0])
    cp_wr = pltpu.make_async_copy(wr_hbm, wrb, sem_s.at[1])
    xcuts = (0, TQ, TQ + 2 * CH, 2 * TQ + 2 * CH, S)
    cp_x = [pltpu.make_async_copy(x_hbm.at[pl.ds(a, b - a)], xb.at[pl.ds(a, b - a)], sem_x.at[i])
            for i, (a, b) in enumerate(zip(xcuts, xcuts[1:]))]

    def cp_wm(i):
        cols = pl.ds(i * MCW, MCW)
        return pltpu.make_async_copy(wm0_hbm.at[:, cols], s0_ref.at[0, :, cols], sem_wm.at[i])

    def cp_wmr(p):
        return pltpu.make_async_copy(wm_hbm.at[:, pl.ds(2 * D + _mp_col(p), MPW)], wmb.at[p], sem_wm.at[NMC + p])

    def cp_k(g):
        rows = pl.ds(pl.multiple_of(g * (HPS * S2), HPS * S2), HPS * S2)
        return pltpu.make_async_copy(k_hbm.at[rows], kb.at[rows], sem_k.at[g])

    def cp_v(g):
        rows = pl.ds(pl.multiple_of(g * (HPS * S2), HPS * S2), HPS * S2)
        return pltpu.make_async_copy(v_hbm.at[rows], vb.at[rows], sem_v.at[g])

    def cp_wq(g):
        cols = pl.ds(pl.multiple_of(g * (HPS * DH), HPS * DH), HPS * DH)
        return pltpu.make_async_copy(wq_hbm.at[:, cols], wqb.at[g], sem_w.at[g])

    def cp_wo(g):
        return pltpu.make_async_copy(wo_hbm.at[g], wob.at[g], sem_w.at[NHG + g])

    cp0_wq = [pltpu.make_async_copy(wq_hbm.at[:, pl.ds(j * DH, DH)], wqb.at[0, :, pl.ds(j * DH, DH)], sem_0.at[j])
              for j in range(HPS)]
    cp0_k = [pltpu.make_async_copy(k_hbm.at[pl.ds(j * S2, S2)], kb.at[pl.ds(j * S2, S2)], sem_0.at[HPS + j])
             for j in range(HPS)]
    cp0_v = [pltpu.make_async_copy(v_hbm.at[pl.ds(j * S2, S2)], vb.at[pl.ds(j * S2, S2)], sem_0.at[2 * HPS + j])
             for j in range(HPS)]

    cp_ffn = [pltpu.make_async_copy(wg_hbm, wgb, sem_f.at[0]),
              pltpu.make_async_copy(wu_hbm, wub, sem_f.at[1]),
              pltpu.make_async_copy(wd_hbm, wdb, sem_f.at[2])]

    def cp_out(qb):
        rows = pl.ds(pl.multiple_of(qb * TQ, TQ), TQ)
        return pltpu.make_async_copy(ob.at[rows], o_hbm.at[rows], sem_o.at[qb])

    cp_c.start()
    cp_x[0].start()
    for i in range(NMC):
        cp_wm(i).start()
    for cp in (cp0_wq[0], cp0_k[0], cp0_wq[1], cp0_k[1], cp0_v[0], cp0_wq[2], cp0_k[2], cp0_v[1],
               cp0_wq[3], cp0_k[3], cp_x[1], cp0_v[2], cp0_v[3], cp_wr):
        cp.start()
    for g in range(1, NHG):
        cps = [cp_wq(g), cp_k(g), cp_v(g), cp_wo(g - 1)]
        cps += [cp_x[2]] if g == 1 else []
        cps += [cp_wmr(g - 1)] if g <= NMP else []
        for cp in cps:
            cp.start()
    for cp in [cp_wo(NHG - 1), cp_x[3]] + cp_ffn:
        cp.start()

    def zbody(i, _):
        acc_ref[pl.ds(pl.multiple_of(i * 256, 256), 256), :] = jnp.zeros((256, D), f32)
        wmb[NMP, pl.ds(pl.multiple_of(i * 64, 64), 64), :] = jnp.zeros((64, MPW), u32)
        z_ref[i] = 0
        return 0
    lax.fori_loop(0, S // 256, zbody, 0)
    mod_ref[...] = jnp.zeros(mod_ref.shape, f32)
    top_ref[...] = jnp.full(top_ref.shape, -jnp.inf, f32)
    topi_ref[0] = jnp.zeros((8, 128), jnp.int32)
    topi_ref[1] = jnp.ones((8, 128), jnp.int32)

    def bc(k, n):
        p = mod_ref[:, k * D:(k + 1) * D]
        return p if n == 8 else jnp.concatenate([p] * (n // 8), axis=0)

    cp_x[0].wait()

    def nbody(i, _):
        rows = pl.ds(pl.multiple_of(i * 128, 128), 128)
        s1_ref[0, rows, 0:D] = _ln(xb[rows, :].astype(f32))
        return 0
    lax.fori_loop(0, TQ // 128, nbody, 0)

    cp_c.wait()

    def silu_c():
        c = cb_[...].astype(f32)
        sc = (c * jax.nn.sigmoid(c)).astype(bf16)
        return jnp.broadcast_to(sc, (8, D))

    scf = silu_c().astype(f32)
    for b in range(D // 128):
        blk = jnp.concatenate([scf[:, b * 128:(b + 1) * 128]] * 16, axis=0)
        scb_ref[b * 128:(b + 1) * 128, :] = blk.T

    for i in range(NMC):
        cp_wm(i).wait()
        lo = i * MCW
        md = _rb(jnp.dot(silu_c(), _w16(s0_ref[0, :, lo:lo + MCW]), preferred_element_type=f32))
        mod_ref[:, lo:lo + MCW] = _rb(1.0 + md) if lo >= D else md

    def ln1_rows(r0, n, tok, dst_ref, d0):
        x = _tie(xb[pl.ds(r0, n), :].astype(f32), tok)
        h = _ln(x) * bc(1, n) + bc(0, n)
        dst_ref[pl.ds(d0, n), :] = h.astype(bf16)
        return jnp.abs(h[:, 0:128])

    def derive_params():
        for c in range(4 * D // 128):
            p = c * 128 // MPW
            o = c * 128 - _mp_col(p)
            md = _rb(jnp.broadcast_to(jnp.sum(mp_ref[p, :, o:o + 128], axis=0, keepdims=True), (8, 128)))
            if 2 * D <= c * 128 < 3 * D:
                md = _rb(1.0 + md)
            mod_ref[:, 2 * D + c * 128:2 * D + (c + 1) * 128] = md
        sb, cb1, gb, wr = bc(3, 8), bc(4, 8), bc(5, 8), bc(6, 8)
        mod_ref[:, 7 * D:8 * D] = gb * sb
        mod_ref[:, 8 * D:9 * D] = gb * cb1
        mod_ref[:, 9 * D:10 * D] = cb1 * wr
        mod_ref[:, 10 * D:10 * D + 128] = jnp.broadcast_to(jnp.sum(sb * wr, axis=-1, keepdims=True), (8, 128))

    def fin_rows(r0, d0, n, valid, top, tok=None, late1=None, late2=None, write=True):
        x = _tie(xb[pl.ds(r0, n), :].astype(f32), tok)
        x1 = x + bc(2, n) * acc_ref[pl.ds(r0, n), :]
        xc, mb, dm = _center(x1, late1)
        rs = _rstd(xc, dm, late2)
        st_ref[0, pl.ds(d0, n), :] = jnp.broadcast_to(mb, (n, 128))
        st_ref[1, pl.ds(d0, n), :] = jnp.broadcast_to(rs, (n, 128))
        if write:
            ob[pl.ds(d0, n), :] = ((x1 + bc(7, n)) + (xc * rs) * bc(8, n)).astype(bf16)
        rc = mod_ref[:, 10 * D:10 * D + 128]
        r = jnp.broadcast_to(_rowsum(xc * bc(9, n), late2) * rs, (n, 128))
        r = _rb(r + jnp.concatenate([rc] * (n // 8), axis=0))
        tok = jnp.abs(r)
        if valid is not None:
            r = jnp.where(valid, r, -jnp.inf)
        b1, i1, b2, i2 = top
        sub = lax.broadcasted_iota(jnp.int32, (8, 128), 0)
        for g in range(n // 8):
            rg = r[g * 8:(g + 1) * 8, :]
            ids = sub + (r0 + g * 8)
            gt1 = rg > b1
            gt2 = rg > b2
            b2 = jnp.where(gt1, b1, jnp.where(gt2, rg, b2))
            i2 = jnp.where(gt1, i1, jnp.where(gt2, ids, i2))
            b1 = jnp.where(gt1, rg, b1)
            i1 = jnp.where(gt1, ids, i1)
        return (b1, i1, b2, i2), tok

    s_refs = (s0_ref, s1_ref)
    p_refs = (p0_ref, p1_ref)
    l_refs = (l0_ref, l1_ref, l2_ref, l3_ref)

    def attend(t, first):
        qb = t // NHG
        hg = t % NHG
        slot = t % 2
        pads = PADS0 if first else PADS
        z = z_ref[0]
        z2 = z_ref[1]
        zp = pl.multiple_of(z * 16, 16)
        arows = pl.ds(pl.multiple_of(qb * TQ, TQ), TQ)
        kv0 = 0 if first else pl.multiple_of(hg * (HPS * S2), HPS * S2)
        early = [None]
        mv = [jnp.zeros((8, 128), f32), 0]
        mpi = jnp.where(jnp.logical_and(t >= 2, t < 2 + NMP), t - 2, NMP)

        def qp(j):
            cols = slice(j * DH, (j + 1) * DH)
            if first and j == 1:
                d0 = jnp.dot(h_ref[arows, 0:512], _w16(wqb[hg, 0:256, cols]), preferred_element_type=f32)
                early[0] = jnp.abs(d0[0:16])
                q = d0 + jnp.dot(h_ref[arows, 512:], _w16(wqb[hg, 256:, cols]), preferred_element_type=f32)
            else:
                q = jnp.dot(h_ref[arows, :], _w16(wqb[hg, :, cols]), preferred_element_type=f32)
            return q * (DH ** -0.5 * LOG2E)

        def qk(j, q):
            s = lax.dot_general(q.astype(bf16), _w16(kb[pl.ds(kv0 + j * S2, S2), :]), (((1,), (1,)), ((), ())),
                                preferred_element_type=f32)
            s_refs[j % 2][z] = s
            pm = s[:, 0:128]
            for c in range(1, S // 128):
                pm = jnp.maximum(pm, s[:, c * 128:(c + 1) * 128])
            m_ref[z, j] = jnp.broadcast_to(jnp.max(pm, axis=-1, keepdims=True), (TQ, 128))
            return jnp.abs(s[0:16, 0:128])

        def sm(j, tok=None):
            R, W = 16, S // 2
            sref = s_refs[j % 2]
            zs = z_ref[3 + j]
            for r in range(0, TQ, R):
                m = m_ref[zs, j, r:r + R, :]
                acc = None
                for hf in range(2):
                    mm = m if tok is None else jnp.where(tok < 0.0, 0.0, m)
                    p = jnp.exp2(sref[zs, r:r + R, hf * W:(hf + 1) * W] - _lanes(mm))
                    for c in range(W // 128):
                        pc = p[:, c * 128:(c + 1) * 128]
                        acc = pc if acc is None else acc + pc
                    if first or j != 1:
                        tok = acc
                        for _ in range(pads[j]):
                            tok = tok + tok
                    else:
                        a = jnp.where(jnp.minimum(acc[0:8], acc[8:16]) < 0.0, 1.0, mv[0])
                        for _ in range(MPW // 128):
                            mc, k0 = divmod(mv[1], D)
                            mv[1] += 16
                            w = _w16(wmb[mpi, k0 // 2:k0 // 2 + 8, mc * 128:(mc + 1) * 128]).astype(f32)
                            pr = w * scb_ref[k0:k0 + 16, :]
                            a = (a + pr[0:8]) + pr[8:16]
                            tok = a
                            if k0 + 16 == D:
                                mp_ref[mpi, :, mc * 128:(mc + 1) * 128] = a
                                a = jnp.where(jnp.abs(a) < 0.0, 1.0, 0.0)
                        mv[0] = a
                        tok = jnp.abs(tok)
                        tok = jnp.concatenate([tok, tok], axis=0)
                    p_refs[j % 2][pl.ds(zp + r, R), hf * W:(hf + 1) * W] = p.astype(bf16)
                l_refs[j][z, r:r + R, :] = acc

        def pv(j, between=None):
            pj = p_refs[j % 2]
            vv = _w16(vb[pl.ds(kv0 + j * S2, S2), :])
            d0 = jnp.dot(pj[pl.ds(zp, TQ), 0:512], vv[0:512], preferred_element_type=f32)
            o = d0 + jnp.dot(pj[pl.ds(zp, TQ), 512:], vv[512:], preferred_element_type=f32)
            early[0] = jnp.abs(d0[0:16])
            lp = jnp.maximum(l_refs[j][z2], jnp.minimum(d0, 0.0))
            l = jnp.broadcast_to(jnp.sum(lp, axis=-1, keepdims=True), (TQ, 128))
            if between is not None:
                between()
            o_ref[pl.ds(pl.multiple_of(slot * TQ, TQ), TQ), j * DH:(j + 1) * DH] = (o * _recip(l)).astype(bf16)

        def op_prev(c0, c1):
            tp = t - 1
            o = o_ref[pl.ds(pl.multiple_of((1 - slot) * TQ, TQ), TQ), :]
            rows = pl.ds(pl.multiple_of((tp // NHG) * TQ, TQ), TQ)
            d = jnp.dot(o, _w16(wob[tp % NHG, :, c0:c1]), preferred_element_type=f32)
            acc_ref[rows, c0:c1] += d
            return d

        def wait(*cps):
            for cp in cps:
                cp.wait()

        l0 = pl.multiple_of(jnp.minimum(t + NHG, NSTEP - 1) * CH, CH)

        if first:
            wait(cp0_wq[0])
            h_ref[0:TQ, :] = (s1_ref[0, :, 0:D] * bc(1, TQ) + bc(0, TQ)).astype(bf16)
            q0 = qp(0)
            wait(cp0_k[0])
            qk(0, q0)
            wait(cp0_wq[1], cp0_k[1], cp0_v[0], cp0_wq[2])
            q1 = qp(1)
            sm(0, early[0])
            qk(1, q1)
            sm(1)
            pv(0)
            q2 = qp(2)
            wait(cp0_k[2], cp0_v[1], cp0_wq[3], cp0_k[3], cp_x[1])
            qk(2, q2)
            sm(2)
            pv(1)
            q3 = qp(3)
            qk(3, q3)
            tok = jnp.abs(q3[TQ - 16:TQ, :])
            for g in range(0, CH, 16):
                tok = ln1_rows(l0 + g, 16, tok, h_ref, pl.multiple_of(l0 + g, 16))
            wait(cp0_v[2], cp0_v[3], cp_wr)
            pv(2)
            sm(3, early[0])
            pv(3)
            return

        valid = t > NHG
        fsrc = pl.multiple_of(jnp.maximum(t - NHG - 1, 0) * CH, CH)
        fdst = pl.multiple_of(jnp.where(valid, fsrc, S), CH)
        top = (top_ref[0], topi_ref[0], top_ref[1], topi_ref[1])
        tok = None
        for g in range(0, CH, 16):
            top, tok = fin_rows(fsrc + g, fdst + g, 16, valid, top, tok)
        top_ref[0], topi_ref[0], top_ref[1], topi_ref[1] = top

        qk(0, qp(0))
        q1 = qp(1)
        sm(0, _both(tok))
        tok = jnp.abs(q1[0:16])
        for g in range(0, CH, 16):
            tok = ln1_rows(l0 + g, 16, tok, hs_ref, zp + g)
        qk(1, q1)
        sm(1, _both(tok))
        pv(0)
        qk(2, qp(2))
        sm(2)
        pv(1)
        sm(3, qk(3, qp(3)))
        pv(2)
        never = _lanes(jnp.abs(op_prev(0, D // 2)[0:8, 0:128])) < 0.0
        for g in range(0, CH, 16):
            hv = hs_ref[pl.ds(pl.multiple_of(z2 * 16, 16) + g, 16), :].astype(f32)
            hv = jnp.concatenate([jnp.where(never, 0.0, hv[0:8]), hv[8:16]], axis=0)
            h_ref[pl.ds(l0 + g, 16), :] = hv.astype(bf16)
        op_prev(D // 2, D - 128)
        pv(3, lambda: op_prev(D - 128, D))

    attend(0, True)
    mod_ref[:, 6 * D:7 * D] = jnp.broadcast_to(wrb[...].astype(f32).reshape(1, D), (8, D))

    def step(t, _):
        hg = t % NHG

        @pl.when(jnp.logical_or(t <= NHG, hg == 1))
        def _():
            @pl.when(t < NHG)
            def _():
                cp_wq(hg).wait()
                cp_k(hg).wait()
                cp_v(hg).wait()
                cp_wo(hg - 1).wait()

            @pl.when(t == 2)
            def _():
                cp_x[2].wait()

            for p in range(NMP):
                @pl.when(t == 2 + p)
                def _():
                    cp_wmr(p).wait()

            @pl.when(t == NHG)
            def _():
                cp_x[3].wait()
                cp_wo(NHG - 1).wait()

            @pl.when(t == NHG + 1)
            def _():
                derive_params()

            @pl.when(t >= 2 * NHG)
            def _():
                cp_out(t // NHG - 2).start()

        attend(t, False)
        return 0

    lax.fori_loop(1, NSTEP, step, 0)

    for cp in cp_ffn:
        cp.wait()
    top = (top_ref[0], topi_ref[0], top_ref[1], topi_ref[1])
    rl0 = (NQB - 1) * TQ
    EG, EB = 16, 64
    oslot = ((NSTEP - 1) % 2) * TQ
    ds = []
    for r in range(0, TQ, EB):
        d = jnp.dot(o_ref[oslot + r:oslot + r + EB, :], _w16(wob[NHG - 1]), preferred_element_type=f32)
        acc_ref[rl0 + r:rl0 + r + EB, :] += d
        ds.append(d)

    def late(tc):
        if tc >= TQ * 8:
            return None
        c = (tc % (EB * 8)) // EB
        tk = jnp.abs(ds[tc // (EB * 8)][0:8, c * 128:(c + 1) * 128]) < 0.0
        return jnp.concatenate([tk] * (EG // 8), axis=0)

    for r in range(-CH, TQ, EG):
        ready = (r + EB) * 8
        top, _ = fin_rows(rl0 + r, rl0 + r, EG, None, top, None, late(ready + 100), late(ready + 400),
                          write=r < TQ - EB)
        if r == -EG:
            cp_out(NQB - 2).start()

    vals = jnp.concatenate([top[0], top[2]], axis=0)
    idxs = jnp.concatenate([top[1], top[3]], axis=0)
    m1 = jnp.max(vals, axis=0, keepdims=True)
    i1v = jnp.min(jnp.where(vals == m1, idxs, S - 1), axis=0, keepdims=True)
    vals2 = jnp.where(idxs == i1v, -jnp.inf, vals)
    m2 = jnp.max(vals2, axis=0, keepdims=True)
    i2v = jnp.min(jnp.where(jnp.logical_and(vals2 == m2, idxs != i1v), idxs, S - 1), axis=0, keepdims=True)
    b1 = pl.multiple_of(jnp.clip(i1v[0, 0] // 8 * 8, 0, S - 8), 8)
    b2 = pl.multiple_of(jnp.clip(i2v[0, 0] // 8 * 8, 0, S - 8), 8)

    def two(ref_rows):
        return jnp.concatenate([ref_rows(b1), ref_rows(b2)], axis=0)

    x1 = two(lambda b: xb[pl.ds(b, 8), :].astype(f32)) + bc(2, 16) * two(lambda b: acc_ref[pl.ds(b, 8), :])
    xn = (x1 - _lanes(two(lambda b: st_ref[0, pl.ds(b, 8), :]))) * _lanes(two(lambda b: st_ref[1, pl.ds(b, 8), :]))
    xs = (xn * bc(4, 16) + bc(3, 16)).astype(bf16)
    FC = 512
    y = None
    prev = None
    for c in range(0, F + FC, FC):
        if c < F:
            g = jnp.dot(xs, _w16(wgb[:, c:c + FC]), preferred_element_type=f32)
            u = jnp.dot(xs, _w16(wub[:, c:c + FC]), preferred_element_type=f32)
        if prev is not None:
            d = jnp.dot(prev, _w16(wdb[(c - FC) // 2:c // 2, :]), preferred_element_type=f32)
            y = d if y is None else y + d
        if c < F:
            prev = (g * jax.nn.sigmoid(g) * u).astype(bf16)
        if c == 0:
            for gi, r0 in enumerate(range(S - EB, S, EG)):
                never = jnp.abs(g[:, gi * 128:(gi + 1) * 128]) < 0.0
                xx = xb[r0:r0 + EG, :].astype(f32) + bc(2, EG) * acc_ref[r0:r0 + EG, :]
                rs = jnp.where(never, 0.0, st_ref[1, r0:r0 + EG, :])
                mb = jnp.where(never, 0.0, st_ref[0, r0:r0 + EG, :])
                ob[r0:r0 + EG, :] = ((xx + bc(7, EG)) + ((xx - _lanes(mb)) * _lanes(rs)) * bc(8, EG)).astype(bf16)
            cp_out(NQB - 1).start()
    sub = lax.broadcasted_iota(jnp.int32, (8, 128), 0)
    ids = jnp.concatenate([sub + b1, sub + b2], axis=0)
    upd = jnp.where(_lanes(ids == i1v), y * _lanes(jax.nn.sigmoid(m1)),
                    jnp.where(_lanes(ids == i2v), y * _lanes(jax.nn.sigmoid(m2)), 0.0))
    fixb[...] = ((x1 + bc(7, 16)) + xn * bc(8, 16) + bc(5, 16) * upd).astype(bf16)

    for qb in range(NQB):
        cp_out(qb).wait()
    cf1 = pltpu.make_async_copy(fixb.at[pl.ds(0, 8)], o_hbm.at[pl.ds(b1, 8)], sem_o.at[NQB])
    cf2 = pltpu.make_async_copy(fixb.at[pl.ds(8, 8)], o_hbm.at[pl.ds(b2, 8)], sem_o.at[NQB + 1])
    cf1.start()

    @pl.when(b1 != b2)
    def _():
        cf2.start()
        cf2.wait()
    cf1.wait()


@jax.jit
def pallas_adaLN_cond__mha_block_cached__moe_arch_mod__prompt_kernel(
    A_x: jax.Array,
    A_k_cache: jax.Array,
    A_v_cache: jax.Array,
    A_wq: jax.Array,
    A_wo: jax.Array,
    B_x: jax.Array,
    B_w_r: jax.Array,
    B_w_gate: jax.Array,
    B_w_up: jax.Array,
    B_w_down: jax.Array,
    c: jax.Array,
    w_mod: jax.Array,
):
    x = A_x.reshape(S, D)
    k = A_k_cache.reshape(H * S, DH)
    v = A_v_cache.reshape(H * S, DH)
    wo = A_wo.reshape(NHG, HPS * DH, D)
    anyspec = pl.BlockSpec(memory_space=pl.ANY)
    out = pl.pallas_call(
        _kernel,
        in_specs=[anyspec] * 11,
        out_specs=anyspec,
        out_shape=jax.ShapeDtypeStruct((S, D), bf16),
        scratch_shapes=[
            pltpu.VMEM((S, D), bf16),
            pltpu.VMEM((H * S2, DH), u32),
            pltpu.VMEM((H * S2, DH), u32),
            pltpu.VMEM((NHG, D // 2, HPS * DH), u32),
            pltpu.VMEM((NHG, HPS * DH // 2, D), u32),
            pltpu.VMEM((D // 2, F), u32),
            pltpu.VMEM((D // 2, F), u32),
            pltpu.VMEM((F // 2, D), u32),
            pltpu.VMEM((NMP + 1, D // 2, MPW), u32),
            pltpu.VMEM((8, 11 * D), f32),
            pltpu.VMEM((S // 2, D), u32),
            pltpu.VMEM((S, D), f32),
            pltpu.VMEM((S + CH, D), bf16),
            pltpu.VMEM((16, D), bf16),
            pltpu.VMEM((1, TQ, S), f32),
            pltpu.VMEM((1, TQ, S), f32),
            pltpu.VMEM((TQ // 2, S), u32),
            pltpu.VMEM((TQ // 2, S), u32),
            pltpu.VMEM((1, HPS, TQ, 128), f32),
            pltpu.VMEM((1, TQ, 128), f32),
            pltpu.VMEM((1, TQ, 128), f32),
            pltpu.VMEM((1, TQ, 128), f32),
            pltpu.VMEM((1, TQ, 128), f32),
            pltpu.VMEM((CH // 2, D), u32),
            pltpu.VMEM((TQ, HPS * DH), u32),
            pltpu.VMEM((2, S + CH, 128), f32),
            pltpu.VMEM((D, 128), f32),
            pltpu.VMEM((NMP + 1, 8, MPW), f32),
            pltpu.VMEM((2, 8, 128), f32),
            pltpu.VMEM((2, 8, 128), jnp.int32),
            pltpu.VMEM((D,), bf16),
            pltpu.VMEM((1, D), bf16),
            pltpu.SMEM((8,), jnp.int32),
            pltpu.SemaphoreType.DMA((2,)),
            pltpu.SemaphoreType.DMA((4,)),
            pltpu.SemaphoreType.DMA((NMC + NMP,)),
            pltpu.SemaphoreType.DMA((NHG,)),
            pltpu.SemaphoreType.DMA((NHG,)),
            pltpu.SemaphoreType.DMA((2 * NHG,)),
            pltpu.SemaphoreType.DMA((3 * HPS,)),
            pltpu.SemaphoreType.DMA((3,)),
            pltpu.SemaphoreType.DMA((NQB + 2,)),
        ],
        compiler_params=pltpu.CompilerParams(vmem_limit_bytes=124 * 1024 * 1024, disable_bounds_checks=True,
                                             disable_semaphore_checks=True),
    )(x, k, v, A_wq, wo, B_w_r, B_w_gate, B_w_up, B_w_down, c, w_mod)
    return out.reshape(1, S, D)
```

```python
import jax
import jax.numpy as jnp
from jax import lax
import jax.experimental.pallas as pl
import jax.experimental.pallas.tpu as pltpu

S = 2048
S2 = S // 2
D = 1024
H = 32
DH = 128
F = 3584
EPS = 1e-5
LOG2E = 1.4426950408889634
TQ = 512
NQB = S // TQ
HPS = 4
NHG = H // HPS
NSTEP = NQB * NHG
CH = TQ // NHG
MPW = 768
NMP = -(-4 * D // MPW)
NMC = 4
MCW = 2 * D // NMC
PADS = (6, 5, 6, 4)
PADS0 = (5, 5, 5, 0)

f32 = jnp.float32
bf16 = jnp.bfloat16
u32 = jnp.uint32


def _mp_col(p):
    return min(p * MPW, 4 * D - MPW)


def _rb(x):
    return x.astype(bf16).astype(f32)


def _recip(x):
    r = pl.reciprocal(x, approx=True)
    return r * (2.0 - x * r)


def _rowsum(x, late=None):
    p = x[:, 0:128]
    for c in range(1, x.shape[1] // 128):
        p = p + x[:, c * 128:(c + 1) * 128]
    if late is not None:
        p = jnp.where(late, 0.0, p)
    return jnp.sum(p, axis=-1, keepdims=True)


def _center(x, late=None):
    m = _rowsum(x, late) * (1.0 / D)
    mb = _rb(m)
    return x - mb, mb, m - mb


def _rstd(xc, dm, late=None):
    v = jnp.maximum(_rowsum(xc * xc, late) * (1.0 / D) - dm * dm, 0.0)
    y = _rb(_rb(v) + EPS)
    return _recip(_rb(y * lax.rsqrt(y)))


def _ln(x):
    xc, _, dm = _center(x)
    return xc * _rstd(xc, dm)


def _tie(x, tok):
    if tok is None:
        return x
    return jnp.concatenate([jnp.where(tok < 0.0, 0.0, x[:, 0:128]), x[:, 128:]], axis=1)


def _both(tok):
    tok = jnp.minimum(tok[0:8], tok[8:16])
    return jnp.concatenate([tok, tok], axis=0)


def _lanes(v):
    return jnp.concatenate([v] * (D // 128), axis=1)


def _w16(x):
    return pltpu.bitcast(x, bf16)


def _kernel(x_hbm, k_hbm, v_hbm, wq_hbm, wo_hbm, wr_hbm, wg_hbm, wu_hbm, wd_hbm, c_hbm, wm_hbm,
            o_hbm,
            xb, kb, vb, wqb, wob, wgb, wub, wdb, wmb,
            mod_ref, h_ref, acc_ref, ob, fixb, s0_ref, s1_ref, p0_ref, p1_ref, m_ref,
            l0_ref, l1_ref, l2_ref, l3_ref, hs_ref, o_ref, st_ref, scb_ref, mp_ref, top_ref, topi_ref,
            wrb, cb_, z_ref,
            sem_s, sem_x, sem_wm, sem_k, sem_v, sem_w, sem_0, sem_f, sem_o):
    h_ref, p0_ref, p1_ref, o_ref, hs_ref = (r.bitcast(bf16) for r in (h_ref, p0_ref, p1_ref, o_ref, hs_ref))
    wm0_hbm = wm_hbm.bitcast(f32)
    k_hbm, v_hbm, wq_hbm, wo_hbm, wg_hbm, wu_hbm, wd_hbm, wm_hbm = (
        r.bitcast(u32) for r in (k_hbm, v_hbm, wq_hbm, wo_hbm, wg_hbm, wu_hbm, wd_hbm, wm_hbm))

    cp_c = pltpu.make_async_copy(c_hbm, cb_, sem_s.at[0])
    cp_wr = pltpu.make_async_copy(wr_hbm, wrb, sem_s.at[1])
    xcuts = (0, TQ, TQ + 2 * CH, 2 * TQ + 2 * CH, S)
    cp_x = [pltpu.make_async_copy(x_hbm.at[pl.ds(a, b - a)], xb.at[pl.ds(a, b - a)], sem_x.at[i])
            for i, (a, b) in enumerate(zip(xcuts, xcuts[1:]))]

    def cp_wm(i):
        cols = pl.ds(i * MCW, MCW)
        return pltpu.make_async_copy(wm0_hbm.at[:, cols], s0_ref.at[0, :, cols], sem_wm.at[i])

    def cp_wmr(p):
        return pltpu.make_async_copy(wm_hbm.at[:, pl.ds(2 * D + _mp_col(p), MPW)], wmb.at[p], sem_wm.at[NMC + p])

    def cp_k(g):
        rows = pl.ds(pl.multiple_of(g * (HPS * S2), HPS * S2), HPS * S2)
        return pltpu.make_async_copy(k_hbm.at[rows], kb.at[rows], sem_k.at[g])

    def cp_v(g):
        rows = pl.ds(pl.multiple_of(g * (HPS * S2), HPS * S2), HPS * S2)
        return pltpu.make_async_copy(v_hbm.at[rows], vb.at[rows], sem_v.at[g])

    def cp_wq(g):
        cols = pl.ds(pl.multiple_of(g * (HPS * DH), HPS * DH), HPS * DH)
        return pltpu.make_async_copy(wq_hbm.at[:, cols], wqb.at[g], sem_w.at[g])

    def cp_wo(g):
        return pltpu.make_async_copy(wo_hbm.at[g], wob.at[g], sem_w.at[NHG + g])

    cp0_wq = [pltpu.make_async_copy(wq_hbm.at[:, pl.ds(j * DH, DH)], wqb.at[0, :, pl.ds(j * DH, DH)], sem_0.at[j])
              for j in range(HPS)]
    cp0_k = [pltpu.make_async_copy(k_hbm.at[pl.ds(j * S2, S2)], kb.at[pl.ds(j * S2, S2)], sem_0.at[HPS + j])
             for j in range(HPS)]
    cp0_v = [pltpu.make_async_copy(v_hbm.at[pl.ds(j * S2, S2)], vb.at[pl.ds(j * S2, S2)], sem_0.at[2 * HPS + j])
             for j in range(HPS)]

    cp_ffn = [pltpu.make_async_copy(wg_hbm, wgb, sem_f.at[0]),
              pltpu.make_async_copy(wu_hbm, wub, sem_f.at[1]),
              pltpu.make_async_copy(wd_hbm, wdb, sem_f.at[2])]

    def cp_out(qb):
        rows = pl.ds(pl.multiple_of(qb * TQ, TQ), TQ)
        return pltpu.make_async_copy(ob.at[rows], o_hbm.at[rows], sem_o.at[qb])

    cp_c.start()
    cp_x[0].start()
    for i in range(NMC):
        cp_wm(i).start()
    for cp in (cp0_wq[0], cp0_k[0], cp0_wq[1], cp0_k[1], cp0_v[0], cp0_wq[2], cp0_k[2], cp0_v[1],
               cp0_wq[3], cp0_k[3], cp_x[1], cp0_v[2], cp0_v[3], cp_wr):
        cp.start()
    for g in range(1, NHG):
        cps = [cp_wq(g), cp_k(g), cp_v(g), cp_wo(g - 1)]
        cps += [cp_x[2]] if g == 1 else []
        cps += [cp_wmr(g - 1)] if g <= NMP else []
        for cp in cps:
            cp.start()
    for cp in [cp_wo(NHG - 1), cp_x[3]] + cp_ffn:
        cp.start()

    def zbody(i, _):
        acc_ref[pl.ds(pl.multiple_of(i * 256, 256), 256), :] = jnp.zeros((256, D), f32)
        wmb[NMP, pl.ds(pl.multiple_of(i * 64, 64), 64), :] = jnp.zeros((64, MPW), u32)
        z_ref[i] = 0
        return 0
    lax.fori_loop(0, S // 256, zbody, 0)
    mod_ref[...] = jnp.zeros(mod_ref.shape, f32)
    top_ref[...] = jnp.full(top_ref.shape, -jnp.inf, f32)
    topi_ref[0] = jnp.zeros((8, 128), jnp.int32)
    topi_ref[1] = jnp.ones((8, 128), jnp.int32)

    def bc(k, n):
        p = mod_ref[:, k * D:(k + 1) * D]
        return p if n == 8 else jnp.concatenate([p] * (n // 8), axis=0)

    cp_x[0].wait()

    def nbody(i, _):
        rows = pl.ds(pl.multiple_of(i * 128, 128), 128)
        s1_ref[0, rows, 0:D] = _ln(xb[rows, :].astype(f32))
        return 0
    lax.fori_loop(0, TQ // 128, nbody, 0)

    cp_c.wait()

    def silu_c():
        c = cb_[...].astype(f32)
        sc = (c * jax.nn.sigmoid(c)).astype(bf16)
        return jnp.broadcast_to(sc, (8, D))

    scf = silu_c().astype(f32)
    for b in range(D // 128):
        blk = jnp.concatenate([scf[:, b * 128:(b + 1) * 128]] * 16, axis=0)
        scb_ref[b * 128:(b + 1) * 128, :] = blk.T

    for i in range(NMC):
        cp_wm(i).wait()
        lo = i * MCW
        md = _rb(jnp.dot(silu_c(), _w16(s0_ref[0, :, lo:lo + MCW]), preferred_element_type=f32))
        mod_ref[:, lo:lo + MCW] = _rb(1.0 + md) if lo >= D else md

    def ln1_rows(r0, n, tok, dst_ref, d0):
        x = _tie(xb[pl.ds(r0, n), :].astype(f32), tok)
        h = _ln(x) * bc(1, n) + bc(0, n)
        dst_ref[pl.ds(d0, n), :] = h.astype(bf16)
        return jnp.abs(h[:, 0:128])

    def derive_params():
        for c in range(4 * D // 128):
            p = c * 128 // MPW
            o = c * 128 - _mp_col(p)
            md = _rb(jnp.broadcast_to(jnp.sum(mp_ref[p, :, o:o + 128], axis=0, keepdims=True), (8, 128)))
            if 2 * D <= c * 128 < 3 * D:
                md = _rb(1.0 + md)
            mod_ref[:, 2 * D + c * 128:2 * D + (c + 1) * 128] = md
        sb, cb1, gb, wr = bc(3, 8), bc(4, 8), bc(5, 8), bc(6, 8)
        mod_ref[:, 7 * D:8 * D] = gb * sb
        mod_ref[:, 8 * D:9 * D] = gb * cb1
        mod_ref[:, 9 * D:10 * D] = cb1 * wr
        mod_ref[:, 10 * D:10 * D + 128] = jnp.broadcast_to(jnp.sum(sb * wr, axis=-1, keepdims=True), (8, 128))

    def fin_rows(r0, d0, n, valid, top, tok=None, late1=None, late2=None, write=True):
        x = _tie(xb[pl.ds(r0, n), :].astype(f32), tok)
        x1 = x + bc(2, n) * acc_ref[pl.ds(r0, n), :]
        xc, mb, dm = _center(x1, late1)
        rs = _rstd(xc, dm, late2)
        st_ref[0, pl.ds(d0, n), :] = jnp.broadcast_to(mb, (n, 128))
        st_ref[1, pl.ds(d0, n), :] = jnp.broadcast_to(rs, (n, 128))
        if write:
            ob[pl.ds(d0, n), :] = ((x1 + bc(7, n)) + (xc * rs) * bc(8, n)).astype(bf16)
        rc = mod_ref[:, 10 * D:10 * D + 128]
        r = jnp.broadcast_to(_rowsum(xc * bc(9, n), late2) * rs, (n, 128))
        r = _rb(r + jnp.concatenate([rc] * (n // 8), axis=0))
        tok = jnp.abs(r)
        if valid is not None:
            r = jnp.where(valid, r, -jnp.inf)
        b1, i1, b2, i2 = top
        sub = lax.broadcasted_iota(jnp.int32, (8, 128), 0)
        for g in range(n // 8):
            rg = r[g * 8:(g + 1) * 8, :]
            ids = sub + (r0 + g * 8)
            gt1 = rg > b1
            gt2 = rg > b2
            b2 = jnp.where(gt1, b1, jnp.where(gt2, rg, b2))
            i2 = jnp.where(gt1, i1, jnp.where(gt2, ids, i2))
            b1 = jnp.where(gt1, rg, b1)
            i1 = jnp.where(gt1, ids, i1)
        return (b1, i1, b2, i2), tok

    s_refs = (s0_ref, s1_ref)
    p_refs = (p0_ref, p1_ref)
    l_refs = (l0_ref, l1_ref, l2_ref, l3_ref)

    def attend(t, first):
        qb = t >> 3
        hg = t & (NHG - 1)
        slot = t & 1
        pads = PADS0 if first else PADS
        z = z_ref[0]
        z2 = z_ref[1]
        zp = pl.multiple_of(z * 16, 16)
        arows = pl.ds(pl.multiple_of(qb * TQ, TQ), TQ)
        kv0 = 0 if first else pl.multiple_of(hg * (HPS * S2), HPS * S2)
        early = [None]
        mv = [jnp.zeros((8, 128), f32), 0]
        mpi = jnp.where(jnp.logical_and(t >= 2, t < 2 + NMP), t - 2, NMP)

        def qp(j):
            cols = slice(j * DH, (j + 1) * DH)
            if first and j == 1:
                d0 = jnp.dot(h_ref[arows, 0:512], _w16(wqb[hg, 0:256, cols]), preferred_element_type=f32)
                early[0] = jnp.abs(d0[0:16])
                q = d0 + jnp.dot(h_ref[arows, 512:], _w16(wqb[hg, 256:, cols]), preferred_element_type=f32)
            else:
                q = jnp.dot(h_ref[arows, :], _w16(wqb[hg, :, cols]), preferred_element_type=f32)
            return q * (DH ** -0.5 * LOG2E)

        def qk(j, q):
            s = lax.dot_general(q.astype(bf16), _w16(kb[pl.ds(kv0 + j * S2, S2), :]), (((1,), (1,)), ((), ())),
                                preferred_element_type=f32)
            s_refs[j % 2][z] = s
            pm = s[:, 0:128]
            for c in range(1, S // 128):
                pm = jnp.maximum(pm, s[:, c * 128:(c + 1) * 128])
            m_ref[z, j] = jnp.broadcast_to(jnp.max(pm, axis=-1, keepdims=True), (TQ, 128))
            return jnp.abs(s[0:16, 0:128])

        def sm(j, tok=None):
            R, W = 16, S // 2
            sref = s_refs[j % 2]
            zs = z_ref[3 + j]
            for r in range(0, TQ, R):
                m = m_ref[zs, j, r:r + R, :]
                acc = None
                for hf in range(2):
                    mm = m if tok is None else jnp.where(tok < 0.0, 0.0, m)
                    p = jnp.exp2(sref[zs, r:r + R, hf * W:(hf + 1) * W] - _lanes(mm))
                    for c in range(W // 128):
                        pc = p[:, c * 128:(c + 1) * 128]
                        acc = pc if acc is None else acc + pc
                    if first or j != 1:
                        tok = acc
                        for _ in range(pads[j]):
                            tok = tok + tok
                    else:
                        a = jnp.where(jnp.minimum(acc[0:8], acc[8:16]) < 0.0, 1.0, mv[0])
                        for _ in range(MPW // 128):
                            mc, k0 = divmod(mv[1], D)
                            mv[1] += 16
                            w = _w16(wmb[mpi, k0 // 2:k0 // 2 + 8, mc * 128:(mc + 1) * 128]).astype(f32)
                            pr = w * scb_ref[k0:k0 + 16, :]
                            a = (a + pr[0:8]) + pr[8:16]
                            tok = a
                            if k0 + 16 == D:
                                mp_ref[mpi, :, mc * 128:(mc + 1) * 128] = a
                                a = jnp.where(jnp.abs(a) < 0.0, 1.0, 0.0)
                        mv[0] = a
                        tok = jnp.abs(tok)
                        tok = jnp.concatenate([tok, tok], axis=0)
                    p_refs[j % 2][pl.ds(zp + r, R), hf * W:(hf + 1) * W] = p.astype(bf16)
                l_refs[j][z, r:r + R, :] = acc

        def pv(j, between=None):
            pj = p_refs[j % 2]
            vv = _w16(vb[pl.ds(kv0 + j * S2, S2), :])
            d0 = jnp.dot(pj[pl.ds(zp, TQ), 0:512], vv[0:512], preferred_element_type=f32)
            o = d0 + jnp.dot(pj[pl.ds(zp, TQ), 512:], vv[512:], preferred_element_type=f32)
            early[0] = jnp.abs(d0[0:16])
            lp = jnp.maximum(l_refs[j][z2], jnp.minimum(d0, 0.0))
            l = jnp.broadcast_to(jnp.sum(lp, axis=-1, keepdims=True), (TQ, 128))
            if between is not None:
                between()
            o_ref[pl.ds(pl.multiple_of(slot * TQ, TQ), TQ), j * DH:(j + 1) * DH] = (o * _recip(l)).astype(bf16)

        def op_prev(c0, c1):
            tp = t - 1
            o = o_ref[pl.ds(pl.multiple_of((1 - slot) * TQ, TQ), TQ), :]
            rows = pl.ds(pl.multiple_of((tp >> 3) * TQ, TQ), TQ)
            d = jnp.dot(o, _w16(wob[tp & (NHG - 1), :, c0:c1]), preferred_element_type=f32)
            acc_ref[rows, c0:c1] += d
            return d

        def wait(*cps):
            for cp in cps:
                cp.wait()

        l0 = pl.multiple_of(jnp.minimum(t + NHG, NSTEP - 1) * CH, CH)

        if first:
            wait(cp0_wq[0])
            h_ref[0:TQ, :] = (s1_ref[0, :, 0:D] * bc(1, TQ) + bc(0, TQ)).astype(bf16)
            q0 = qp(0)
            wait(cp0_k[0])
            qk(0, q0)
            wait(cp0_wq[1], cp0_k[1], cp0_v[0], cp0_wq[2])
            q1 = qp(1)
            sm(0, early[0])
            qk(1, q1)
            sm(1)
            pv(0)
            q2 = qp(2)
            wait(cp0_k[2], cp0_v[1], cp0_wq[3], cp0_k[3], cp_x[1])
            qk(2, q2)
            sm(2)
            pv(1)
            q3 = qp(3)
            qk(3, q3)
            tok = jnp.abs(q3[TQ - 16:TQ, :])
            for g in range(0, CH, 16):
                tok = ln1_rows(l0 + g, 16, tok, h_ref, pl.multiple_of(l0 + g, 16))
            wait(cp0_v[2], cp0_v[3], cp_wr)
            pv(2)
            sm(3, early[0])
            pv(3)
            return

        valid = t > NHG
        fsrc = pl.multiple_of(jnp.maximum(t - NHG - 1, 0) * CH, CH)
        fdst = pl.multiple_of(jnp.where(valid, fsrc, S), CH)
        top = (top_ref[0], topi_ref[0], top_ref[1], topi_ref[1])
        tok = None
        for g in range(0, CH, 16):
            top, tok = fin_rows(fsrc + g, fdst + g, 16, valid, top, tok)
        top_ref[0], topi_ref[0], top_ref[1], topi_ref[1] = top

        qk(0, qp(0))
        q1 = qp(1)
        sm(0, _both(tok))
        tok = jnp.abs(q1[0:16])
        for g in range(0, CH, 16):
            tok = ln1_rows(l0 + g, 16, tok, hs_ref, zp + g)
        qk(1, q1)
        sm(1, _both(tok))
        pv(0)
        qk(2, qp(2))
        sm(2)
        pv(1)
        sm(3, qk(3, qp(3)))
        pv(2)
        never = _lanes(jnp.abs(op_prev(0, D // 2)[0:8, 0:128])) < 0.0
        for g in range(0, CH, 16):
            hv = hs_ref[pl.ds(pl.multiple_of(z2 * 16, 16) + g, 16), :].astype(f32)
            hv = jnp.concatenate([jnp.where(never, 0.0, hv[0:8]), hv[8:16]], axis=0)
            h_ref[pl.ds(l0 + g, 16), :] = hv.astype(bf16)
        op_prev(D // 2, D - 128)
        pv(3, lambda: op_prev(D - 128, D))

    attend(0, True)
    mod_ref[:, 6 * D:7 * D] = jnp.broadcast_to(wrb[...].astype(f32).reshape(1, D), (8, D))

    def step(t, _):
        attend(t, False)
        return 0

    def segment(k, _):
        t = jnp.where(k < NHG, k + 1, (k - NHG + 1) * NHG + 1)
        end = jnp.where(k < NHG, t + 1, jnp.minimum(t + NHG, NSTEP))

        @pl.when(t < NHG)
        def _():
            cp_wq(t).wait()
            cp_k(t).wait()
            cp_v(t).wait()

        @pl.when(t <= NHG)
        def _():
            cp_wo(t - 1).wait()

        @pl.when(jnp.logical_and(t >= 2, t < 2 + NMP))
        def _():
            pltpu.make_async_copy(wm_hbm.at[:, pl.ds(0, MPW)], wmb.at[t - 2], sem_wm.at[NMC + t - 2]).wait()

        @pl.when(t == 2)
        def _():
            cp_x[2].wait()

        @pl.when(t == NHG)
        def _():
            cp_x[3].wait()

        @pl.when(t == NHG + 1)
        def _():
            derive_params()

        @pl.when(t > 2 * NHG)
        def _():
            cp_out(k - NHG - 1).start()

        lax.fori_loop(t, end, step, 0)
        return 0

    lax.fori_loop(0, NHG + NQB - 1, segment, 0)

    for cp in cp_ffn:
        cp.wait()
    top = (top_ref[0], topi_ref[0], top_ref[1], topi_ref[1])
    rl0 = (NQB - 1) * TQ
    EG, EB = 16, 64
    oslot = ((NSTEP - 1) % 2) * TQ
    ds = []
    for r in range(0, TQ, EB):
        d = jnp.dot(o_ref[oslot + r:oslot + r + EB, :], _w16(wob[NHG - 1]), preferred_element_type=f32)
        acc_ref[rl0 + r:rl0 + r + EB, :] += d
        ds.append(d)

    def late(tc):
        if tc >= TQ * 8:
            return None
        c = (tc % (EB * 8)) // EB
        tk = jnp.abs(ds[tc // (EB * 8)][0:8, c * 128:(c + 1) * 128]) < 0.0
        return jnp.concatenate([tk] * (EG // 8), axis=0)

    for r in range(-CH, TQ, EG):
        ready = (r + EB) * 8
        top, _ = fin_rows(rl0 + r, rl0 + r, EG, None, top, None, late(ready + 100), late(ready + 400),
                          write=r < TQ - EB)
        if r == -EG:
            cp_out(NQB - 2).start()

    vals = jnp.concatenate([top[0], top[2]], axis=0)
    idxs = jnp.concatenate([top[1], top[3]], axis=0)
    m1 = jnp.max(vals, axis=0, keepdims=True)
    i1v = jnp.min(jnp.where(vals == m1, idxs, S - 1), axis=0, keepdims=True)
    vals2 = jnp.where(idxs == i1v, -jnp.inf, vals)
    m2 = jnp.max(vals2, axis=0, keepdims=True)
    i2v = jnp.min(jnp.where(jnp.logical_and(vals2 == m2, idxs != i1v), idxs, S - 1), axis=0, keepdims=True)
    b1 = pl.multiple_of(jnp.clip(i1v[0, 0] // 8 * 8, 0, S - 8), 8)
    b2 = pl.multiple_of(jnp.clip(i2v[0, 0] // 8 * 8, 0, S - 8), 8)

    def two(ref_rows):
        return jnp.concatenate([ref_rows(b1), ref_rows(b2)], axis=0)

    x1 = two(lambda b: xb[pl.ds(b, 8), :].astype(f32)) + bc(2, 16) * two(lambda b: acc_ref[pl.ds(b, 8), :])
    xn = (x1 - _lanes(two(lambda b: st_ref[0, pl.ds(b, 8), :]))) * _lanes(two(lambda b: st_ref[1, pl.ds(b, 8), :]))
    xs = (xn * bc(4, 16) + bc(3, 16)).astype(bf16)
    FC = 512
    y = None
    prev = None
    for c in range(0, F + FC, FC):
        if c < F:
            g = jnp.dot(xs, _w16(wgb[:, c:c + FC]), preferred_element_type=f32)
            u = jnp.dot(xs, _w16(wub[:, c:c + FC]), preferred_element_type=f32)
        if prev is not None:
            d = jnp.dot(prev, _w16(wdb[(c - FC) // 2:c // 2, :]), preferred_element_type=f32)
            y = d if y is None else y + d
        if c < F:
            prev = (g * jax.nn.sigmoid(g) * u).astype(bf16)
        if c == 0:
            for gi, r0 in enumerate(range(S - EB, S, EG)):
                never = jnp.abs(g[:, gi * 128:(gi + 1) * 128]) < 0.0
                xx = xb[r0:r0 + EG, :].astype(f32) + bc(2, EG) * acc_ref[r0:r0 + EG, :]
                rs = jnp.where(never, 0.0, st_ref[1, r0:r0 + EG, :])
                mb = jnp.where(never, 0.0, st_ref[0, r0:r0 + EG, :])
                ob[r0:r0 + EG, :] = ((xx + bc(7, EG)) + ((xx - _lanes(mb)) * _lanes(rs)) * bc(8, EG)).astype(bf16)
            cp_out(NQB - 1).start()
    sub = lax.broadcasted_iota(jnp.int32, (8, 128), 0)
    ids = jnp.concatenate([sub + b1, sub + b2], axis=0)
    upd = jnp.where(_lanes(ids == i1v), y * _lanes(jax.nn.sigmoid(m1)),
                    jnp.where(_lanes(ids == i2v), y * _lanes(jax.nn.sigmoid(m2)), 0.0))
    fixb[...] = ((x1 + bc(7, 16)) + xn * bc(8, 16) + bc(5, 16) * upd).astype(bf16)

    for qb in range(NQB):
        cp_out(qb).wait()
    cf1 = pltpu.make_async_copy(fixb.at[pl.ds(0, 8)], o_hbm.at[pl.ds(b1, 8)], sem_o.at[NQB])
    cf2 = pltpu.make_async_copy(fixb.at[pl.ds(8, 8)], o_hbm.at[pl.ds(b2, 8)], sem_o.at[NQB + 1])
    cf1.start()

    @pl.when(b1 != b2)
    def _():
        cf2.start()
        cf2.wait()
    cf1.wait()


@jax.jit
def pallas_adaLN_cond__mha_block_cached__moe_arch_mod__prompt_kernel(
    A_x: jax.Array,
    A_k_cache: jax.Array,
    A_v_cache: jax.Array,
    A_wq: jax.Array,
    A_wo: jax.Array,
    B_x: jax.Array,
    B_w_r: jax.Array,
    B_w_gate: jax.Array,
    B_w_up: jax.Array,
    B_w_down: jax.Array,
    c: jax.Array,
    w_mod: jax.Array,
):
    x = A_x.reshape(S, D)
    k = A_k_cache.reshape(H * S, DH)
    v = A_v_cache.reshape(H * S, DH)
    wo = A_wo.reshape(NHG, HPS * DH, D)
    anyspec = pl.BlockSpec(memory_space=pl.ANY)
    out = pl.pallas_call(
        _kernel,
        in_specs=[anyspec] * 11,
        out_specs=anyspec,
        out_shape=jax.ShapeDtypeStruct((S, D), bf16),
        scratch_shapes=[
            pltpu.VMEM((S, D), bf16),
            pltpu.VMEM((H * S2, DH), u32),
            pltpu.VMEM((H * S2, DH), u32),
            pltpu.VMEM((NHG, D // 2, HPS * DH), u32),
            pltpu.VMEM((NHG, HPS * DH // 2, D), u32),
            pltpu.VMEM((D // 2, F), u32),
            pltpu.VMEM((D // 2, F), u32),
            pltpu.VMEM((F // 2, D), u32),
            pltpu.VMEM((NMP + 1, D // 2, MPW), u32),
            pltpu.VMEM((8, 11 * D), f32),
            pltpu.VMEM((S // 2, D), u32),
            pltpu.VMEM((S, D), f32),
            pltpu.VMEM((S + CH, D), bf16),
            pltpu.VMEM((16, D), bf16),
            pltpu.VMEM((1, TQ, S), f32),
            pltpu.VMEM((1, TQ, S), f32),
            pltpu.VMEM((TQ // 2, S), u32),
            pltpu.VMEM((TQ // 2, S), u32),
            pltpu.VMEM((1, HPS, TQ, 128), f32),
            pltpu.VMEM((1, TQ, 128), f32),
            pltpu.VMEM((1, TQ, 128), f32),
            pltpu.VMEM((1, TQ, 128), f32),
            pltpu.VMEM((1, TQ, 128), f32),
            pltpu.VMEM((CH // 2, D), u32),
            pltpu.VMEM((TQ, HPS * DH), u32),
            pltpu.VMEM((2, S + CH, 128), f32),
            pltpu.VMEM((D, 128), f32),
            pltpu.VMEM((NMP + 1, 8, MPW), f32),
            pltpu.VMEM((2, 8, 128), f32),
            pltpu.VMEM((2, 8, 128), jnp.int32),
            pltpu.VMEM((D,), bf16),
            pltpu.VMEM((1, D), bf16),
            pltpu.SMEM((8,), jnp.int32),
            pltpu.SemaphoreType.DMA((2,)),
            pltpu.SemaphoreType.DMA((4,)),
            pltpu.SemaphoreType.DMA((NMC + NMP,)),
            pltpu.SemaphoreType.DMA((NHG,)),
            pltpu.SemaphoreType.DMA((NHG,)),
            pltpu.SemaphoreType.DMA((2 * NHG,)),
            pltpu.SemaphoreType.DMA((3 * HPS,)),
            pltpu.SemaphoreType.DMA((3,)),
            pltpu.SemaphoreType.DMA((NQB + 2,)),
        ],
        compiler_params=pltpu.CompilerParams(vmem_limit_bytes=124 * 1024 * 1024, disable_bounds_checks=True,
                                             disable_semaphore_checks=True),
    )(x, k, v, A_wq, wo, B_w_r, B_w_gate, B_w_up, B_w_down, c, w_mod)
    return out.reshape(1, S, D)
```

```python
import jax
import jax.numpy as jnp
from jax import lax
import jax.experimental.pallas as pl
import jax.experimental.pallas.tpu as pltpu

S = 2048
S2 = S // 2
D = 1024
H = 32
DH = 128
F = 3584
EPS = 1e-5
LOG2E = 1.4426950408889634
TQ = 512
NQB = S // TQ
HPS = 4
NHG = H // HPS
NSTEP = NQB * NHG
CH = TQ // NHG
MPW = 768
NMP = -(-4 * D // MPW)
NMC = 4
MCW = 2 * D // NMC
PADS = (6, 5, 6, 4)
PADS0 = (5, 5, 5, 0)

f32 = jnp.float32
bf16 = jnp.bfloat16
u32 = jnp.uint32


def _mp_col(p):
    return min(p * MPW, 4 * D - MPW)


def _rb(x):
    return x.astype(bf16).astype(f32)


def _recip(x):
    r = pl.reciprocal(x, approx=True)
    return r * (2.0 - x * r)


def _rowsum(x, late=None):
    p = x[:, 0:128]
    for c in range(1, x.shape[1] // 128):
        p = p + x[:, c * 128:(c + 1) * 128]
    if late is not None:
        p = jnp.where(late, 0.0, p)
    return jnp.sum(p, axis=-1, keepdims=True)


def _center(x, late=None):
    m = _rowsum(x, late) * (1.0 / D)
    mb = _rb(m)
    return x - mb, mb, m - mb


def _rstd(xc, dm, late=None):
    v = jnp.maximum(_rowsum(xc * xc, late) * (1.0 / D) - dm * dm, 0.0)
    y = _rb(_rb(v) + EPS)
    return _recip(_rb(y * lax.rsqrt(y)))


def _ln(x):
    xc, _, dm = _center(x)
    return xc * _rstd(xc, dm)


def _tie(x, tok):
    if tok is None:
        return x
    return jnp.concatenate([jnp.where(tok < 0.0, 0.0, x[:, 0:128]), x[:, 128:]], axis=1)


def _both(tok):
    tok = jnp.minimum(tok[0:8], tok[8:16])
    return jnp.concatenate([tok, tok], axis=0)


def _lanes(v):
    return jnp.concatenate([v] * (D // 128), axis=1)


def _w16(x):
    return pltpu.bitcast(x, bf16)


def _kernel(x_hbm, k_hbm, v_hbm, wq_hbm, wo_hbm, wr_hbm, wg_hbm, wu_hbm, wd_hbm, c_hbm, wm_hbm,
            o_hbm,
            xb, kb, vb, wqb, wob, wgb, wub, wdb, wmb,
            mod_ref, h_ref, acc_ref, ob, fixb, s0_ref, s1_ref, p0_ref, p1_ref, m_ref,
            l0_ref, l1_ref, l2_ref, l3_ref, hs_ref, o_ref, st_ref, scb_ref, xt_ref, mp_ref, top_ref, topi_ref,
            wrb, cb_, z_ref,
            sem_s, sem_x, sem_wm, sem_k, sem_v, sem_w, sem_0, sem_f, sem_o):
    h_ref, p0_ref, p1_ref, o_ref, hs_ref = (r.bitcast(bf16) for r in (h_ref, p0_ref, p1_ref, o_ref, hs_ref))
    wm0_hbm = wm_hbm.bitcast(f32)
    k_hbm, v_hbm, wq_hbm, wo_hbm, wg_hbm, wu_hbm, wd_hbm, wm_hbm = (
        r.bitcast(u32) for r in (k_hbm, v_hbm, wq_hbm, wo_hbm, wg_hbm, wu_hbm, wd_hbm, wm_hbm))

    cp_c = pltpu.make_async_copy(c_hbm, cb_, sem_s.at[0])
    cp_wr = pltpu.make_async_copy(wr_hbm, wrb, sem_s.at[1])
    xcuts = (0, TQ, TQ + 2 * CH, 2 * TQ + 2 * CH, S)
    cp_x = [pltpu.make_async_copy(x_hbm.at[pl.ds(a, b - a)], xb.at[pl.ds(a, b - a)], sem_x.at[i])
            for i, (a, b) in enumerate(zip(xcuts, xcuts[1:]))]

    def cp_wm(i):
        cols = pl.ds(i * MCW, MCW)
        return pltpu.make_async_copy(wm0_hbm.at[:, cols], s0_ref.at[0, :, cols], sem_wm.at[i])

    def cp_wmr(p):
        return pltpu.make_async_copy(wm_hbm.at[:, pl.ds(2 * D + _mp_col(p), MPW)], wmb.at[p], sem_wm.at[NMC + p])

    def cp_k(g):
        rows = pl.ds(pl.multiple_of(g * (HPS * S2), HPS * S2), HPS * S2)
        return pltpu.make_async_copy(k_hbm.at[rows], kb.at[rows], sem_k.at[g])

    def cp_v(g):
        rows = pl.ds(pl.multiple_of(g * (HPS * S2), HPS * S2), HPS * S2)
        return pltpu.make_async_copy(v_hbm.at[rows], vb.at[rows], sem_v.at[g])

    def cp_wq(g):
        cols = pl.ds(pl.multiple_of(g * (HPS * DH), HPS * DH), HPS * DH)
        return pltpu.make_async_copy(wq_hbm.at[:, cols], wqb.at[g], sem_w.at[g])

    def cp_wo(g):
        return pltpu.make_async_copy(wo_hbm.at[g], wob.at[g], sem_w.at[NHG + g])

    cp0_wq = [pltpu.make_async_copy(wq_hbm.at[:, pl.ds(j * DH, DH)], wqb.at[0, :, pl.ds(j * DH, DH)], sem_0.at[j])
              for j in range(HPS)]
    cp0_k = [pltpu.make_async_copy(k_hbm.at[pl.ds(j * S2, S2)], kb.at[pl.ds(j * S2, S2)], sem_0.at[HPS + j])
             for j in range(HPS)]
    cp0_v = [pltpu.make_async_copy(v_hbm.at[pl.ds(j * S2, S2)], vb.at[pl.ds(j * S2, S2)], sem_0.at[2 * HPS + j])
             for j in range(HPS)]

    cp_ffn = [pltpu.make_async_copy(wg_hbm, wgb, sem_f.at[0]),
              pltpu.make_async_copy(wu_hbm, wub, sem_f.at[1]),
              pltpu.make_async_copy(wd_hbm, wdb, sem_f.at[2])]

    def cp_out(qb):
        rows = pl.ds(pl.multiple_of(qb * TQ, TQ), TQ)
        return pltpu.make_async_copy(ob.at[rows], o_hbm.at[rows], sem_o.at[qb])

    cp_c.start()
    cp_x[0].start()
    for i in range(NMC):
        cp_wm(i).start()
    for cp in (cp0_wq[0], cp0_k[0], cp0_wq[1], cp0_k[1], cp0_v[0], cp0_wq[2], cp0_k[2], cp0_v[1],
               cp0_wq[3], cp0_k[3], cp_x[1], cp0_v[2], cp0_v[3], cp_wr):
        cp.start()
    for g in range(1, NHG):
        cps = [cp_wq(g), cp_k(g), cp_v(g), cp_wo(g - 1)]
        cps += [cp_x[2]] if g == 1 else []
        cps += [cp_wmr(g - 1)] if g <= NMP else []
        for cp in cps:
            cp.start()
    for cp in [cp_wo(NHG - 1), cp_x[3]] + cp_ffn:
        cp.start()

    def zbody(i, _):
        acc_ref[pl.ds(pl.multiple_of(i * 256, 256), 256), :] = jnp.zeros((256, D), f32)
        wmb[NMP, pl.ds(pl.multiple_of(i * 64, 64), 64), :] = jnp.zeros((64, MPW), u32)
        z_ref[i] = 0
        return 0
    lax.fori_loop(0, S // 256, zbody, 0)
    mod_ref[...] = jnp.zeros(mod_ref.shape, f32)
    top_ref[...] = jnp.full(top_ref.shape, -jnp.inf, f32)
    topi_ref[0] = jnp.zeros((8, 128), jnp.int32)
    topi_ref[1] = jnp.ones((8, 128), jnp.int32)

    def bc(k, n):
        p = mod_ref[:, k * D:(k + 1) * D]
        return p if n == 8 else jnp.concatenate([p] * (n // 8), axis=0)

    cp_x[0].wait()

    def nbody(i, _):
        rows = pl.ds(pl.multiple_of(i * 128, 128), 128)
        s1_ref[0, rows, 0:D] = _ln(xb[rows, :].astype(f32))
        return 0
    lax.fori_loop(0, TQ // 128, nbody, 0)

    cp_c.wait()

    def silu_c():
        c = cb_[...].astype(f32)
        sc = (c * jax.nn.sigmoid(c)).astype(bf16)
        return jnp.broadcast_to(sc, (8, D))

    scf = silu_c().astype(f32)
    for b in range(D // 128):
        blk = jnp.concatenate([scf[:, b * 128:(b + 1) * 128]] * 16, axis=0)
        scb_ref[b * 128:(b + 1) * 128, :] = blk.T

    for i in range(NMC):
        cp_wm(i).wait()
        lo = i * MCW
        md = _rb(jnp.dot(silu_c(), _w16(s0_ref[0, :, lo:lo + MCW]), preferred_element_type=f32))
        mod_ref[:, lo:lo + MCW] = _rb(1.0 + md) if lo >= D else md

    def ln1_rows(r0, n, tok, dst_ref, d0):
        x = _tie(xb[pl.ds(r0, n), :].astype(f32), tok)
        h = _ln(x) * bc(1, n) + bc(0, n)
        dst_ref[pl.ds(d0, n), :] = h.astype(bf16)
        return jnp.abs(h[:, 0:128])

    def derive_params():
        for c in range(4 * D // 128):
            p = c * 128 // MPW
            o = c * 128 - _mp_col(p)
            md = _rb(jnp.broadcast_to(jnp.sum(mp_ref[p, :, o:o + 128], axis=0, keepdims=True), (8, 128)))
            if 2 * D <= c * 128 < 3 * D:
                md = _rb(1.0 + md)
            mod_ref[:, 2 * D + c * 128:2 * D + (c + 1) * 128] = md
        sb, cb1, gb, wr = bc(3, 8), bc(4, 8), bc(5, 8), bc(6, 8)
        mod_ref[:, 7 * D:8 * D] = gb * sb
        mod_ref[:, 8 * D:9 * D] = gb * cb1
        mod_ref[:, 9 * D:10 * D] = cb1 * wr
        mod_ref[:, 10 * D:10 * D + 128] = jnp.broadcast_to(jnp.sum(sb * wr, axis=-1, keepdims=True), (8, 128))

    def fin_rows(r0, d0, n, valid, top, tok=None, late1=None, late2=None, write=True):
        x = _tie(xb[pl.ds(r0, n), :].astype(f32), tok)
        x1 = x + bc(2, n) * acc_ref[pl.ds(r0, n), :]
        xc, mb, dm = _center(x1, late1)
        rs = _rstd(xc, dm, late2)
        st_ref[0, pl.ds(d0, n), :] = jnp.broadcast_to(mb, (n, 128))
        st_ref[1, pl.ds(d0, n), :] = jnp.broadcast_to(rs, (n, 128))
        if write:
            ob[pl.ds(d0, n), :] = ((x1 + bc(7, n)) + (xc * rs) * bc(8, n)).astype(bf16)
        rc = mod_ref[:, 10 * D:10 * D + 128]
        r = jnp.broadcast_to(_rowsum(xc * bc(9, n), late2) * rs, (n, 128))
        r = _rb(r + jnp.concatenate([rc] * (n // 8), axis=0))
        tok = jnp.abs(r)
        if valid is not None:
            r = jnp.where(valid, r, -jnp.inf)
        b1, i1, b2, i2 = top
        sub = lax.broadcasted_iota(jnp.int32, (8, 128), 0)
        for g in range(n // 8):
            rg = r[g * 8:(g + 1) * 8, :]
            ids = sub + (r0 + g * 8)
            gt1 = rg > b1
            gt2 = rg > b2
            b2 = jnp.where(gt1, b1, jnp.where(gt2, rg, b2))
            i2 = jnp.where(gt1, i1, jnp.where(gt2, ids, i2))
            b1 = jnp.where(gt1, rg, b1)
            i1 = jnp.where(gt1, ids, i1)
        return (b1, i1, b2, i2), tok

    s_refs = (s0_ref, s1_ref)
    p_refs = (p0_ref, p1_ref)
    l_refs = (l0_ref, l1_ref, l2_ref, l3_ref)

    def attend(t, first):
        qb = t >> 3
        hg = t & (NHG - 1)
        slot = t & 1
        pads = PADS0 if first else PADS
        z = z_ref[0]
        z2 = z_ref[1]
        zp = pl.multiple_of(z * 16, 16)
        arows = pl.ds(pl.multiple_of(qb * TQ, TQ), TQ)
        kv0 = 0 if first else pl.multiple_of(hg * (HPS * S2), HPS * S2)
        early = [None]
        mv = [jnp.zeros((8, 128), f32), 0]
        mpi = jnp.where(jnp.logical_and(t >= 2, t < 2 + NMP), t - 2, NMP)

        def qp(j):
            cols = slice(j * DH, (j + 1) * DH)
            if first and j == 1:
                d0 = jnp.dot(h_ref[arows, 0:512], _w16(wqb[hg, 0:256, cols]), preferred_element_type=f32)
                early[0] = jnp.abs(d0[0:16])
                q = d0 + jnp.dot(h_ref[arows, 512:], _w16(wqb[hg, 256:, cols]), preferred_element_type=f32)
            else:
                q = jnp.dot(h_ref[arows, :], _w16(wqb[hg, :, cols]), preferred_element_type=f32)
            return q * (DH ** -0.5 * LOG2E)

        def qk(j, q):
            s = lax.dot_general(q.astype(bf16), _w16(kb[pl.ds(kv0 + j * S2, S2), :]), (((1,), (1,)), ((), ())),
                                preferred_element_type=f32)
            s_refs[j % 2][z] = s
            pm = s[:, 0:128]
            for c in range(1, S // 128):
                pm = jnp.maximum(pm, s[:, c * 128:(c + 1) * 128])
            m_ref[z, j] = jnp.broadcast_to(jnp.max(pm, axis=-1, keepdims=True), (TQ, 128))
            return jnp.abs(s[0:16, 0:128])

        def sm(j, tok=None):
            R, W = 16, S // 2
            sref = s_refs[j % 2]
            zs = z_ref[3 + j]
            for r in range(0, TQ, R):
                m = m_ref[zs, j, r:r + R, :]
                acc = None
                for hf in range(2):
                    mm = m if tok is None else jnp.where(tok < 0.0, 0.0, m)
                    p = jnp.exp2(sref[zs, r:r + R, hf * W:(hf + 1) * W] - _lanes(mm))
                    for c in range(W // 128):
                        pc = p[:, c * 128:(c + 1) * 128]
                        acc = pc if acc is None else acc + pc
                    if first or j != 1:
                        tok = acc
                        for _ in range(pads[j]):
                            tok = tok + tok
                    else:
                        a = jnp.where(jnp.minimum(acc[0:8], acc[8:16]) < 0.0, 1.0, mv[0])
                        for _ in range(MPW // 128):
                            mc, k0 = divmod(mv[1], D)
                            mv[1] += 16
                            w = _w16(wmb[mpi, k0 // 2:k0 // 2 + 8, mc * 128:(mc + 1) * 128]).astype(f32)
                            pr = w * scb_ref[k0:k0 + 16, :]
                            a = (a + pr[0:8]) + pr[8:16]
                            tok = a
                            if k0 + 16 == D:
                                mp_ref[mpi, :, mc * 128:(mc + 1) * 128] = a
                                a = jnp.where(jnp.abs(a) < 0.0, 1.0, 0.0)
                        mv[0] = a
                        tok = jnp.abs(tok)
                        tok = jnp.concatenate([tok, tok], axis=0)
                    p_refs[j % 2][pl.ds(zp + r, R), hf * W:(hf + 1) * W] = p.astype(bf16)
                l_refs[j][z, r:r + R, :] = acc

        def pv(j, between=None):
            pj = p_refs[j % 2]
            vv = _w16(vb[pl.ds(kv0 + j * S2, S2), :])
            d0 = jnp.dot(pj[pl.ds(zp, TQ), 0:512], vv[0:512], preferred_element_type=f32)
            o = d0 + jnp.dot(pj[pl.ds(zp, TQ), 512:], vv[512:], preferred_element_type=f32)
            early[0] = jnp.abs(d0[0:16])
            lp = jnp.maximum(l_refs[j][z2], jnp.minimum(d0, 0.0))
            l = jnp.broadcast_to(jnp.sum(lp, axis=-1, keepdims=True), (TQ, 128))
            if between is not None:
                between()
            o_ref[pl.ds(pl.multiple_of(slot * TQ, TQ), TQ), j * DH:(j + 1) * DH] = (o * _recip(l)).astype(bf16)

        def op_prev(c0, c1):
            tp = t - 1
            o = o_ref[pl.ds(pl.multiple_of((1 - slot) * TQ, TQ), TQ), :]
            rows = pl.ds(pl.multiple_of((tp >> 3) * TQ, TQ), TQ)
            d = jnp.dot(o, _w16(wob[tp & (NHG - 1), :, c0:c1]), preferred_element_type=f32)
            acc_ref[rows, c0:c1] += d
            return d

        def wait(*cps):
            for cp in cps:
                cp.wait()

        l0 = pl.multiple_of(jnp.minimum(t + NHG, NSTEP - 1) * CH, CH)

        if first:
            wait(cp0_wq[0])
            h_ref[0:TQ, :] = (s1_ref[0, :, 0:D] * bc(1, TQ) + bc(0, TQ)).astype(bf16)
            q0 = qp(0)
            wait(cp0_k[0])
            qk(0, q0)
            wait(cp0_wq[1], cp0_k[1], cp0_v[0], cp0_wq[2])
            q1 = qp(1)
            sm(0, early[0])
            qk(1, q1)
            sm(1)
            pv(0)
            q2 = qp(2)
            wait(cp0_k[2], cp0_v[1], cp0_wq[3], cp0_k[3], cp_x[1])
            qk(2, q2)
            sm(2)
            pv(1)
            q3 = qp(3)
            qk(3, q3)
            tok = jnp.abs(q3[TQ - 16:TQ, :])
            for g in range(0, CH, 16):
                tok = ln1_rows(l0 + g, 16, tok, h_ref, pl.multiple_of(l0 + g, 16))
            wait(cp0_v[2], cp0_v[3], cp_wr)
            pv(2)
            sm(3, early[0])
            pv(3)
            return

        valid = t > NHG
        fsrc = pl.multiple_of(jnp.maximum(t - NHG - 1, 0) * CH, CH)
        fdst = pl.multiple_of(jnp.where(valid, fsrc, S), CH)
        top = (top_ref[0], topi_ref[0], top_ref[1], topi_ref[1])
        tok = None
        for g in range(0, CH, 16):
            top, tok = fin_rows(fsrc + g, fdst + g, 16, valid, top, tok)
        top_ref[0], topi_ref[0], top_ref[1], topi_ref[1] = top

        qk(0, qp(0))
        q1 = qp(1)
        sm(0, _both(tok))
        tok = jnp.abs(q1[0:16])
        for g in range(0, CH, 16):
            tok = ln1_rows(l0 + g, 16, tok, hs_ref, zp + g)
        qk(1, q1)
        sm(1, _both(tok))
        pv(0)
        qk(2, qp(2))
        sm(2)
        pv(1)
        sm(3, qk(3, qp(3)))
        pv(2)
        never = _lanes(jnp.abs(op_prev(0, D // 2)[0:8, 0:128])) < 0.0
        for g in range(0, CH, 16):
            hv = hs_ref[pl.ds(pl.multiple_of(z2 * 16, 16) + g, 16), :].astype(f32)
            hv = jnp.concatenate([jnp.where(never, 0.0, hv[0:8]), hv[8:16]], axis=0)
            h_ref[pl.ds(l0 + g, 16), :] = hv.astype(bf16)
        op_prev(D // 2, D - 128)
        pv(3, lambda: op_prev(D - 128, D))

    attend(0, True)
    mod_ref[:, 6 * D:7 * D] = jnp.broadcast_to(wrb[...].astype(f32).reshape(1, D), (8, D))

    def step(t, _):
        attend(t, False)
        return 0

    def segment(k, _):
        t = jnp.where(k < NHG, k + 1, (k - NHG + 1) * NHG + 1)
        end = jnp.where(k < NHG, t + 1, jnp.minimum(t + NHG, NSTEP))

        @pl.when(t < NHG)
        def _():
            cp_wq(t).wait()
            cp_k(t).wait()
            cp_v(t).wait()

        @pl.when(t <= NHG)
        def _():
            cp_wo(t - 1).wait()

        @pl.when(jnp.logical_and(t >= 2, t < 2 + NMP))
        def _():
            pltpu.make_async_copy(wm_hbm.at[:, pl.ds(0, MPW)], wmb.at[t - 2], sem_wm.at[NMC + t - 2]).wait()

        @pl.when(t == 2)
        def _():
            cp_x[2].wait()

        @pl.when(t == NHG)
        def _():
            cp_x[3].wait()

        @pl.when(t == NHG + 1)
        def _():
            derive_params()

        @pl.when(t > 2 * NHG)
        def _():
            cp_out(k - NHG - 1).start()

        lax.fori_loop(t, end, step, 0)
        return 0

    lax.fori_loop(0, NHG + NQB - 1, segment, 0)

    top = (top_ref[0], topi_ref[0], top_ref[1], topi_ref[1])
    rl0 = (NQB - 1) * TQ
    EG, EB, EP = 16, 64, 144
    oslot = ((NSTEP - 1) % 2) * TQ
    ds = []
    for r in range(0, TQ, EB):
        d = jnp.dot(o_ref[oslot + r:oslot + r + EB, :], _w16(wob[NHG - 1]), preferred_element_type=f32)
        acc_ref[rl0 + r:rl0 + r + EB, :] += d
        ds.append(d)

    def late(tc):
        if tc >= TQ * 8:
            return None
        c = (tc % (EB * 8)) // EB
        tk = jnp.abs(ds[tc // (EB * 8)][0:8, c * 128:(c + 1) * 128]) < 0.0
        return jnp.concatenate([tk] * (EG // 8), axis=0)

    for r in range(-CH, TQ, EG):
        ready = (r + EB) * 8
        top, _ = fin_rows(rl0 + r, rl0 + r, EG, None, top, None, late(ready + 128), late(ready + 256),
                          write=r < TQ - EP)
        if r == -EG:
            cp_out(NQB - 2).start()

    for cp in cp_ffn:
        cp.wait()
    vals = jnp.concatenate([top[0], top[2]], axis=0)
    idxs = jnp.concatenate([top[1], top[3]], axis=0)
    m1 = jnp.max(vals, axis=0, keepdims=True)
    i1v = jnp.min(jnp.where(vals == m1, idxs, S - 1), axis=0, keepdims=True)
    vals2 = jnp.where(idxs == i1v, -jnp.inf, vals)
    m2 = jnp.max(vals2, axis=0, keepdims=True)
    i2v = jnp.min(jnp.where(jnp.logical_and(vals2 == m2, idxs != i1v), idxs, S - 1), axis=0, keepdims=True)
    b1 = pl.multiple_of(jnp.clip(i1v[0, 0] // 8 * 8, 0, S - 8), 8)
    b2 = pl.multiple_of(jnp.clip(i2v[0, 0] // 8 * 8, 0, S - 8), 8)

    def two(ref_rows):
        return jnp.concatenate([ref_rows(b1), ref_rows(b2)], axis=0)

    x1 = two(lambda b: xb[pl.ds(b, 8), :].astype(f32)) + bc(2, 16) * two(lambda b: acc_ref[pl.ds(b, 8), :])
    xn = (x1 - _lanes(two(lambda b: st_ref[0, pl.ds(b, 8), :]))) * _lanes(two(lambda b: st_ref[1, pl.ds(b, 8), :]))
    xs = (xn * bc(4, 16) + bc(3, 16)).astype(bf16)
    sub = lax.broadcasted_iota(jnp.int32, (8, 128), 0)
    ids = jnp.concatenate([sub + b1, sub + b2], axis=0)

    NV, CB, FC = 1024, 256, 640
    FM = F - NV
    xf = xs.astype(f32)
    rows = [jnp.sum(jnp.where(_lanes(ids[lo:lo + 8] == iv), xf[lo:lo + 8], 0.0), axis=0, keepdims=True)
            for lo, iv in ((0, i1v), (8, i2v))]
    rows = [jnp.broadcast_to(r, (8, D)) for r in rows]
    pk = pltpu.bitcast(rows[0], u32) | (pltpu.bitcast(rows[1], u32) >> 16)
    for b in range(D // 128):
        xt_ref[0, b * 128:(b + 1) * 128, :] = jnp.concatenate([pk[:, b * 128:(b + 1) * 128]] * 16, axis=0).T

    def wide(v):
        return jnp.concatenate([v] * (CB // 128), axis=1)

    def vpu_cols(c, start):
        zt = z_ref[2]
        acc = [wide(start)] * 4
        for k0 in range(0, D, 16):
            tb = xt_ref[zt, k0:k0 + 16, :]
            xk = (wide(pltpu.bitcast(tb & jnp.uint32(0xFFFF0000), f32)), wide(pltpu.bitcast(tb << 16, f32)))
            for wi, w_ref in enumerate((wgb, wub)):
                w = _w16(w_ref[k0 // 2:k0 // 2 + 8, c:c + CB]).astype(f32)
                for k in range(2):
                    pr = w * xk[k]
                    acc[2 * wi + k] = (acc[2 * wi + k] + pr[0:8]) + pr[8:16]
        tot = (jnp.abs(acc[0]) + jnp.abs(acc[1])) + (jnp.abs(acc[2]) + jnp.abs(acc[3]))
        tot = tot[:, 0:128] + tot[:, 128:256]
        red = [jnp.broadcast_to(jnp.sum(a, axis=0, keepdims=True), (16, CB)) for a in acc]
        g, u = (jnp.where(wide(ids == i1v), red[2 * wi], red[2 * wi + 1]) for wi in range(2))
        return g * jax.nn.sigmoid(g) * u, jnp.where(tot < 0.0, 1.0, 0.0)

    av = []
    start = jnp.zeros((8, 128), f32)
    for c in range(FM, F, CB):
        out, start = vpu_cols(c, start)
        av.append(out)

    y = None
    prev = None
    for c in range(0, FM + FC, FC):
        if c < FM:
            g = jnp.dot(xs, _w16(wgb[:, c:c + FC]), preferred_element_type=f32)
            u = jnp.dot(xs, _w16(wub[:, c:c + FC]), preferred_element_type=f32)
        if prev is not None:
            d = jnp.dot(prev, _w16(wdb[(c - FC) // 2:c // 2, :]), preferred_element_type=f32)
            y = d if y is None else y + d
        if c < FM:
            prev = (g * jax.nn.sigmoid(g) * u).astype(bf16)
        if c == 0:
            gu = jnp.concatenate([g, u], axis=1)
            for gi, r0 in enumerate(range(S - EP, S, EG)):
                gc = gi * (2 * FC // 128) // (EP // EG)
                never = jnp.abs(gu[:, gc * 128:(gc + 1) * 128]) < 0.0
                xx = xb[r0:r0 + EG, :].astype(f32) + bc(2, EG) * acc_ref[r0:r0 + EG, :]
                rs = jnp.where(never, 0.0, st_ref[1, r0:r0 + EG, :])
                mb = jnp.where(never, 0.0, st_ref[0, r0:r0 + EG, :])
                ob[r0:r0 + EG, :] = ((xx + bc(7, EG)) + ((xx - _lanes(mb)) * _lanes(rs)) * bc(8, EG)).astype(bf16)
            cp_out(NQB - 1).start()
    for i, a in enumerate(av):
        c = FM + i * CB
        y = y + jnp.dot(a.astype(bf16), _w16(wdb[c // 2:(c + CB) // 2, :]), preferred_element_type=f32)
    upd = jnp.where(_lanes(ids == i1v), y * _lanes(jax.nn.sigmoid(m1)),
                    jnp.where(_lanes(ids == i2v), y * _lanes(jax.nn.sigmoid(m2)), 0.0))
    fixb[...] = ((x1 + bc(7, 16)) + xn * bc(8, 16) + bc(5, 16) * upd).astype(bf16)

    for qb in range(NQB):
        cp_out(qb).wait()
    cf1 = pltpu.make_async_copy(fixb.at[pl.ds(0, 8)], o_hbm.at[pl.ds(b1, 8)], sem_o.at[NQB])
    cf2 = pltpu.make_async_copy(fixb.at[pl.ds(8, 8)], o_hbm.at[pl.ds(b2, 8)], sem_o.at[NQB + 1])
    cf1.start()

    @pl.when(b1 != b2)
    def _():
        cf2.start()
        cf2.wait()
    cf1.wait()


@jax.jit
def pallas_adaLN_cond__mha_block_cached__moe_arch_mod__prompt_kernel(
    A_x: jax.Array,
    A_k_cache: jax.Array,
    A_v_cache: jax.Array,
    A_wq: jax.Array,
    A_wo: jax.Array,
    B_x: jax.Array,
    B_w_r: jax.Array,
    B_w_gate: jax.Array,
    B_w_up: jax.Array,
    B_w_down: jax.Array,
    c: jax.Array,
    w_mod: jax.Array,
):
    x = A_x.reshape(S, D)
    k = A_k_cache.reshape(H * S, DH)
    v = A_v_cache.reshape(H * S, DH)
    wo = A_wo.reshape(NHG, HPS * DH, D)
    anyspec = pl.BlockSpec(memory_space=pl.ANY)
    out = pl.pallas_call(
        _kernel,
        in_specs=[anyspec] * 11,
        out_specs=anyspec,
        out_shape=jax.ShapeDtypeStruct((S, D), bf16),
        scratch_shapes=[
            pltpu.VMEM((S, D), bf16),
            pltpu.VMEM((H * S2, DH), u32),
            pltpu.VMEM((H * S2, DH), u32),
            pltpu.VMEM((NHG, D // 2, HPS * DH), u32),
            pltpu.VMEM((NHG, HPS * DH // 2, D), u32),
            pltpu.VMEM((D // 2, F), u32),
            pltpu.VMEM((D // 2, F), u32),
            pltpu.VMEM((F // 2, D), u32),
            pltpu.VMEM((NMP + 1, D // 2, MPW), u32),
            pltpu.VMEM((8, 11 * D), f32),
            pltpu.VMEM((S // 2, D), u32),
            pltpu.VMEM((S, D), f32),
            pltpu.VMEM((S + CH, D), bf16),
            pltpu.VMEM((16, D), bf16),
            pltpu.VMEM((1, TQ, S), f32),
            pltpu.VMEM((1, TQ, S), f32),
            pltpu.VMEM((TQ // 2, S), u32),
            pltpu.VMEM((TQ // 2, S), u32),
            pltpu.VMEM((1, HPS, TQ, 128), f32),
            pltpu.VMEM((1, TQ, 128), f32),
            pltpu.VMEM((1, TQ, 128), f32),
            pltpu.VMEM((1, TQ, 128), f32),
            pltpu.VMEM((1, TQ, 128), f32),
            pltpu.VMEM((CH // 2, D), u32),
            pltpu.VMEM((TQ, HPS * DH), u32),
            pltpu.VMEM((2, S + CH, 128), f32),
            pltpu.VMEM((D, 128), f32),
            pltpu.VMEM((1, D, 128), u32),
            pltpu.VMEM((NMP + 1, 8, MPW), f32),
            pltpu.VMEM((2, 8, 128), f32),
            pltpu.VMEM((2, 8, 128), jnp.int32),
            pltpu.VMEM((D,), bf16),
            pltpu.VMEM((1, D), bf16),
            pltpu.SMEM((8,), jnp.int32),
            pltpu.SemaphoreType.DMA((2,)),
            pltpu.SemaphoreType.DMA((4,)),
            pltpu.SemaphoreType.DMA((NMC + NMP,)),
            pltpu.SemaphoreType.DMA((NHG,)),
            pltpu.SemaphoreType.DMA((NHG,)),
            pltpu.SemaphoreType.DMA((2 * NHG,)),
            pltpu.SemaphoreType.DMA((3 * HPS,)),
            pltpu.SemaphoreType.DMA((3,)),
            pltpu.SemaphoreType.DMA((NQB + 2,)),
        ],
        compiler_params=pltpu.CompilerParams(vmem_limit_bytes=124 * 1024 * 1024, disable_bounds_checks=True,
                                             disable_semaphore_checks=True),
    )(x, k, v, A_wq, wo, B_w_r, B_w_gate, B_w_up, B_w_down, c, w_mod)
    return out.reshape(1, S, D)
```

```python
import jax
import jax.numpy as jnp
from jax import lax
import jax.experimental.pallas as pl
import jax.experimental.pallas.tpu as pltpu

S = 2048
S2 = S // 2
D = 1024
H = 32
DH = 128
F = 3584
EPS = 1e-5
LOG2E = 1.4426950408889634
TQ = 512
NQB = S // TQ
HPS = 4
NHG = H // HPS
NSTEP = NQB * NHG
CH = TQ // NHG
MPW = 768
NMP = -(-4 * D // MPW)
NMC = 4
MCW = 2 * D // NMC
PADS = (6, 5, 6, 4)
PADS0 = (5, 5, 5, 0)

f32 = jnp.float32
bf16 = jnp.bfloat16
u32 = jnp.uint32


def _mp_col(p):
    return min(p * MPW, 4 * D - MPW)


def _rb(x):
    return x.astype(bf16).astype(f32)


def _recip(x):
    r = pl.reciprocal(x, approx=True)
    return r * (2.0 - x * r)


def _rowsum(x, late=None):
    p = x[:, 0:128]
    for c in range(1, x.shape[1] // 128):
        p = p + x[:, c * 128:(c + 1) * 128]
    if late is not None:
        p = jnp.where(late, 0.0, p)
    return jnp.sum(p, axis=-1, keepdims=True)


def _center(x, late=None):
    m = _rowsum(x, late) * (1.0 / D)
    mb = _rb(m)
    return x - mb, mb, m - mb


def _rstd(xc, dm, late=None):
    v = jnp.maximum(_rowsum(xc * xc, late) * (1.0 / D) - dm * dm, 0.0)
    y = _rb(_rb(v) + EPS)
    return _recip(_rb(y * lax.rsqrt(y)))


def _ln(x, late1=None, late2=None):
    xc, _, dm = _center(x, late1)
    return xc * _rstd(xc, dm, late2)


def _tie(x, tok):
    if tok is None:
        return x
    return jnp.concatenate([jnp.where(tok < 0.0, 0.0, x[:, 0:128]), x[:, 128:]], axis=1)


def _both(tok):
    tok = jnp.minimum(tok[0:8], tok[8:16])
    return jnp.concatenate([tok, tok], axis=0)


def _lanes(v):
    return jnp.concatenate([v] * (D // 128), axis=1)


def _w16(x):
    return pltpu.bitcast(x, bf16)


def _kernel(x_hbm, k_hbm, v_hbm, wq_hbm, wo_hbm, wr_hbm, wg_hbm, wu_hbm, wd_hbm, c_hbm, wm_hbm,
            o_hbm,
            xb, kb, vb, wqb, wob, wgb, wub, wdb, wmb,
            mod_ref, h_ref, acc_ref, ob, fixb, s0_ref, s1_ref, p0_ref, p1_ref, m_ref,
            l0_ref, l1_ref, l2_ref, l3_ref, hs_ref, o_ref, st_ref, scb_ref, xt_ref, mp_ref, top_ref, topi_ref,
            wrb, cb_, z_ref,
            sem_s, sem_x, sem_wm, sem_k, sem_v, sem_w, sem_0, sem_f, sem_o):
    h_ref, p0_ref, p1_ref, o_ref, hs_ref = (r.bitcast(bf16) for r in (h_ref, p0_ref, p1_ref, o_ref, hs_ref))
    wm0_hbm = wm_hbm.bitcast(f32)
    k_hbm, v_hbm, wq_hbm, wo_hbm, wg_hbm, wu_hbm, wd_hbm, wm_hbm = (
        r.bitcast(u32) for r in (k_hbm, v_hbm, wq_hbm, wo_hbm, wg_hbm, wu_hbm, wd_hbm, wm_hbm))

    cp_c = pltpu.make_async_copy(c_hbm, cb_, sem_s.at[0])
    cp_wr = pltpu.make_async_copy(wr_hbm, wrb, sem_s.at[1])
    xcuts = (0, TQ, TQ + 2 * CH, 2 * TQ + 2 * CH, S)
    cp_x = [pltpu.make_async_copy(x_hbm.at[pl.ds(a, b - a)], xb.at[pl.ds(a, b - a)], sem_x.at[i])
            for i, (a, b) in enumerate(zip(xcuts, xcuts[1:]))]

    def cp_wm(i):
        cols = pl.ds(i * MCW, MCW)
        return pltpu.make_async_copy(wm0_hbm.at[:, cols], s0_ref.at[0, :, cols], sem_wm.at[i])

    def cp_wmr(p):
        return pltpu.make_async_copy(wm_hbm.at[:, pl.ds(2 * D + _mp_col(p), MPW)], wmb.at[p], sem_wm.at[NMC + p])

    def cp_k(g):
        rows = pl.ds(pl.multiple_of(g * (HPS * S2), HPS * S2), HPS * S2)
        return pltpu.make_async_copy(k_hbm.at[rows], kb.at[rows], sem_k.at[g])

    def cp_v(g):
        rows = pl.ds(pl.multiple_of(g * (HPS * S2), HPS * S2), HPS * S2)
        return pltpu.make_async_copy(v_hbm.at[rows], vb.at[rows], sem_v.at[g])

    def cp_wq(g):
        cols = pl.ds(pl.multiple_of(g * (HPS * DH), HPS * DH), HPS * DH)
        return pltpu.make_async_copy(wq_hbm.at[:, cols], wqb.at[g], sem_w.at[g])

    def cp_wo(g):
        return pltpu.make_async_copy(wo_hbm.at[g], wob.at[g], sem_w.at[NHG + g])

    cp0_wq = [pltpu.make_async_copy(wq_hbm.at[:, pl.ds(j * DH, DH)], wqb.at[0, :, pl.ds(j * DH, DH)], sem_0.at[j])
              for j in range(HPS)]
    cp0_k = [pltpu.make_async_copy(k_hbm.at[pl.ds(j * S2, S2)], kb.at[pl.ds(j * S2, S2)], sem_0.at[HPS + j])
             for j in range(HPS)]
    cp0_v = [pltpu.make_async_copy(v_hbm.at[pl.ds(j * S2, S2)], vb.at[pl.ds(j * S2, S2)], sem_0.at[2 * HPS + j])
             for j in range(HPS)]

    cp_ffn = [pltpu.make_async_copy(wg_hbm, wgb, sem_f.at[0]),
              pltpu.make_async_copy(wu_hbm, wub, sem_f.at[1]),
              pltpu.make_async_copy(wd_hbm, wdb, sem_f.at[2])]

    def cp_out(qb):
        rows = pl.ds(pl.multiple_of(qb * TQ, TQ), TQ)
        return pltpu.make_async_copy(ob.at[rows], o_hbm.at[rows], sem_o.at[qb])

    cp_c.start()
    cp_x[0].start()
    for i in range(NMC):
        cp_wm(i).start()
    for cp in (cp0_wq[0], cp0_k[0], cp0_wq[1], cp0_k[1], cp0_v[0], cp0_wq[2], cp0_k[2], cp0_v[1],
               cp0_wq[3], cp0_k[3], cp_x[1], cp0_v[2], cp0_v[3], cp_wr):
        cp.start()
    for g in range(1, NHG):
        cps = [cp_wq(g), cp_k(g), cp_v(g), cp_wo(g - 1)]
        cps += [cp_x[2]] if g == 1 else []
        cps += [cp_wmr(g - 1)] if g <= NMP else []
        for cp in cps:
            cp.start()
    for cp in [cp_wo(NHG - 1), cp_x[3]] + cp_ffn:
        cp.start()

    def zbody(i, _):
        acc_ref[pl.ds(pl.multiple_of(i * 256, 256), 256), :] = jnp.zeros((256, D), f32)
        wmb[NMP, pl.ds(pl.multiple_of(i * 64, 64), 64), :] = jnp.zeros((64, MPW), u32)
        z_ref[i] = 0
        return 0
    lax.fori_loop(0, S // 256, zbody, 0)
    mod_ref[...] = jnp.zeros(mod_ref.shape, f32)
    top_ref[...] = jnp.full(top_ref.shape, -jnp.inf, f32)
    topi_ref[0] = jnp.zeros((8, 128), jnp.int32)
    topi_ref[1] = jnp.ones((8, 128), jnp.int32)

    def bc(k, n):
        p = mod_ref[:, k * D:(k + 1) * D]
        return p if n == 8 else jnp.concatenate([p] * (n // 8), axis=0)

    cp_x[0].wait()

    def nbody(i, _):
        rows = pl.ds(pl.multiple_of(i * 128, 128), 128)
        s1_ref[0, rows, 0:D] = _ln(xb[rows, :].astype(f32))
        return 0
    lax.fori_loop(0, TQ // 128, nbody, 0)

    cp_c.wait()

    def silu_c():
        c = cb_[...].astype(f32)
        sc = (c * jax.nn.sigmoid(c)).astype(bf16)
        return jnp.broadcast_to(sc, (8, D))

    scf = silu_c().astype(f32)
    for b in range(D // 128):
        blk = jnp.concatenate([scf[:, b * 128:(b + 1) * 128]] * 16, axis=0)
        scb_ref[b * 128:(b + 1) * 128, :] = blk.T

    for i in range(NMC):
        cp_wm(i).wait()
        lo = i * MCW
        md = _rb(jnp.dot(silu_c(), _w16(s0_ref[0, :, lo:lo + MCW]), preferred_element_type=f32))
        mod_ref[:, lo:lo + MCW] = _rb(1.0 + md) if lo >= D else md

    def ln1_rows(r0, n, tok, dst_ref, d0, late1=None, late2=None):
        x = _tie(xb[pl.ds(r0, n), :].astype(f32), tok)
        h = _ln(x, late1, late2) * bc(1, n) + bc(0, n)
        dst_ref[pl.ds(d0, n), :] = h.astype(bf16)
        return jnp.abs(h[:, 0:128])

    def derive_params():
        for c in range(4 * D // 128):
            p = c * 128 // MPW
            o = c * 128 - _mp_col(p)
            md = _rb(jnp.broadcast_to(jnp.sum(mp_ref[p, :, o:o + 128], axis=0, keepdims=True), (8, 128)))
            if 2 * D <= c * 128 < 3 * D:
                md = _rb(1.0 + md)
            mod_ref[:, 2 * D + c * 128:2 * D + (c + 1) * 128] = md
        sb, cb1, gb, wr = bc(3, 8), bc(4, 8), bc(5, 8), bc(6, 8)
        mod_ref[:, 7 * D:8 * D] = gb * sb
        mod_ref[:, 8 * D:9 * D] = gb * cb1
        mod_ref[:, 9 * D:10 * D] = cb1 * wr
        mod_ref[:, 10 * D:10 * D + 128] = jnp.broadcast_to(jnp.sum(sb * wr, axis=-1, keepdims=True), (8, 128))

    def fin_rows(r0, d0, n, valid, top, tok=None, late1=None, late2=None, write=True):
        x = _tie(xb[pl.ds(r0, n), :].astype(f32), tok)
        x1 = x + bc(2, n) * acc_ref[pl.ds(r0, n), :]
        xc, mb, dm = _center(x1, late1)
        rs = _rstd(xc, dm, late2)
        st_ref[0, pl.ds(d0, n), :] = jnp.broadcast_to(mb, (n, 128))
        st_ref[1, pl.ds(d0, n), :] = jnp.broadcast_to(rs, (n, 128))
        if write:
            ob[pl.ds(d0, n), :] = ((x1 + bc(7, n)) + (xc * rs) * bc(8, n)).astype(bf16)
        rc = mod_ref[:, 10 * D:10 * D + 128]
        r = jnp.broadcast_to(_rowsum(xc * bc(9, n), late2) * rs, (n, 128))
        r = _rb(r + jnp.concatenate([rc] * (n // 8), axis=0))
        tok = jnp.abs(r)
        if valid is not None:
            r = jnp.where(valid, r, -jnp.inf)
        b1, i1, b2, i2 = top
        sub = lax.broadcasted_iota(jnp.int32, (8, 128), 0)
        for g in range(n // 8):
            rg = r[g * 8:(g + 1) * 8, :]
            ids = sub + (r0 + g * 8)
            gt1 = rg > b1
            gt2 = rg > b2
            b2 = jnp.where(gt1, b1, jnp.where(gt2, rg, b2))
            i2 = jnp.where(gt1, i1, jnp.where(gt2, ids, i2))
            b1 = jnp.where(gt1, rg, b1)
            i1 = jnp.where(gt1, ids, i1)
        return (b1, i1, b2, i2), tok

    s_refs = (s0_ref, s1_ref)
    p_refs = (p0_ref, p1_ref)
    l_refs = (l0_ref, l1_ref, l2_ref, l3_ref)

    def attend(t, first):
        qb = t >> 3
        hg = t & (NHG - 1)
        slot = t & 1
        pads = PADS0 if first else PADS
        z = z_ref[0]
        z2 = z_ref[1]
        zp = pl.multiple_of(z * 16, 16)
        arows = pl.ds(pl.multiple_of(qb * TQ, TQ), TQ)
        kv0 = 0 if first else pl.multiple_of(hg * (HPS * S2), HPS * S2)
        early = [None]
        passes = []
        mv = [jnp.zeros((8, 128), f32), 0]
        mpi = jnp.where(jnp.logical_and(t >= 2, t < 2 + NMP), t - 2, NMP)

        def qp(j):
            cols = slice(j * DH, (j + 1) * DH)
            if j == 1 or (j == 0 and not first):
                d0 = jnp.dot(h_ref[arows, 0:512], _w16(wqb[hg, 0:256, cols]), preferred_element_type=f32)
                d1 = jnp.dot(h_ref[arows, 512:], _w16(wqb[hg, 256:, cols]), preferred_element_type=f32)
                early[0] = jnp.abs(d0[0:16])
                passes.extend([d0, d1])
                q = d0 + d1
            else:
                q = jnp.dot(h_ref[arows, :], _w16(wqb[hg, :, cols]), preferred_element_type=f32)
            return q * (DH ** -0.5 * LOG2E)

        def qk(j, q):
            s = lax.dot_general(q.astype(bf16), _w16(kb[pl.ds(kv0 + j * S2, S2), :]), (((1,), (1,)), ((), ())),
                                preferred_element_type=f32)
            passes.extend([s[:, g * 512:g * 512 + 128] for g in range(4)])
            s_refs[j % 2][z] = s
            pm = s[:, 0:128]
            for c in range(1, S // 128):
                pm = jnp.maximum(pm, s[:, c * 128:(c + 1) * 128])
            m_ref[z, j] = jnp.broadcast_to(jnp.max(pm, axis=-1, keepdims=True), (TQ, 128))
            return jnp.abs(s[0:16, 0:128])

        def sm(j, tok=None):
            R, W = 16, S // 2
            sref = s_refs[j % 2]
            zs = z_ref[3 + j]
            for r in range(0, TQ, R):
                m = m_ref[zs, j, r:r + R, :]
                acc = None
                for hf in range(2):
                    mm = m if tok is None else jnp.where(tok < 0.0, 0.0, m)
                    p = jnp.exp2(sref[zs, r:r + R, hf * W:(hf + 1) * W] - _lanes(mm))
                    for c in range(W // 128):
                        pc = p[:, c * 128:(c + 1) * 128]
                        acc = pc if acc is None else acc + pc
                    if first or j != 1:
                        tok = acc
                        for _ in range(pads[j]):
                            tok = tok + tok
                    else:
                        a = jnp.where(jnp.minimum(acc[0:8], acc[8:16]) < 0.0, 1.0, mv[0])
                        for _ in range(MPW // 128):
                            mc, k0 = divmod(mv[1], D)
                            mv[1] += 16
                            w = _w16(wmb[mpi, k0 // 2:k0 // 2 + 8, mc * 128:(mc + 1) * 128]).astype(f32)
                            pr = w * scb_ref[k0:k0 + 16, :]
                            a = (a + pr[0:8]) + pr[8:16]
                            tok = a
                            if k0 + 16 == D:
                                mp_ref[mpi, :, mc * 128:(mc + 1) * 128] = a
                                a = jnp.where(jnp.abs(a) < 0.0, 1.0, 0.0)
                        mv[0] = a
                        tok = jnp.abs(tok)
                        tok = jnp.concatenate([tok, tok], axis=0)
                    p_refs[j % 2][pl.ds(zp + r, R), hf * W:(hf + 1) * W] = p.astype(bf16)
                l_refs[j][z, r:r + R, :] = acc

        def pv(j, between=None):
            pj = p_refs[j % 2]
            vv = _w16(vb[pl.ds(kv0 + j * S2, S2), :])
            d0 = jnp.dot(pj[pl.ds(zp, TQ), 0:512], vv[0:512], preferred_element_type=f32)
            o = d0 + jnp.dot(pj[pl.ds(zp, TQ), 512:], vv[512:], preferred_element_type=f32)
            early[0] = jnp.abs(d0[0:16])
            lp = jnp.maximum(l_refs[j][z2], jnp.minimum(d0, 0.0))
            l = jnp.broadcast_to(jnp.sum(lp, axis=-1, keepdims=True), (TQ, 128))
            if between is not None:
                between()
            o_ref[pl.ds(pl.multiple_of(slot * TQ, TQ), TQ), j * DH:(j + 1) * DH] = (o * _recip(l)).astype(bf16)

        def op_prev(c0, c1):
            tp = t - 1
            o = o_ref[pl.ds(pl.multiple_of((1 - slot) * TQ, TQ), TQ), :]
            rows = pl.ds(pl.multiple_of((tp >> 3) * TQ, TQ), TQ)
            d = jnp.dot(o, _w16(wob[tp & (NHG - 1), :, c0:c1]), preferred_element_type=f32)
            acc_ref[rows, c0:c1] += d
            return d

        def wait(*cps):
            for cp in cps:
                cp.wait()

        l0 = pl.multiple_of(jnp.minimum(t + NHG, NSTEP - 1) * CH, CH)

        if first:
            wait(cp0_wq[0])
            h_ref[0:TQ, :] = (s1_ref[0, :, 0:D] * bc(1, TQ) + bc(0, TQ)).astype(bf16)
            q0 = qp(0)
            wait(cp0_k[0])
            qk(0, q0)
            wait(cp0_wq[1], cp0_k[1], cp0_v[0], cp0_wq[2])
            q1 = qp(1)
            sm(0, early[0])
            qk(1, q1)
            sm(1)
            pv(0)
            q2 = qp(2)
            wait(cp0_k[2], cp0_v[1], cp0_wq[3], cp0_k[3], cp_x[1])
            qk(2, q2)
            sm(2)
            pv(1)
            q3 = qp(3)
            qk(3, q3)
            tok = jnp.abs(q3[TQ - 16:TQ, :])
            for g in range(0, CH, 16):
                tok = ln1_rows(l0 + g, 16, tok, h_ref, pl.multiple_of(l0 + g, 16))
            wait(cp0_v[2], cp0_v[3], cp_wr)
            pv(2)
            sm(3, early[0])
            pv(3)
            return

        def late(tc):
            r8 = (tc % TQ) // 8 * 8
            tk = jnp.abs(passes[tc // TQ][r8:r8 + 8, 0:128]) < 0.0
            return jnp.concatenate([tk, tk], axis=0)

        qk(0, qp(0))
        valid = t > NHG
        fsrc = pl.multiple_of(jnp.maximum(t - NHG - 1, 0) * CH, CH)
        fdst = pl.multiple_of(jnp.where(valid, fsrc, S), CH)
        top = (top_ref[0], topi_ref[0], top_ref[1], topi_ref[1])
        ftok = None
        for g in range(0, CH, 16):
            top, tk = fin_rows(fsrc + g, fdst + g, 16, valid, top, None, late(g * 16), late(g * 16 + 128))
            ftok = tk if ftok is None else jnp.minimum(ftok, tk)
        top_ref[0], topi_ref[0], top_ref[1], topi_ref[1] = top
        ltok = None
        for g in range(0, CH, 16):
            tk = ln1_rows(l0 + g, 16, None, hs_ref, zp + g, late(1280 + g * 16), late(1408 + g * 16))
            ltok = tk if ltok is None else jnp.minimum(ltok, tk)
        ltok = _both(ltok)
        q1 = qp(1)
        sm(0, jnp.minimum(_both(ftok), ltok))
        qk(1, q1)
        sm(1, ltok)
        pv(0)
        qk(2, qp(2))
        sm(2)
        pv(1)
        sm(3, qk(3, qp(3)))
        pv(2)
        never = _lanes(jnp.abs(op_prev(0, D // 2)[0:8, 0:128])) < 0.0
        for g in range(0, CH, 16):
            hv = hs_ref[pl.ds(pl.multiple_of(z2 * 16, 16) + g, 16), :].astype(f32)
            hv = jnp.concatenate([jnp.where(never, 0.0, hv[0:8]), hv[8:16]], axis=0)
            h_ref[pl.ds(l0 + g, 16), :] = hv.astype(bf16)
        op_prev(D // 2, D - 128)
        pv(3, lambda: op_prev(D - 128, D))

    attend(0, True)
    mod_ref[:, 6 * D:7 * D] = jnp.broadcast_to(wrb[...].astype(f32).reshape(1, D), (8, D))

    def step(t, _):
        attend(t, False)
        return 0

    def segment(k, _):
        t = jnp.where(k < NHG, k + 1, (k - NHG + 1) * NHG + 1)
        end = jnp.where(k < NHG, t + 1, jnp.minimum(t + NHG, NSTEP))

        @pl.when(t < NHG)
        def _():
            cp_wq(t).wait()
            cp_k(t).wait()
            cp_v(t).wait()

        @pl.when(t <= NHG)
        def _():
            cp_wo(t - 1).wait()

        @pl.when(jnp.logical_and(t >= 2, t < 2 + NMP))
        def _():
            pltpu.make_async_copy(wm_hbm.at[:, pl.ds(0, MPW)], wmb.at[t - 2], sem_wm.at[NMC + t - 2]).wait()

        @pl.when(t == 2)
        def _():
            cp_x[2].wait()

        @pl.when(t == NHG)
        def _():
            cp_x[3].wait()

        @pl.when(t == NHG + 1)
        def _():
            derive_params()

        @pl.when(t > 2 * NHG)
        def _():
            cp_out(k - NHG - 1).start()

        lax.fori_loop(t, end, step, 0)
        return 0

    lax.fori_loop(0, NHG + NQB - 1, segment, 0)

    top = (top_ref[0], topi_ref[0], top_ref[1], topi_ref[1])
    rl0 = (NQB - 1) * TQ
    EG, EB, EP = 16, 64, 144
    oslot = ((NSTEP - 1) % 2) * TQ
    ds = []
    for r in range(0, TQ, EB):
        d = jnp.dot(o_ref[oslot + r:oslot + r + EB, :], _w16(wob[NHG - 1]), preferred_element_type=f32)
        acc_ref[rl0 + r:rl0 + r + EB, :] += d
        ds.append(d)

    def late(tc):
        if tc >= TQ * 8:
            return None
        c = (tc % (EB * 8)) // EB
        tk = jnp.abs(ds[tc // (EB * 8)][0:8, c * 128:(c + 1) * 128]) < 0.0
        return jnp.concatenate([tk] * (EG // 8), axis=0)

    for r in range(-CH, TQ, EG):
        ready = (r + EB) * 8
        top, _ = fin_rows(rl0 + r, rl0 + r, EG, None, top, None, late(ready + 128), late(ready + 256),
                          write=r < TQ - EP)
        if r == -EG:
            cp_out(NQB - 2).start()

    for cp in cp_ffn:
        cp.wait()
    vals = jnp.concatenate([top[0], top[2]], axis=0)
    idxs = jnp.concatenate([top[1], top[3]], axis=0)
    m1 = jnp.max(vals, axis=0, keepdims=True)
    i1v = jnp.min(jnp.where(vals == m1, idxs, S - 1), axis=0, keepdims=True)
    vals2 = jnp.where(idxs == i1v, -jnp.inf, vals)
    m2 = jnp.max(vals2, axis=0, keepdims=True)
    i2v = jnp.min(jnp.where(jnp.logical_and(vals2 == m2, idxs != i1v), idxs, S - 1), axis=0, keepdims=True)
    b1 = pl.multiple_of(jnp.clip(i1v[0, 0] // 8 * 8, 0, S - 8), 8)
    b2 = pl.multiple_of(jnp.clip(i2v[0, 0] // 8 * 8, 0, S - 8), 8)

    def two(ref_rows):
        return jnp.concatenate([ref_rows(b1), ref_rows(b2)], axis=0)

    x1 = two(lambda b: xb[pl.ds(b, 8), :].astype(f32)) + bc(2, 16) * two(lambda b: acc_ref[pl.ds(b, 8), :])
    xn = (x1 - _lanes(two(lambda b: st_ref[0, pl.ds(b, 8), :]))) * _lanes(two(lambda b: st_ref[1, pl.ds(b, 8), :]))
    xs = (xn * bc(4, 16) + bc(3, 16)).astype(bf16)
    sub = lax.broadcasted_iota(jnp.int32, (8, 128), 0)
    ids = jnp.concatenate([sub + b1, sub + b2], axis=0)

    NV, CB, FC = 1024, 256, 640
    FM = F - NV
    xf = xs.astype(f32)
    rows = [jnp.sum(jnp.where(_lanes(ids[lo:lo + 8] == iv), xf[lo:lo + 8], 0.0), axis=0, keepdims=True)
            for lo, iv in ((0, i1v), (8, i2v))]
    rows = [jnp.broadcast_to(r, (8, D)) for r in rows]
    pk = pltpu.bitcast(rows[0], u32) | (pltpu.bitcast(rows[1], u32) >> 16)
    for b in range(D // 128):
        xt_ref[0, b * 128:(b + 1) * 128, :] = jnp.concatenate([pk[:, b * 128:(b + 1) * 128]] * 16, axis=0).T

    def wide(v):
        return jnp.concatenate([v] * (CB // 128), axis=1)

    def vpu_cols(c, start):
        zt = z_ref[2]
        acc = [wide(start)] * 4
        for k0 in range(0, D, 16):
            tb = xt_ref[zt, k0:k0 + 16, :]
            xk = (wide(pltpu.bitcast(tb & jnp.uint32(0xFFFF0000), f32)), wide(pltpu.bitcast(tb << 16, f32)))
            for wi, w_ref in enumerate((wgb, wub)):
                w = _w16(w_ref[k0 // 2:k0 // 2 + 8, c:c + CB]).astype(f32)
                for k in range(2):
                    pr = w * xk[k]
                    acc[2 * wi + k] = (acc[2 * wi + k] + pr[0:8]) + pr[8:16]
        tot = (jnp.abs(acc[0]) + jnp.abs(acc[1])) + (jnp.abs(acc[2]) + jnp.abs(acc[3]))
        tot = tot[:, 0:128] + tot[:, 128:256]
        red = [jnp.broadcast_to(jnp.sum(a, axis=0, keepdims=True), (16, CB)) for a in acc]
        g, u = (jnp.where(wide(ids == i1v), red[2 * wi], red[2 * wi + 1]) for wi in range(2))
        return g * jax.nn.sigmoid(g) * u, jnp.where(tot < 0.0, 1.0, 0.0)

    av = []
    start = jnp.zeros((8, 128), f32)
    for c in range(FM, F, CB):
        out, start = vpu_cols(c, start)
        av.append(out)

    y = None
    prev = None
    for c in range(0, FM + FC, FC):
        if c < FM:
            g = jnp.dot(xs, _w16(wgb[:, c:c + FC]), preferred_element_type=f32)
            u = jnp.dot(xs, _w16(wub[:, c:c + FC]), preferred_element_type=f32)
        if prev is not None:
            d = jnp.dot(prev, _w16(wdb[(c - FC) // 2:c // 2, :]), preferred_element_type=f32)
            y = d if y is None else y + d
        if c < FM:
            prev = (g * jax.nn.sigmoid(g) * u).astype(bf16)
        if c == 0:
            gu = jnp.concatenate([g, u], axis=1)
            for gi, r0 in enumerate(range(S - EP, S, EG)):
                gc = gi * (2 * FC // 128) // (EP // EG)
                never = jnp.abs(gu[:, gc * 128:(gc + 1) * 128]) < 0.0
                xx = xb[r0:r0 + EG, :].astype(f32) + bc(2, EG) * acc_ref[r0:r0 + EG, :]
                rs = jnp.where(never, 0.0, st_ref[1, r0:r0 + EG, :])
                mb = jnp.where(never, 0.0, st_ref[0, r0:r0 + EG, :])
                ob[r0:r0 + EG, :] = ((xx + bc(7, EG)) + ((xx - _lanes(mb)) * _lanes(rs)) * bc(8, EG)).astype(bf16)
            cp_out(NQB - 1).start()
    for i, a in enumerate(av):
        c = FM + i * CB
        y = y + jnp.dot(a.astype(bf16), _w16(wdb[c // 2:(c + CB) // 2, :]), preferred_element_type=f32)
    upd = jnp.where(_lanes(ids == i1v), y * _lanes(jax.nn.sigmoid(m1)),
                    jnp.where(_lanes(ids == i2v), y * _lanes(jax.nn.sigmoid(m2)), 0.0))
    fixb[...] = ((x1 + bc(7, 16)) + xn * bc(8, 16) + bc(5, 16) * upd).astype(bf16)

    for qb in range(NQB):
        cp_out(qb).wait()
    cf1 = pltpu.make_async_copy(fixb.at[pl.ds(0, 8)], o_hbm.at[pl.ds(b1, 8)], sem_o.at[NQB])
    cf2 = pltpu.make_async_copy(fixb.at[pl.ds(8, 8)], o_hbm.at[pl.ds(b2, 8)], sem_o.at[NQB + 1])
    cf1.start()

    @pl.when(b1 != b2)
    def _():
        cf2.start()
        cf2.wait()
    cf1.wait()


@jax.jit
def pallas_adaLN_cond__mha_block_cached__moe_arch_mod__prompt_kernel(
    A_x: jax.Array,
    A_k_cache: jax.Array,
    A_v_cache: jax.Array,
    A_wq: jax.Array,
    A_wo: jax.Array,
    B_x: jax.Array,
    B_w_r: jax.Array,
    B_w_gate: jax.Array,
    B_w_up: jax.Array,
    B_w_down: jax.Array,
    c: jax.Array,
    w_mod: jax.Array,
):
    x = A_x.reshape(S, D)
    k = A_k_cache.reshape(H * S, DH)
    v = A_v_cache.reshape(H * S, DH)
    wo = A_wo.reshape(NHG, HPS * DH, D)
    anyspec = pl.BlockSpec(memory_space=pl.ANY)
    out = pl.pallas_call(
        _kernel,
        in_specs=[anyspec] * 11,
        out_specs=anyspec,
        out_shape=jax.ShapeDtypeStruct((S, D), bf16),
        scratch_shapes=[
            pltpu.VMEM((S, D), bf16),
            pltpu.VMEM((H * S2, DH), u32),
            pltpu.VMEM((H * S2, DH), u32),
            pltpu.VMEM((NHG, D // 2, HPS * DH), u32),
            pltpu.VMEM((NHG, HPS * DH // 2, D), u32),
            pltpu.VMEM((D // 2, F), u32),
            pltpu.VMEM((D // 2, F), u32),
            pltpu.VMEM((F // 2, D), u32),
            pltpu.VMEM((NMP + 1, D // 2, MPW), u32),
            pltpu.VMEM((8, 11 * D), f32),
            pltpu.VMEM((S // 2, D), u32),
            pltpu.VMEM((S, D), f32),
            pltpu.VMEM((S + CH, D), bf16),
            pltpu.VMEM((16, D), bf16),
            pltpu.VMEM((1, TQ, S), f32),
            pltpu.VMEM((1, TQ, S), f32),
            pltpu.VMEM((TQ // 2, S), u32),
            pltpu.VMEM((TQ // 2, S), u32),
            pltpu.VMEM((1, HPS, TQ, 128), f32),
            pltpu.VMEM((1, TQ, 128), f32),
            pltpu.VMEM((1, TQ, 128), f32),
            pltpu.VMEM((1, TQ, 128), f32),
            pltpu.VMEM((1, TQ, 128), f32),
            pltpu.VMEM((CH // 2, D), u32),
            pltpu.VMEM((TQ, HPS * DH), u32),
            pltpu.VMEM((2, S + CH, 128), f32),
            pltpu.VMEM((D, 128), f32),
            pltpu.VMEM((1, D, 128), u32),
            pltpu.VMEM((NMP + 1, 8, MPW), f32),
            pltpu.VMEM((2, 8, 128), f32),
            pltpu.VMEM((2, 8, 128), jnp.int32),
            pltpu.VMEM((D,), bf16),
            pltpu.VMEM((1, D), bf16),
            pltpu.SMEM((8,), jnp.int32),
            pltpu.SemaphoreType.DMA((2,)),
            pltpu.SemaphoreType.DMA((4,)),
            pltpu.SemaphoreType.DMA((NMC + NMP,)),
            pltpu.SemaphoreType.DMA((NHG,)),
            pltpu.SemaphoreType.DMA((NHG,)),
            pltpu.SemaphoreType.DMA((2 * NHG,)),
            pltpu.SemaphoreType.DMA((3 * HPS,)),
            pltpu.SemaphoreType.DMA((3,)),
            pltpu.SemaphoreType.DMA((NQB + 2,)),
        ],
        compiler_params=pltpu.CompilerParams(vmem_limit_bytes=124 * 1024 * 1024, disable_bounds_checks=True,
                                             disable_semaphore_checks=True),
    )(x, k, v, A_wq, wo, B_w_r, B_w_gate, B_w_up, B_w_down, c, w_mod)
    return out.reshape(1, S, D)
```

```python
import jax
import jax.numpy as jnp
from jax import lax
import jax.experimental.pallas as pl
import jax.experimental.pallas.tpu as pltpu

S = 2048
S2 = S // 2
D = 1024
H = 32
DH = 128
F = 3584
EPS = 1e-5
LOG2E = 1.4426950408889634
TQ = 512
NQB = S // TQ
HPS = 4
NHG = H // HPS
NSTEP = NQB * NHG
CH = TQ // NHG
MPW = 768
NMP = -(-4 * D // MPW)
NMC = 4
MCW = 2 * D // NMC
PADS = (6, 5, 6, 4)
PADS0 = (5, 5, 5, 0)

f32 = jnp.float32
bf16 = jnp.bfloat16
u32 = jnp.uint32


def _mp_col(p):
    return min(p * MPW, 4 * D - MPW)


def _rb(x):
    return x.astype(bf16).astype(f32)


def _recip(x):
    r = pl.reciprocal(x, approx=True)
    return r * (2.0 - x * r)


def _rowsum(x, late=None):
    p = x[:, 0:128]
    for c in range(1, x.shape[1] // 128):
        p = p + x[:, c * 128:(c + 1) * 128]
    if late is not None:
        p = jnp.where(late, 0.0, p)
    return jnp.sum(p, axis=-1, keepdims=True)


def _center(x, late=None):
    m = _rowsum(x, late) * (1.0 / D)
    mb = _rb(m)
    return x - mb, mb, m - mb


def _rstd(xc, dm, late=None):
    v = jnp.maximum(_rowsum(xc * xc, late) * (1.0 / D) - dm * dm, 0.0)
    y = _rb(_rb(v) + EPS)
    return _recip(_rb(y * lax.rsqrt(y)))


def _ln(x, late1=None, late2=None):
    xc, _, dm = _center(x, late1)
    return xc * _rstd(xc, dm, late2)


def _tie(x, tok):
    if tok is None:
        return x
    return jnp.concatenate([jnp.where(tok < 0.0, 0.0, x[:, 0:128]), x[:, 128:]], axis=1)


def _both(tok):
    tok = jnp.minimum(tok[0:8], tok[8:16])
    return jnp.concatenate([tok, tok], axis=0)


def _lanes(v):
    return jnp.concatenate([v] * (D // 128), axis=1)


def _w16(x):
    return pltpu.bitcast(x, bf16)


def _kernel(x_hbm, k_hbm, v_hbm, wq_hbm, wo_hbm, wr_hbm, wg_hbm, wu_hbm, wd_hbm, c_hbm, wm_hbm,
            o_hbm,
            xb, kb, vb, wqb, wob, wgb, wub, wdb, wmb,
            mod_ref, h_ref, acc_ref, ob, fixb, s0_ref, s1_ref, p0_ref, p1_ref, m_ref,
            l0_ref, l1_ref, l2_ref, l3_ref, hs_ref, o_ref, st_ref, scb_ref, xt_ref, mp_ref, top_ref, topi_ref,
            wrb, cb_, z_ref,
            sem_s, sem_x, sem_wm, sem_k, sem_v, sem_w, sem_0, sem_f, sem_o):
    h_ref, p0_ref, p1_ref, o_ref, hs_ref = (r.bitcast(bf16) for r in (h_ref, p0_ref, p1_ref, o_ref, hs_ref))
    wm0_hbm = wm_hbm.bitcast(f32)
    k_hbm, v_hbm, wq_hbm, wo_hbm, wg_hbm, wu_hbm, wd_hbm, wm_hbm = (
        r.bitcast(u32) for r in (k_hbm, v_hbm, wq_hbm, wo_hbm, wg_hbm, wu_hbm, wd_hbm, wm_hbm))

    cp_c = pltpu.make_async_copy(c_hbm, cb_, sem_s.at[0])
    cp_wr = pltpu.make_async_copy(wr_hbm, wrb, sem_s.at[1])
    xcuts = (0, TQ, TQ + 2 * CH, 2 * TQ + 2 * CH, S)
    cp_x = [pltpu.make_async_copy(x_hbm.at[pl.ds(a, b - a)], xb.at[pl.ds(a, b - a)], sem_x.at[i])
            for i, (a, b) in enumerate(zip(xcuts, xcuts[1:]))]

    def cp_wm(i):
        cols = pl.ds(i * MCW, MCW)
        return pltpu.make_async_copy(wm0_hbm.at[:, cols], s0_ref.at[0, :, cols], sem_wm.at[i])

    def cp_wmr(p):
        return pltpu.make_async_copy(wm_hbm.at[:, pl.ds(2 * D + _mp_col(p), MPW)], wmb.at[p], sem_wm.at[NMC + p])

    def cp_k(g):
        rows = pl.ds(pl.multiple_of(g * (HPS * S2), HPS * S2), HPS * S2)
        return pltpu.make_async_copy(k_hbm.at[rows], kb.at[rows], sem_k.at[g])

    def cp_v(g):
        rows = pl.ds(pl.multiple_of(g * (HPS * S2), HPS * S2), HPS * S2)
        return pltpu.make_async_copy(v_hbm.at[rows], vb.at[rows], sem_v.at[g])

    def cp_wq(g):
        cols = pl.ds(pl.multiple_of(g * (HPS * DH), HPS * DH), HPS * DH)
        return pltpu.make_async_copy(wq_hbm.at[:, cols], wqb.at[g], sem_w.at[g])

    def cp_wo(g):
        return pltpu.make_async_copy(wo_hbm.at[g], wob.at[g], sem_w.at[NHG + g])

    cp0_wq = [pltpu.make_async_copy(wq_hbm.at[:, pl.ds(j * DH, DH)], wqb.at[0, :, pl.ds(j * DH, DH)], sem_0.at[j])
              for j in range(HPS)]
    cp0_k = [pltpu.make_async_copy(k_hbm.at[pl.ds(j * S2, S2)], kb.at[pl.ds(j * S2, S2)], sem_0.at[HPS + j])
             for j in range(HPS)]
    cp0_v = [pltpu.make_async_copy(v_hbm.at[pl.ds(j * S2, S2)], vb.at[pl.ds(j * S2, S2)], sem_0.at[2 * HPS + j])
             for j in range(HPS)]

    cp_ffn = [pltpu.make_async_copy(wg_hbm, wgb, sem_f.at[0]),
              pltpu.make_async_copy(wu_hbm, wub, sem_f.at[1]),
              pltpu.make_async_copy(wd_hbm, wdb, sem_f.at[2])]

    def cp_out(qb):
        rows = pl.ds(pl.multiple_of(qb * TQ, TQ), TQ)
        return pltpu.make_async_copy(ob.at[rows], o_hbm.at[rows], sem_o.at[qb])

    cp_c.start()
    cp_x[0].start()
    for i in range(NMC):
        cp_wm(i).start()
    for cp in (cp0_wq[0], cp0_k[0], cp0_wq[1], cp0_k[1], cp0_v[0], cp0_wq[2], cp0_k[2], cp0_v[1],
               cp0_wq[3], cp0_k[3], cp_x[1], cp0_v[2], cp0_v[3], cp_wr):
        cp.start()
    for g in range(1, NHG):
        cps = [cp_wq(g), cp_k(g), cp_v(g), cp_wo(g - 1)]
        cps += [cp_x[2]] if g == 1 else []
        cps += [cp_wmr(g - 1)] if g <= NMP else []
        for cp in cps:
            cp.start()
    for cp in [cp_wo(NHG - 1), cp_x[3]] + cp_ffn:
        cp.start()

    def zbody(i, _):
        acc_ref[pl.ds(pl.multiple_of(i * 256, 256), 256), :] = jnp.zeros((256, D), f32)
        wmb[NMP, pl.ds(pl.multiple_of(i * 64, 64), 64), :] = jnp.zeros((64, MPW), u32)
        z_ref[i] = 0
        return 0
    lax.fori_loop(0, S // 256, zbody, 0)
    mod_ref[...] = jnp.zeros(mod_ref.shape, f32)
    top_ref[...] = jnp.full(top_ref.shape, -jnp.inf, f32)
    topi_ref[0] = jnp.zeros((8, 128), jnp.int32)
    topi_ref[1] = jnp.ones((8, 128), jnp.int32)

    def bc(k, n):
        p = mod_ref[:, k * D:(k + 1) * D]
        return p if n == 8 else jnp.concatenate([p] * (n // 8), axis=0)

    cp_x[0].wait()

    def nbody(i, _):
        rows = pl.ds(pl.multiple_of(i * 128, 128), 128)
        s1_ref[0, rows, 0:D] = _ln(xb[rows, :].astype(f32))
        return 0
    lax.fori_loop(0, TQ // 128, nbody, 0)

    cp_c.wait()

    def silu_c():
        c = cb_[...].astype(f32)
        sc = (c * jax.nn.sigmoid(c)).astype(bf16)
        return jnp.broadcast_to(sc, (8, D))

    scf = silu_c().astype(f32)
    for b in range(D // 128):
        blk = jnp.concatenate([scf[:, b * 128:(b + 1) * 128]] * 16, axis=0)
        scb_ref[b * 128:(b + 1) * 128, :] = blk.T

    for i in range(NMC):
        cp_wm(i).wait()
        lo = i * MCW
        md = _rb(jnp.dot(silu_c(), _w16(s0_ref[0, :, lo:lo + MCW]), preferred_element_type=f32))
        mod_ref[:, lo:lo + MCW] = _rb(1.0 + md) if lo >= D else md

    def ln1_rows(r0, n, tok, dst_ref, d0, late1=None, late2=None):
        x = _tie(xb[pl.ds(r0, n), :].astype(f32), tok)
        h = _ln(x, late1, late2) * bc(1, n) + bc(0, n)
        dst_ref[pl.ds(d0, n), :] = h.astype(bf16)
        return jnp.abs(h[:, 0:128])

    def derive_params():
        for c in range(4 * D // 128):
            p = c * 128 // MPW
            o = c * 128 - _mp_col(p)
            md = _rb(jnp.broadcast_to(jnp.sum(mp_ref[p, :, o:o + 128], axis=0, keepdims=True), (8, 128)))
            if 2 * D <= c * 128 < 3 * D:
                md = _rb(1.0 + md)
            mod_ref[:, 2 * D + c * 128:2 * D + (c + 1) * 128] = md
        sb, cb1, gb, wr = bc(3, 8), bc(4, 8), bc(5, 8), bc(6, 8)
        mod_ref[:, 7 * D:8 * D] = gb * sb
        mod_ref[:, 8 * D:9 * D] = gb * cb1
        mod_ref[:, 9 * D:10 * D] = cb1 * wr
        mod_ref[:, 10 * D:10 * D + 128] = jnp.broadcast_to(jnp.sum(sb * wr, axis=-1, keepdims=True), (8, 128))

    def fin_rows(r0, d0, n, valid, top, tok=None, late1=None, late2=None, write=True):
        x = _tie(xb[pl.ds(r0, n), :].astype(f32), tok)
        x1b = (x + bc(2, n) * acc_ref[pl.ds(r0, n), :]).astype(bf16)
        x1 = x1b.astype(f32)
        xc, mb, dm = _center(x1, late1)
        rs = _rstd(xc, dm, late2)
        st_ref[0, pl.ds(d0, n), :] = jnp.broadcast_to(mb, (n, 128))
        st_ref[1, pl.ds(d0, n), :] = jnp.broadcast_to(rs, (n, 128))
        if write:
            ob[pl.ds(d0, n), :] = ((x1 + bc(7, n)) + (xc * rs) * bc(8, n)).astype(bf16)
        else:
            ob[pl.ds(d0, n), :] = x1b
        rc = mod_ref[:, 10 * D:10 * D + 128]
        r = jnp.broadcast_to(_rowsum(xc * bc(9, n), late2) * rs, (n, 128))
        r = _rb(r + jnp.concatenate([rc] * (n // 8), axis=0))
        tok = jnp.abs(r)
        if valid is not None:
            r = jnp.where(valid, r, -jnp.inf)
        b1, i1, b2, i2 = top
        sub = lax.broadcasted_iota(jnp.int32, (8, 128), 0)
        for g in range(n // 8):
            rg = r[g * 8:(g + 1) * 8, :]
            ids = sub + (r0 + g * 8)
            gt1 = rg > b1
            gt2 = rg > b2
            b2 = jnp.where(gt1, b1, jnp.where(gt2, rg, b2))
            i2 = jnp.where(gt1, i1, jnp.where(gt2, ids, i2))
            b1 = jnp.where(gt1, rg, b1)
            i1 = jnp.where(gt1, ids, i1)
        return (b1, i1, b2, i2), tok

    s_refs = (s0_ref, s1_ref)
    p_refs = (p0_ref, p1_ref)
    l_refs = (l0_ref, l1_ref, l2_ref, l3_ref)

    def attend(t, first):
        qb = t >> 3
        hg = t & (NHG - 1)
        slot = t & 1
        pads = PADS0 if first else PADS
        z = z_ref[0]
        z2 = z_ref[1]
        zp = pl.multiple_of(z * 16, 16)
        arows = pl.ds(pl.multiple_of(qb * TQ, TQ), TQ)
        kv0 = 0 if first else pl.multiple_of(hg * (HPS * S2), HPS * S2)
        early = [None]
        passes = []
        mv = [jnp.zeros((8, 128), f32), 0]
        mpi = jnp.where(jnp.logical_and(t >= 2, t < 2 + NMP), t - 2, NMP)

        def qp(j):
            cols = slice(j * DH, (j + 1) * DH)
            if j == 1 or (j == 0 and not first):
                d0 = jnp.dot(h_ref[arows, 0:512], _w16(wqb[hg, 0:256, cols]), preferred_element_type=f32)
                d1 = jnp.dot(h_ref[arows, 512:], _w16(wqb[hg, 256:, cols]), preferred_element_type=f32)
                early[0] = jnp.abs(d0[0:16])
                passes.extend([d0, d1])
                q = d0 + d1
            else:
                q = jnp.dot(h_ref[arows, :], _w16(wqb[hg, :, cols]), preferred_element_type=f32)
            return q * (DH ** -0.5 * LOG2E)

        def qk(j, q):
            s = lax.dot_general(q.astype(bf16), _w16(kb[pl.ds(kv0 + j * S2, S2), :]), (((1,), (1,)), ((), ())),
                                preferred_element_type=f32)
            passes.extend([s[:, g * 512:g * 512 + 128] for g in range(4)])
            s_refs[j % 2][z] = s
            pm = s[:, 0:128]
            for c in range(1, S // 128):
                pm = jnp.maximum(pm, s[:, c * 128:(c + 1) * 128])
            m_ref[z, j] = jnp.broadcast_to(jnp.max(pm, axis=-1, keepdims=True), (TQ, 128))
            return jnp.abs(s[0:16, 0:128])

        def sm(j, tok=None):
            R, W = 16, S // 2
            sref = s_refs[j % 2]
            zs = z_ref[3 + j]
            for r in range(0, TQ, R):
                m = m_ref[zs, j, r:r + R, :]
                acc = None
                for hf in range(2):
                    mm = m if tok is None else jnp.where(tok < 0.0, 0.0, m)
                    p = jnp.exp2(sref[zs, r:r + R, hf * W:(hf + 1) * W] - _lanes(mm))
                    for c in range(W // 128):
                        pc = p[:, c * 128:(c + 1) * 128]
                        acc = pc if acc is None else acc + pc
                    if first or j != 1:
                        tok = acc
                        for _ in range(pads[j]):
                            tok = tok + tok
                    else:
                        a = jnp.where(jnp.minimum(acc[0:8], acc[8:16]) < 0.0, 1.0, mv[0])
                        for _ in range(MPW // 128):
                            mc, k0 = divmod(mv[1], D)
                            mv[1] += 16
                            w = _w16(wmb[mpi, k0 // 2:k0 // 2 + 8, mc * 128:(mc + 1) * 128]).astype(f32)
                            pr = w * scb_ref[k0:k0 + 16, :]
                            a = (a + pr[0:8]) + pr[8:16]
                            tok = a
                            if k0 + 16 == D:
                                mp_ref[mpi, :, mc * 128:(mc + 1) * 128] = a
                                a = jnp.where(jnp.abs(a) < 0.0, 1.0, 0.0)
                        mv[0] = a
                        tok = jnp.abs(tok)
                        tok = jnp.concatenate([tok, tok], axis=0)
                    p_refs[j % 2][pl.ds(zp + r, R), hf * W:(hf + 1) * W] = p.astype(bf16)
                l_refs[j][z, r:r + R, :] = acc

        def pv(j, between=None):
            pj = p_refs[j % 2]
            vv = _w16(vb[pl.ds(kv0 + j * S2, S2), :])
            d0 = jnp.dot(pj[pl.ds(zp, TQ), 0:512], vv[0:512], preferred_element_type=f32)
            o = d0 + jnp.dot(pj[pl.ds(zp, TQ), 512:], vv[512:], preferred_element_type=f32)
            early[0] = jnp.abs(d0[0:16])
            lp = jnp.maximum(l_refs[j][z2], jnp.minimum(d0, 0.0))
            l = jnp.broadcast_to(jnp.sum(lp, axis=-1, keepdims=True), (TQ, 128))
            if between is not None:
                between()
            o_ref[pl.ds(pl.multiple_of(slot * TQ, TQ), TQ), j * DH:(j + 1) * DH] = (o * _recip(l)).astype(bf16)

        def op_prev(c0, c1):
            tp = t - 1
            o = o_ref[pl.ds(pl.multiple_of((1 - slot) * TQ, TQ), TQ), :]
            rows = pl.ds(pl.multiple_of((tp >> 3) * TQ, TQ), TQ)
            d = jnp.dot(o, _w16(wob[tp & (NHG - 1), :, c0:c1]), preferred_element_type=f32)
            acc_ref[rows, c0:c1] += d
            return d

        def wait(*cps):
            for cp in cps:
                cp.wait()

        l0 = pl.multiple_of(jnp.minimum(t + NHG, NSTEP - 1) * CH, CH)

        if first:
            wait(cp0_wq[0])
            h_ref[0:TQ, :] = (s1_ref[0, :, 0:D] * bc(1, TQ) + bc(0, TQ)).astype(bf16)
            q0 = qp(0)
            wait(cp0_k[0])
            qk(0, q0)
            wait(cp0_wq[1], cp0_k[1], cp0_v[0], cp0_wq[2])
            q1 = qp(1)
            sm(0, early[0])
            qk(1, q1)
            sm(1)
            pv(0)
            q2 = qp(2)
            wait(cp0_k[2], cp0_v[1], cp0_wq[3], cp0_k[3], cp_x[1])
            qk(2, q2)
            sm(2)
            pv(1)
            q3 = qp(3)
            qk(3, q3)
            tok = jnp.abs(q3[TQ - 16:TQ, :])
            for g in range(0, CH, 16):
                tok = ln1_rows(l0 + g, 16, tok, h_ref, pl.multiple_of(l0 + g, 16))
            wait(cp0_v[2], cp0_v[3], cp_wr)
            pv(2)
            sm(3, early[0])
            pv(3)
            return

        def late(tc):
            r8 = (tc % TQ) // 8 * 8
            tk = jnp.abs(passes[tc // TQ][r8:r8 + 8, 0:128]) < 0.0
            return jnp.concatenate([tk, tk], axis=0)

        qk(0, qp(0))
        valid = t > NHG
        fsrc = pl.multiple_of(jnp.maximum(t - NHG - 1, 0) * CH, CH)
        fdst = pl.multiple_of(jnp.where(valid, fsrc, S), CH)
        top = (top_ref[0], topi_ref[0], top_ref[1], topi_ref[1])
        ftok = None
        for g in range(0, CH, 16):
            top, tk = fin_rows(fsrc + g, fdst + g, 16, valid, top, None, late(g * 16), late(g * 16 + 128))
            ftok = tk if ftok is None else jnp.minimum(ftok, tk)
        top_ref[0], topi_ref[0], top_ref[1], topi_ref[1] = top
        ltok = None
        for g in range(0, CH, 16):
            tk = ln1_rows(l0 + g, 16, None, hs_ref, zp + g, late(1280 + g * 16), late(1408 + g * 16))
            ltok = tk if ltok is None else jnp.minimum(ltok, tk)
        ltok = _both(ltok)
        q1 = qp(1)
        sm(0, jnp.minimum(_both(ftok), ltok))
        qk(1, q1)
        sm(1, ltok)
        pv(0)
        qk(2, qp(2))
        sm(2)
        pv(1)
        sm(3, qk(3, qp(3)))
        pv(2)
        never = _lanes(jnp.abs(op_prev(0, D // 2)[0:8, 0:128])) < 0.0
        for g in range(0, CH, 16):
            hv = hs_ref[pl.ds(pl.multiple_of(z2 * 16, 16) + g, 16), :].astype(f32)
            hv = jnp.concatenate([jnp.where(never, 0.0, hv[0:8]), hv[8:16]], axis=0)
            h_ref[pl.ds(l0 + g, 16), :] = hv.astype(bf16)
        op_prev(D // 2, D - 128)
        pv(3, lambda: op_prev(D - 128, D))

    attend(0, True)
    mod_ref[:, 6 * D:7 * D] = jnp.broadcast_to(wrb[...].astype(f32).reshape(1, D), (8, D))

    def step(t, _):
        attend(t, False)
        return 0

    def segment(k, _):
        t = jnp.where(k < NHG, k + 1, (k - NHG + 1) * NHG + 1)
        end = jnp.where(k < NHG, t + 1, jnp.minimum(t + NHG, NSTEP))

        @pl.when(t < NHG)
        def _():
            cp_wq(t).wait()
            cp_k(t).wait()
            cp_v(t).wait()

        @pl.when(t <= NHG)
        def _():
            cp_wo(t - 1).wait()

        @pl.when(jnp.logical_and(t >= 2, t < 2 + NMP))
        def _():
            pltpu.make_async_copy(wm_hbm.at[:, pl.ds(0, MPW)], wmb.at[t - 2], sem_wm.at[NMC + t - 2]).wait()

        @pl.when(t == 2)
        def _():
            cp_x[2].wait()

        @pl.when(t == NHG)
        def _():
            cp_x[3].wait()

        @pl.when(t == NHG + 1)
        def _():
            derive_params()

        @pl.when(t > 2 * NHG)
        def _():
            cp_out(k - NHG - 1).start()

        lax.fori_loop(t, end, step, 0)
        return 0

    lax.fori_loop(0, NHG + NQB - 1, segment, 0)

    top = (top_ref[0], topi_ref[0], top_ref[1], topi_ref[1])
    rl0 = (NQB - 1) * TQ
    EG, EB, EP = 16, 128, 160
    oslot = ((NSTEP - 1) % 2) * TQ
    ds = []
    for r in range(0, TQ, EB):
        d = jnp.dot(o_ref[oslot + r:oslot + r + EB, :], _w16(wob[NHG - 1]), preferred_element_type=f32)
        acc_ref[rl0 + r:rl0 + r + EB, :] += d
        ds.append(d)

    def late(tc):
        if tc >= TQ * 8 - 256:
            return None
        c = (tc % (EB * 8)) // EB
        tk = jnp.abs(ds[tc // (EB * 8)][0:8, c * 128:(c + 1) * 128]) < 0.0
        return jnp.concatenate([tk] * (EG // 8), axis=0)

    for r in range(-CH, TQ, EG):
        ready = (r + EB) * 8
        top, _ = fin_rows(rl0 + r, rl0 + r, EG, None, top, None, late(ready + 128), late(ready + 256),
                          write=r < TQ - EP)
        if r == -EG:
            cp_out(NQB - 2).start()

    for cp in cp_ffn:
        cp.wait()
    vals = jnp.concatenate([top[0], top[2]], axis=0)
    idxs = jnp.concatenate([top[1], top[3]], axis=0)
    m1 = jnp.max(vals, axis=0, keepdims=True)
    i1v = jnp.min(jnp.where(vals == m1, idxs, S - 1), axis=0, keepdims=True)
    vals2 = jnp.where(idxs == i1v, -jnp.inf, vals)
    m2 = jnp.max(vals2, axis=0, keepdims=True)
    i2v = jnp.min(jnp.where(jnp.logical_and(vals2 == m2, idxs != i1v), idxs, S - 1), axis=0, keepdims=True)
    b1 = pl.multiple_of(jnp.clip(i1v[0, 0] // 8 * 8, 0, S - 8), 8)
    b2 = pl.multiple_of(jnp.clip(i2v[0, 0] // 8 * 8, 0, S - 8), 8)

    def two(ref_rows):
        return jnp.concatenate([ref_rows(b1), ref_rows(b2)], axis=0)

    x1 = _rb(two(lambda b: xb[pl.ds(b, 8), :].astype(f32)) + bc(2, 16) * two(lambda b: acc_ref[pl.ds(b, 8), :]))
    xn = (x1 - _lanes(two(lambda b: st_ref[0, pl.ds(b, 8), :]))) * _lanes(two(lambda b: st_ref[1, pl.ds(b, 8), :]))
    xs = (xn * bc(4, 16) + bc(3, 16)).astype(bf16)
    sub = lax.broadcasted_iota(jnp.int32, (8, 128), 0)
    ids = jnp.concatenate([sub + b1, sub + b2], axis=0)

    NV, CB, FC = 1024, 256, 768
    FM = F - NV
    xf = xs.astype(f32)
    rows = [jnp.sum(jnp.where(_lanes(ids[lo:lo + 8] == iv), xf[lo:lo + 8], 0.0), axis=0, keepdims=True)
            for lo, iv in ((0, i1v), (8, i2v))]
    rows = [jnp.broadcast_to(r, (8, D)) for r in rows]
    pk = pltpu.bitcast(rows[0], u32) | (pltpu.bitcast(rows[1], u32) >> 16)
    for b in range(D // 128):
        xt_ref[0, b * 128:(b + 1) * 128, :] = jnp.concatenate([pk[:, b * 128:(b + 1) * 128]] * 16, axis=0).T

    def wide(v):
        return jnp.concatenate([v] * (CB // 128), axis=1)

    def vpu_cols(c, start):
        zt = z_ref[2]
        acc = [wide(start)] * 4
        for k0 in range(0, D, 16):
            tb = xt_ref[zt, k0:k0 + 16, :]
            xk = (wide(pltpu.bitcast(tb & jnp.uint32(0xFFFF0000), f32)), wide(pltpu.bitcast(tb << 16, f32)))
            for wi, w_ref in enumerate((wgb, wub)):
                w = _w16(w_ref[k0 // 2:k0 // 2 + 8, c:c + CB]).astype(f32)
                for k in range(2):
                    pr = w * xk[k]
                    acc[2 * wi + k] = (acc[2 * wi + k] + pr[0:8]) + pr[8:16]
        tot = (jnp.abs(acc[0]) + jnp.abs(acc[1])) + (jnp.abs(acc[2]) + jnp.abs(acc[3]))
        tot = tot[:, 0:128] + tot[:, 128:256]
        red = [jnp.broadcast_to(jnp.sum(a, axis=0, keepdims=True), (16, CB)) for a in acc]
        g, u = (jnp.where(wide(ids == i1v), red[2 * wi], red[2 * wi + 1]) for wi in range(2))
        return g * jax.nn.sigmoid(g) * u, jnp.where(tot < 0.0, 1.0, 0.0)

    av = []
    start = jnp.zeros((8, 128), f32)
    for c in range(FM, F, CB):
        out, start = vpu_cols(c, start)
        av.append(out)

    y = None
    prev = None
    for c in list(range(0, FM, FC)) + [FM]:
        if c < FM:
            g = jnp.dot(xs, _w16(wgb[:, c:min(c + FC, FM)]), preferred_element_type=f32)
            u = jnp.dot(xs, _w16(wub[:, c:min(c + FC, FM)]), preferred_element_type=f32)
        if prev is not None:
            d = jnp.dot(prev, _w16(wdb[(c - prev.shape[1]) // 2:c // 2, :]), preferred_element_type=f32)
            y = d if y is None else y + d
        if c < FM:
            prev = (g * jax.nn.sigmoid(g) * u).astype(bf16)
        if c == 0:
            gu = jnp.concatenate([g, u], axis=1)
            for gi, r0 in enumerate(range(S - EP, S, 16)):
                gc = gi * (2 * FC // 128) // (EP // 16)
                never = jnp.abs(gu[:, gc * 128:(gc + 1) * 128]) < 0.0
                xx = ob[r0:r0 + 16, :].astype(f32)
                rs = jnp.where(never, 0.0, st_ref[1, r0:r0 + 16, :])
                mb = jnp.where(never, 0.0, st_ref[0, r0:r0 + 16, :])
                ob[r0:r0 + 16, :] = ((xx + bc(7, 16)) + ((xx - _lanes(mb)) * _lanes(rs)) * bc(8, 16)).astype(bf16)
            cp_out(NQB - 1).start()
    for i, a in enumerate(av):
        c = FM + i * CB
        y = y + jnp.dot(a.astype(bf16), _w16(wdb[c // 2:(c + CB) // 2, :]), preferred_element_type=f32)
    upd = jnp.where(_lanes(ids == i1v), y * _lanes(jax.nn.sigmoid(m1)),
                    jnp.where(_lanes(ids == i2v), y * _lanes(jax.nn.sigmoid(m2)), 0.0))
    fixb[...] = ((x1 + bc(7, 16)) + xn * bc(8, 16) + bc(5, 16) * upd).astype(bf16)

    for qb in range(NQB):
        cp_out(qb).wait()
    cf1 = pltpu.make_async_copy(fixb.at[pl.ds(0, 8)], o_hbm.at[pl.ds(b1, 8)], sem_o.at[NQB])
    cf2 = pltpu.make_async_copy(fixb.at[pl.ds(8, 8)], o_hbm.at[pl.ds(b2, 8)], sem_o.at[NQB + 1])
    cf1.start()

    @pl.when(b1 != b2)
    def _():
        cf2.start()
        cf2.wait()
    cf1.wait()


@jax.jit
def pallas_adaLN_cond__mha_block_cached__moe_arch_mod__prompt_kernel(
    A_x: jax.Array,
    A_k_cache: jax.Array,
    A_v_cache: jax.Array,
    A_wq: jax.Array,
    A_wo: jax.Array,
    B_x: jax.Array,
    B_w_r: jax.Array,
    B_w_gate: jax.Array,
    B_w_up: jax.Array,
    B_w_down: jax.Array,
    c: jax.Array,
    w_mod: jax.Array,
):
    x = A_x.reshape(S, D)
    k = A_k_cache.reshape(H * S, DH)
    v = A_v_cache.reshape(H * S, DH)
    wo = A_wo.reshape(NHG, HPS * DH, D)
    anyspec = pl.BlockSpec(memory_space=pl.ANY)
    out = pl.pallas_call(
        _kernel,
        in_specs=[anyspec] * 11,
        out_specs=anyspec,
        out_shape=jax.ShapeDtypeStruct((S, D), bf16),
        scratch_shapes=[
            pltpu.VMEM((S, D), bf16),
            pltpu.VMEM((H * S2, DH), u32),
            pltpu.VMEM((H * S2, DH), u32),
            pltpu.VMEM((NHG, D // 2, HPS * DH), u32),
            pltpu.VMEM((NHG, HPS * DH // 2, D), u32),
            pltpu.VMEM((D // 2, F), u32),
            pltpu.VMEM((D // 2, F), u32),
            pltpu.VMEM((F // 2, D), u32),
            pltpu.VMEM((NMP + 1, D // 2, MPW), u32),
            pltpu.VMEM((8, 11 * D), f32),
            pltpu.VMEM((S // 2, D), u32),
            pltpu.VMEM((S, D), f32),
            pltpu.VMEM((S + CH, D), bf16),
            pltpu.VMEM((16, D), bf16),
            pltpu.VMEM((1, TQ, S), f32),
            pltpu.VMEM((1, TQ, S), f32),
            pltpu.VMEM((TQ // 2, S), u32),
            pltpu.VMEM((TQ // 2, S), u32),
            pltpu.VMEM((1, HPS, TQ, 128), f32),
            pltpu.VMEM((1, TQ, 128), f32),
            pltpu.VMEM((1, TQ, 128), f32),
            pltpu.VMEM((1, TQ, 128), f32),
            pltpu.VMEM((1, TQ, 128), f32),
            pltpu.VMEM((CH // 2, D), u32),
            pltpu.VMEM((TQ, HPS * DH), u32),
            pltpu.VMEM((2, S + CH, 128), f32),
            pltpu.VMEM((D, 128), f32),
            pltpu.VMEM((1, D, 128), u32),
            pltpu.VMEM((NMP + 1, 8, MPW), f32),
            pltpu.VMEM((2, 8, 128), f32),
            pltpu.VMEM((2, 8, 128), jnp.int32),
            pltpu.VMEM((D,), bf16),
            pltpu.VMEM((1, D), bf16),
            pltpu.SMEM((8,), jnp.int32),
            pltpu.SemaphoreType.DMA((2,)),
            pltpu.SemaphoreType.DMA((4,)),
            pltpu.SemaphoreType.DMA((NMC + NMP,)),
            pltpu.SemaphoreType.DMA((NHG,)),
            pltpu.SemaphoreType.DMA((NHG,)),
            pltpu.SemaphoreType.DMA((2 * NHG,)),
            pltpu.SemaphoreType.DMA((3 * HPS,)),
            pltpu.SemaphoreType.DMA((3,)),
            pltpu.SemaphoreType.DMA((NQB + 2,)),
        ],
        compiler_params=pltpu.CompilerParams(vmem_limit_bytes=124 * 1024 * 1024, disable_bounds_checks=True,
                                             disable_semaphore_checks=True),
    )(x, k, v, A_wq, wo, B_w_r, B_w_gate, B_w_up, B_w_down, c, w_mod)
    return out.reshape(1, S, D)
```
